```python
import jax
import jax.numpy as jnp

def _softmax(x, axis=-1):
    return jax.nn.softmax(x, axis=axis)
def _gelu(x):
    return jax.nn.gelu(x, approximate=True)
def _silu(x):
    return jax.nn.silu(x)
def _sigmoid(x):
    return jax.nn.sigmoid(x)
def _layernorm(x, axis=-1, eps=1e-5):
    m = jnp.mean(x, axis=axis, keepdims=True)
    v = jnp.var(x, axis=axis, keepdims=True)
    return (x - m) / jnp.sqrt(v + eps)
def _scatter_add(tgt, idx, src, axis=0):
    return tgt.at[idx].add(src)
def _segment_sum(src, seg, n):
    return jax.ops.segment_sum(src, seg, n)
class _Rng:
    def __init__(self, key):
        self._k = key
    def _next(self):
        self._k, sub = jax.random.split(self._k)
        return sub
    def normal(self, shape):
        return jax.random.normal(self._next(), shape, dtype=jnp.bfloat16)
    def randint(self, lo, hi, shape):
        return jax.random.randint(self._next(), shape, lo, hi, dtype=jnp.int32)
    def uniform(self, shape, lo=0.0, hi=1.0):
        return jax.random.uniform(self._next(), shape, jnp.bfloat16, lo, hi)
    def permutation(self, n):
        return jax.random.permutation(self._next(), n)


kernel_name = 'interleave_layers__sliding_local_dilated__glu_gated_bilinear__prompt'

def setup_inputs():
    _rng = _Rng(jax.random.key(int.from_bytes(__import__("os").urandom(4), "little")))
    _w = (lambda a: (lambda t: t.astype(jnp.bfloat16) if jnp.issubdtype(t.dtype, jnp.floating) else t)(jnp.asarray(a)))
    def _A_setup():
        B, S, D = 1, 2048, 576
        return {
            "x": _w((lambda *s: _rng.normal(s) * 0.05)(B, S, D)),
            "wqkv": _w((lambda *s: _rng.normal(s) * 0.05)(D, 3 * D)),
            "wo": _w((lambda *s: _rng.normal(s) * 0.05)(D, D)),
        }
    _A_in = _A_setup()

    def _B_setup():
        B, S, D, F = 1, 2048, 576, 4608
        return {
            "x": _w((lambda *s: _rng.normal(s) * 0.05)(B, S, D)),
            "w_gate": _w((lambda *s: _rng.normal(s) * 0.05)(D, F) * (D ** -0.5)),
            "w_up": _w((lambda *s: _rng.normal(s) * 0.05)(D, F) * (D ** -0.5)),
            "w_down": _w((lambda *s: _rng.normal(s) * 0.05)(F, D) * (F ** -0.5)),
        }
    _B_in = _B_setup()

    return {
        "A_x": _A_in["x"],
        "A_wqkv": _A_in["wqkv"],
        "A_wo": _A_in["wo"],
        "B_x": _B_in["x"],
        "B_w_gate": _B_in["w_gate"],
        "B_w_up": _B_in["w_up"],
        "B_w_down": _B_in["w_down"],
    }

def reference(A_x, A_wqkv, A_wo, B_x, B_w_gate, B_w_up, B_w_down):
    def _A_ref(x, wqkv, wo):
        B, S, D = x.shape
        H = 32; Dh = D // H
        W, dil = 8, 2
        qkv = (lambda x, *d: x.transpose(*d))((x @ wqkv).reshape(B, S, 3, H, Dh), 2, 0, 3, 1, 4)
        q, k, v = qkv[0], qkv[1], qkv[2]
        scale = Dh ** -0.5
        pos = jnp.arange(S)
        off = jnp.arange(W) * dil
        idx = pos[:, None] - off[None, :]
        mask = idx >= 0
        idx_c = jnp.where(mask, idx, 0).reshape(-1)
        kg = k[:, :, idx_c, :].reshape(B, H, S, W, Dh)
        vg = v[:, :, idx_c, :].reshape(B, H, S, W, Dh)
        logits = jnp.einsum("bhsd,bhswd->bhsw", q, kg) * scale
        logits = jnp.where(mask[None, None, :, :], logits, -1e9)
        attn = _softmax(logits, axis=-1)
        o = jnp.einsum("bhsw,bhswd->bhsd", attn, vg)
        return (lambda x, *d: x.transpose(*d))(o, 0, 2, 1, 3).reshape(B, S, D) @ wo

    def _B_ref(x, w_gate, w_up, w_down):
        g = jnp.einsum("bsd,df->bsf", x, w_gate)
        u = jnp.einsum("bsd,df->bsf", x, w_up)
        h = g * u
        return jnp.einsum("bsf,fd->bsd", h, w_down)

    x = A_x
    x = x + _A_ref(_layernorm(x, axis=-1), A_wqkv, A_wo)
    x = x + _B_ref(_layernorm(x, axis=-1), B_w_gate, B_w_up, B_w_down)
    x = x + _A_ref(_layernorm(x, axis=-1), A_wqkv, A_wo)
    x = x + _B_ref(_layernorm(x, axis=-1), B_w_gate, B_w_up, B_w_down)
    return x
```

```python
import functools
import math

import jax
import jax.numpy as jnp
from jax import lax
import jax.experimental.pallas as pl
import jax.experimental.pallas.tpu as pltpu

S, D, F = 2048, 576, 4608
H, DH, W, DIL = 32, 18, 8, 2
NQ = 14 * 128
HALO = 16
TM = 256
FC = 1152
RB = 32
EPS = 1e-5
bf16, f32, u32 = jnp.bfloat16, jnp.float32, jnp.uint32
NT = (((1,), (1,)), ((), ()))
SCALE = DH ** -0.5
EXP2_C = SCALE * math.log2(math.e)
NEG = -1e9 / SCALE


def _ln_t(xt):
    m = jnp.mean(xt, axis=0, keepdims=True)
    xc = xt - m
    v = jnp.mean(xc * xc, axis=0, keepdims=True)
    return xc * lax.rsqrt(v + EPS)


def _prep_weights(wqkv_ref, wo_ref, wq_ref, wot_ref, t1_ref, t2_ref):
    wp = pltpu.bitcast(wqkv_ref[...], u32)
    wp = jnp.concatenate([wp, jnp.zeros((384 - 288, 3 * D), u32)], axis=0)
    for c in range(3):
        t1_ref[c] = wp[c * 128:(c + 1) * 128, :].T

    def rows(c, t, d):
        return t1_ref[c, pl.ds(t * D + d, H, stride=DH), :]

    outs = []
    for c in range(3):
        parts = []
        for t in range(3):
            parts += [rows(c, t, d) for d in range(16)]
        parts += [rows(c, 0, 16), rows(c, 0, 17), rows(c, 2, 16), rows(c, 2, 17)]
        parts += [rows(c, 1, 16), rows(c, 1, 17), jnp.zeros((64, 128), u32)]
        outs.append(jnp.concatenate(parts, axis=0).T)
    wq = jnp.concatenate(outs, axis=0)[:288]
    wq_ref[...] = pltpu.bitcast(wq, bf16)

    wo = wo_ref[...].astype(f32)
    wo = jnp.concatenate([wo, jnp.zeros((D, 64), f32)], axis=1)
    for c in range(5):
        t2_ref[c] = wo[:, c * 128:(c + 1) * 128]
    outs = []
    for c in range(5):
        parts = [t2_ref[c, pl.ds(d, H, stride=DH), :] for d in range(16)]
        parts += [jnp.zeros((64, 128), f32)]
        parts += [t2_ref[c, pl.ds(d, H, stride=DH), :] for d in (16, 17)]
        outs.append(jnp.concatenate(parts, axis=0).T.astype(bf16))
    wot_ref[...] = jnp.concatenate(outs, axis=0)[:D]


def _kernel(xt_ref, wqkv_ref, wo_ref, wg_ref, wu_ref, wdt_ref, o_ref,
            wq_ref, wot_ref, t1_ref, t2_ref, qkv_ref, att_ref):
    i = pl.program_id(0)

    @pl.when(i == 0)
    def _():
        _prep_weights(wqkv_ref, wo_ref, wq_ref, wot_ref, t1_ref, t2_ref)

    xt = xt_ref[...].astype(f32)
    for layer in range(2):
        buf = qkv_ref.at[layer]
        xn = _ln_t(xt).T.astype(bf16)
        qkv = jnp.dot(xn, wq_ref[...], preferred_element_type=f32)

        @pl.when(i > 0)
        def _():
            for c in range(4, 14):
                buf[c, 0:HALO, :] = buf[c, TM:TM + HALO, :]

        for c in range(14):
            buf[c, HALO:HALO + TM, :] = qkv[:, c * 128:(c + 1) * 128]

        @pl.when(i == 0)
        def _():
            for c in range(4, 14):
                buf[c, 0:HALO, :] = jnp.broadcast_to(buf[c, HALO:HALO + 1, :], (HALO, 128))

        qi = (0, 1, 2, 3, 12)
        ki = (4, 5, 6, 7, 13)
        vi = (8, 9, 10, 11, 12)

        def body(j, _):
            r0 = pl.multiple_of(j * RB, RB)
            pos = i * TM + r0 + lax.broadcasted_iota(jnp.int32, (RB, 128), 0)
            q = [buf[c, pl.ds(r0 + HALO, RB), :] for c in qi]
            ls = []
            for w in range(W):
                acc = None
                for c in range(5):
                    t = q[c] * buf[ki[c], pl.ds(r0 + HALO - DIL * w, RB), :]
                    acc = t if acc is None else acc + t
                acc = acc + pltpu.roll(acc, 64, 1)
                acc = acc + pltpu.roll(acc, 32, 1)
                if w > 0:
                    acc = jnp.where(pos >= DIL * w, acc, NEG)
                ls.append(acc)
            m = functools.reduce(jnp.maximum, ls)
            ps = [jnp.exp2((l - m) * EXP2_C) for l in ls]
            inv = 1.0 / functools.reduce(jnp.add, ps)
            for c in range(5):
                acc = None
                for w in range(W):
                    t = ps[w] * buf[vi[c], pl.ds(r0 + HALO - DIL * w, RB), :]
                    acc = t if acc is None else acc + t
                att_ref[pl.ds(r0, RB), c * 128:(c + 1) * 128] = (acc * inv).astype(bf16)
            return 0

        lax.fori_loop(0, TM // RB, body, 0)
        xt = xt + lax.dot_general(wot_ref[...], att_ref[...], NT, preferred_element_type=f32)

        xn = _ln_t(xt).T.astype(bf16)
        acc = xt
        for c in range(F // FC):
            g = jnp.dot(xn, wg_ref[:, c * FC:(c + 1) * FC], preferred_element_type=f32)
            u = jnp.dot(xn, wu_ref[:, c * FC:(c + 1) * FC], preferred_element_type=f32)
            h = (g * u).astype(bf16)
            acc = acc + lax.dot_general(wdt_ref[:, c * FC:(c + 1) * FC], h, NT, preferred_element_type=f32)
        xt = acc
    o_ref[...] = xt.astype(bf16)


@jax.jit
def pallas_interleave_layers__sliding_local_dilated__glu_gated_bilinear__prompt_kernel(
    A_x, A_wqkv, A_wo, B_x, B_w_gate, B_w_up, B_w_down):
    xt = A_x[0].T
    wdt = B_w_down.T
    whole = lambda shape: pl.BlockSpec(shape, lambda i: (0, 0), pipeline_mode=pl.Buffered(1))
    out_t = pl.pallas_call(
        _kernel,
        grid=(S // TM,),
        in_specs=[pl.BlockSpec((D, TM), lambda i: (0, i)),
                  whole((D, 3 * D)), whole((D, D)), whole((D, F)), whole((D, F)), whole((D, F))],
        out_specs=pl.BlockSpec((D, TM), lambda i: (0, i)),
        out_shape=jax.ShapeDtypeStruct((D, S), bf16),
        scratch_shapes=[
            pltpu.VMEM((D, NQ), bf16),
            pltpu.VMEM((D, 640), bf16),
            pltpu.VMEM((3, 3 * D, 128), u32),
            pltpu.VMEM((5, D, 128), f32),
            pltpu.VMEM((2, 14, HALO + TM, 128), f32),
            pltpu.VMEM((TM, 640), bf16),
        ],
        compiler_params=pltpu.CompilerParams(dimension_semantics=("arbitrary",),
                                             vmem_limit_bytes=100 * 1024 * 1024),
    )(xt, A_wqkv, A_wo, B_w_gate, B_w_up, wdt)
    return out_t.T[None]
```

```python
import functools
import math

import jax
import jax.numpy as jnp
from jax import lax
import jax.experimental.pallas as pl
import jax.experimental.pallas.tpu as pltpu

S, D, F = 2048, 576, 4608
H, DH, W, DIL = 32, 18, 8, 2
NQ = 14 * 128
HALO = 16
TA = 256
TF = 512
FI = 2304
HI = FI // 2
HE = 384
RB = 32
NA = S // TA
NSTEP = 2 * NA
LAG = TF // TA
EPS = 1e-5
bf16, f32, u32, i32 = jnp.bfloat16, jnp.float32, jnp.uint32, jnp.int32
NT = (((1,), (1,)), ((), ()))
SCALE = DH ** -0.5
EXP2_C = SCALE * math.log2(math.e)
NEG = -1e9 / SCALE

dot = functools.partial(jnp.dot, preferred_element_type=f32)


def dnt(a, b):
    return lax.dot_general(a, b, NT, preferred_element_type=f32)


def cat0(*xs):
    return jnp.concatenate(xs, axis=0)


def cat1(*xs):
    return jnp.concatenate(xs, axis=1)


def addb(a, b):
    return (a.astype(f32) + b.astype(f32)).astype(bf16)


def subb(a, b):
    return (a.astype(f32) - b.astype(f32)).astype(bf16)


def tb(x):
    return x.T.astype(bf16)


def _ln_t(xt):
    m = jnp.mean(xt, axis=0, keepdims=True)
    xc = xt - m
    v = jnp.mean(xc * xc, axis=0, keepdims=True)
    return xc * lax.rsqrt(v + EPS)


def _share_dot(p1, p2, ps, w):
    k = w.shape[0]
    a, b = k - 128, k - 64
    s = dot(ps, w[a:])
    return dot(p1, w[:b]) + s, dot(p2, cat0(w[:a], w[b:])) + s


def _prep_wqkv(wqkv_ref, wq_ref, t1_ref):
    wp = pltpu.bitcast(wqkv_ref[...], u32)
    wp = cat0(wp, jnp.zeros((384 - 288, 3 * D), u32))
    for c in range(3):
        t1_ref[c] = wp[c * 128:(c + 1) * 128, :].T

    def rows(c, t, d):
        return t1_ref[c, pl.ds(t * D + d, H, stride=DH), :]

    outs = []
    for c in range(3):
        parts = []
        for t in range(3):
            parts += [rows(c, t, d) for d in range(16)]
        parts += [rows(c, 0, 16), rows(c, 0, 17), rows(c, 2, 16), rows(c, 2, 17)]
        parts += [rows(c, 1, 16), rows(c, 1, 17), jnp.zeros((64, 128), u32)]
        outs.append(cat0(*parts).T)
    wq_ref[...] = pltpu.bitcast(cat0(*outs)[:288], bf16)


def _prep_wo(wo_ref, wot_ref, t2_ref):
    wo = cat1(wo_ref[...].astype(f32), jnp.zeros((D, 64), f32))
    for c in range(5):
        t2_ref[c] = wo[:, c * 128:(c + 1) * 128]
    outs = []
    for c in range(5):
        parts = [t2_ref[c, pl.ds(d, H, stride=DH), :] for d in range(16)]
        parts += [jnp.zeros((64, 128), f32)]
        parts += [t2_ref[c, pl.ds(d, H, stride=DH), :] for d in (16, 17)]
        outs.append(tb(cat0(*parts)))
    wot_ref[...] = cat0(*outs)[:D]


def _attn_qkv(s, xt, wq_ref, qkv_ref):
    item = s % NA
    t0 = pl.multiple_of(item * TA, TA)
    hf = TA // 2

    z = _ln_t(xt)
    z1, z2 = z[:, :hf], z[:, hf:]
    p1 = tb(cat0(z1[:448], z1[448:512] - z2[448:512]))
    p2 = tb(cat0(z2[:448], z2[512:] - z1[512:]))
    ps = tb(cat0(z2[448:512], z1[512:]))
    c1, c2 = _share_dot(p1, p2, ps, wq_ref[...])
    for c in range(14):
        qkv_ref[c, pl.ds(t0 + HALO, hf), :] = c1[:, c * 128:(c + 1) * 128]
        qkv_ref[c, pl.ds(t0 + HALO + hf, hf), :] = c2[:, c * 128:(c + 1) * 128]
    hrow = pl.multiple_of(jnp.where(item == 0, 0, S + HALO), HALO)
    for c in range(4, 14):
        qkv_ref[c, pl.ds(hrow, HALO), :] = jnp.broadcast_to(c1[0:1, c * 128:(c + 1) * 128], (HALO, 128))


def _attn_core(s, qkv_ref):
    t0 = pl.multiple_of((s % NA) * TA, TA)
    qi = (0, 1, 2, 3, 12)
    ki = (4, 5, 6, 7, 13)
    vi = (8, 9, 10, 11, 12)
    att = []
    for j in range(TA // RB):
        r0 = t0 + (j * RB + HALO)
        q = [qkv_ref[c, pl.ds(r0, RB), :] for c in qi]
        ls = []
        for w in range(W):
            acc = None
            for c in range(5):
                t = q[c] * qkv_ref[ki[c], pl.ds(r0 - DIL * w, RB), :]
                acc = t if acc is None else acc + t
            acc = acc + pltpu.roll(acc, 64, 1)
            acc = acc + pltpu.roll(acc, 32, 1)
            if w > 0 and j == 0:
                pos = t0 + lax.broadcasted_iota(i32, (HALO, 128), 0)
                top = jnp.where(pos >= DIL * w, acc[:HALO], NEG)
                acc = top if RB == HALO else cat0(top, acc[HALO:])
            ls.append(acc)
        m = functools.reduce(jnp.maximum, ls)
        pr = [jnp.exp2((l - m) * EXP2_C) for l in ls]
        inv = 1.0 / functools.reduce(jnp.add, pr)
        outs = []
        for c in range(5):
            acc = None
            for w in range(W):
                t = pr[w] * qkv_ref[vi[c], pl.ds(r0 - DIL * w, RB), :]
                acc = t if acc is None else acc + t
            outs.append((acc * inv).astype(bf16))
        att.append(cat1(*outs))
    return cat0(*att)


def _attn_post(s, xt, att, x_ref, wot_ref, lm_ref, lp_ref, ls_ref):
    t0 = pl.multiple_of((s % NA) * TA, TA)
    hf = TA // 2
    xt = xt + dnt(wot_ref[...], att)
    x_ref[:, pl.ds(t0, TA)] = xt

    z = _ln_t(xt)
    a11, a12, r1 = z[:256, :hf], z[256:512, :hf], z[512:, :hf]
    a21, a22, r2 = z[:256, hf:], z[256:512, hf:], z[512:, hf:]
    par = (s // LAG) % 2
    sub = s % LAG
    rm = pl.ds(pl.multiple_of(sub * hf, hf), hf)
    for n, v in enumerate((a11 + a22, a11, a22)):
        lm_ref[par, n, rm, :] = tb(v)
    lo = lax.broadcasted_iota(i32, (64, hf), 1) < 64
    q4 = hf // 2
    rq = pl.ds(pl.multiple_of(sub * q4, q4), q4)
    sh = []
    for n, (zm, zc) in enumerate(((a21 + a22, r2), (a11 + a12, r1), (a21 - a11, r2), (a12 - a22, r1))):
        zb = zm[192:]
        zbr = pltpu.roll(zb, 64, 1)
        zcr = pltpu.roll(zc, 64, 1)
        p = tb(cat0(zm[:192], jnp.where(lo, zb - zbr, zc - zcr)))
        lp_ref[par, 2 * n, rq, :] = p[:q4]
        lp_ref[par, 2 * n + 1, rq, :] = p[q4:]
        sh.append((zb, zbr, zc, zcr))
    for n in (0, 2):
        (_, zbr0, zc0, _), (zb1, _, _, zcr1) = sh[n], sh[n + 1]
        p = tb(cat0(jnp.where(lo, zbr0, zb1), jnp.where(lo, zc0, zcr1)))
        ls_ref[par, n, rq, :] = p[:q4]
        ls_ref[par, n + 1, rq, :] = p[q4:]


def _load_lhs(f, lm_ref, lp_ref, ls_ref):
    par = (f // LAG) % 2
    return ([lm_ref[par, n] for n in range(3)], [lp_ref[par, n] for n in range(8)],
            [ls_ref[par, n] for n in range(4)])


def _gu(lhs, w1, w2):
    lm, lp, ls = lhs
    q4 = TA // 4

    def share(n, w):
        c1, c2 = _share_dot(lp[2 * n], lp[2 * n + 1], ls[n], w)
        parts = []
        for a in range(LAG):
            parts += [c1[a * q4:(a + 1) * q4], c2[a * q4:(a + 1) * q4]]
        return cat0(*parts)

    b11, b21, r1 = w1[:256], w1[256:512], w1[512:]
    b12, b22 = w2[:256], w2[256:512]
    ws = addb(w1, w2)
    m1 = dot(lm[0], addb(b11, b22))
    m3 = dot(lm[1], subb(b12, b22))
    m4 = dot(lm[2], subb(b21, b11))
    m2 = share(0, cat0(b11, r1))
    m5 = share(1, w2[256:])
    m6 = share(2, cat0(ws[:256], ws[512:]))
    m7 = share(3, ws[256:])
    return m1 + m4 - m5 + m7, m3 + m5, m2 + m4, m1 - m2 + m3 + m6


def _cols(c, hw):
    o1 = pl.multiple_of(c * (2 * hw), 128)
    return pl.ds(o1, hw), pl.ds(pl.multiple_of(o1 + hw, 128), hw)


def _ffn_proj(sl, lhs, w_ref):
    return _gu(lhs, w_ref[:, sl[0]], w_ref[:, sl[1]])


def _ffn_down(f, sl, hs, wdt_ref, x_ref, ob_ref, mid=None):
    sl1, sl2 = sl
    d1, d2 = wdt_ref[:, sl1], wdt_ref[:, sl2]
    a11, a21 = d1[:288], d1[288:]
    a12, a22 = d2[:288], d2[288:]
    b11, b21, b12, b22 = hs
    c = lambda x: x.astype(bf16)
    m1 = dnt(addb(a11, a22), c(b11 + b22))
    m2 = dnt(addb(a21, a22), c(b11))
    m3 = dnt(a11, c(b12 - b22))
    m4 = dnt(a22, c(b21 - b11))
    m5 = dnt(addb(a11, a12), c(b22))
    if mid is not None:
        mid()
    m6 = dnt(subb(a21, a11), c(b11 + b12))
    m7 = dnt(subb(a12, a22), c(b21 + b22))
    tok1 = cat0(m1 + m4 - m5 + m7, m2 + m4)
    tok2 = cat0(m3 + m5, m1 - m2 + m3 + m6)
    hf = TA // 2
    parts = []
    for a in range(LAG):
        parts += [tok1[:, a * hf:(a + 1) * hf], tok2[:, a * hf:(a + 1) * hf]]
    c0 = ((f // LAG) % (S // TF)) * TF
    cols = pl.ds(c0 if isinstance(c0, int) else pl.multiple_of(c0, TF), TF)
    xn = x_ref[:, cols] + cat1(*parts)
    x_ref[:, cols] = xn
    ob_ref[:, cols] = xn.astype(bf16)


def _kernel(xt_hbm, wqkv_hbm, wo_hbm, wg_hbm, wu_hbm, wdt_hbm, o_hbm,
            xb_ref, wqkv_ref, wo_ref, wg_ref, wu_ref, wdt_ref,
            wq_ref, wot_ref, t1_ref, t2_ref, x_ref, qkv_ref, lm_ref, lp_ref, ls_ref, ob_ref,
            sem_in, sem_w, sem_out):
    cp_x0 = pltpu.make_async_copy(xt_hbm.at[:, pl.ds(0, TF)], xb_ref.at[:, pl.ds(0, TF)], sem_in.at[0])
    cp_wqkv = pltpu.make_async_copy(wqkv_hbm, wqkv_ref, sem_in.at[1])
    cp_wo = pltpu.make_async_copy(wo_hbm, wo_ref, sem_in.at[2])
    cp_x1 = pltpu.make_async_copy(xt_hbm.at[:, pl.ds(TF, S - TF)], xb_ref.at[:, pl.ds(TF, S - TF)], sem_in.at[3])

    def cp_w(half, n):
        src, dst = ((wg_hbm, wg_ref), (wu_hbm, wu_ref), (wdt_hbm, wdt_ref))[n]
        sl = pl.ds(half * FI, FI)
        return pltpu.make_async_copy(src.at[:, sl], dst.at[:, sl], sem_w.at[half * 3 + n])

    def cp_out(t):
        sl = pl.ds(t * TF if isinstance(t, int) else pl.multiple_of(t * TF, TF), TF)
        return pltpu.make_async_copy(ob_ref.at[:, sl], o_hbm.at[:, sl], sem_out.at[t])

    cp_wqkv.start()
    cp_wqkv.wait()
    cp_x0.start()
    cp_wo.start()
    _prep_wqkv(wqkv_ref, wq_ref, t1_ref)
    cp_x0.wait()
    cp_wo.wait()
    cp_x1.start()
    for n in range(3):
        cp_w(0, n).start()
    _prep_wo(wo_ref, wot_ref, t2_ref)

    def pro(s, carry):
        xt = xb_ref[:, pl.ds(pl.multiple_of(s * TA, TA), TA)].astype(f32)
        _attn_qkv(s, xt, wq_ref, qkv_ref)
        att = _attn_core(s, qkv_ref)
        _attn_post(s, xt, att, x_ref, wot_ref, lm_ref, lp_ref, ls_ref)
        return carry

    lax.fori_loop(0, LAG, pro, 0)
    cp_x1.wait()
    for n in range(3):
        cp_w(1, n).start()
    x_ref[:, TF:] = xb_ref[:, TF:].astype(f32)

    def wait_weights(f):
        for half in range(LAG):
            @pl.when(f == half)
            def _():
                for n in range(3):
                    cp_w(half, n).wait()

    def start_out(f):
        @pl.when(jnp.logical_and(f >= NA, f % LAG == LAG - 1))
        def _():
            cp_out((f - NA) // LAG).start()

    def fused(s, carry):
        f = s - LAG
        wait_weights(f)
        xt = x_ref[:, pl.ds(pl.multiple_of((s % NA) * TA, TA), TA)]
        lhs = _load_lhs(f, lm_ref, lp_ref, ls_ref)
        sl = _cols(f % LAG, HI)
        g = _ffn_proj(sl, lhs, wg_ref)
        u = _ffn_proj(sl, lhs, wu_ref)
        _attn_qkv(s, xt, wq_ref, qkv_ref)
        att = _attn_core(s, qkv_ref)
        hs = [a * b for a, b in zip(g, u)]
        _ffn_down(f, sl, hs, wdt_ref, x_ref, ob_ref,
                  mid=lambda: _attn_post(s, xt, att, x_ref, wot_ref, lm_ref, lp_ref, ls_ref))
        start_out(f)
        return carry

    lax.fori_loop(LAG, NSTEP, fused, 0)

    def epi(c, carry):
        f = NSTEP - 1
        sl = _cols(c, HE)
        lhs = _load_lhs(f, lm_ref, lp_ref, ls_ref)
        hs = [a * b for a, b in zip(_ffn_proj(sl, lhs, wg_ref), _ffn_proj(sl, lhs, wu_ref))]
        _ffn_down(f, sl, hs, wdt_ref, x_ref, ob_ref)
        return carry

    lax.fori_loop(0, F // (2 * HE), epi, 0)
    cp_out(S // TF - 1).start()
    for t in range(S // TF):
        cp_out(t).wait()


@jax.jit
def pallas_interleave_layers__sliding_local_dilated__glu_gated_bilinear__prompt_kernel(
    A_x, A_wqkv, A_wo, B_x, B_w_gate, B_w_up, B_w_down):
    xt = A_x[0].T
    wdt = B_w_down.T
    hbm = pl.BlockSpec(memory_space=pl.ANY)
    out_t = pl.pallas_call(
        _kernel,
        in_specs=[hbm] * 6,
        out_specs=hbm,
        out_shape=jax.ShapeDtypeStruct((D, S), bf16),
        scratch_shapes=[
            pltpu.VMEM((D, S), bf16),
            pltpu.VMEM((D, 3 * D), bf16),
            pltpu.VMEM((D, D), bf16),
            pltpu.VMEM((D, F), bf16),
            pltpu.VMEM((D, F), bf16),
            pltpu.VMEM((D, F), bf16),
            pltpu.VMEM((D, NQ), bf16),
            pltpu.VMEM((D, 640), bf16),
            pltpu.VMEM((3, 3 * D, 128), u32),
            pltpu.VMEM((5, D, 128), f32),
            pltpu.VMEM((D, S), f32),
            pltpu.VMEM((14, S + 2 * HALO, 128), f32),
            pltpu.VMEM((2, 3, TF // 2, 256), bf16),
            pltpu.VMEM((2, 8, TF // 4, 256), bf16),
            pltpu.VMEM((2, 4, TF // 4, 128), bf16),
            pltpu.VMEM((D, S), bf16),
            pltpu.SemaphoreType.DMA((4,)),
            pltpu.SemaphoreType.DMA((3 * LAG,)),
            pltpu.SemaphoreType.DMA((S // TF,)),
        ],
        compiler_params=pltpu.CompilerParams(vmem_limit_bytes=110 * 1024 * 1024),
    )(xt, A_wqkv, A_wo, B_w_gate, B_w_up, wdt)
    return out_t.T[None]
```

```python
import functools
import math

import jax
import jax.numpy as jnp
from jax import lax
import jax.experimental.pallas as pl
import jax.experimental.pallas.tpu as pltpu

S, D, F = 2048, 576, 4608
H, DH, W, DIL = 32, 18, 8, 2
NQ = 14 * 128
HALO = 16
QROWS = S + 2 * HALO + 8
TA = 256
TF = 512
FH = F // 2
CW = 384
NCK = FH // CW
LAG = TF // TA
CPI = NCK // LAG
NCH = 2
RB = 32
SB = 64
NA = S // TA
NSTEP = 2 * NA
EPS = 1e-5
bf16, f32, u32, i32 = jnp.bfloat16, jnp.float32, jnp.uint32, jnp.int32
NT = (((1,), (1,)), ((), ()))
SCALE = DH ** -0.5
EXP2_C = SCALE * math.log2(math.e)
NEG = -1e9 / SCALE

dot = functools.partial(jnp.dot, preferred_element_type=f32)


def dnt(a, b):
    return lax.dot_general(a, b, NT, preferred_element_type=f32)


def cat0(*xs):
    return xs[0] if len(xs) == 1 else jnp.concatenate(xs, axis=0)


def cat1(*xs):
    return xs[0] if len(xs) == 1 else jnp.concatenate(xs, axis=1)


def tb(x):
    return x.T.astype(bf16)


def pkb(x):
    return pltpu.bitcast(x.astype(bf16), u32)


def pkt(x):
    return pltpu.bitcast(tb(x), u32)


def up(x):
    return pltpu.bitcast(x, bf16)


def _chain_sum(load, fn):
    acc = None
    for r in range(0, D, 8 * NCH):
        t = fn(load(r, 8 * NCH))
        acc = t if acc is None else acc + t
    return jnp.sum(acc, axis=0, keepdims=True)


def _ln_t(load, m=None):
    if m is None:
        m = _chain_sum(load, lambda v: v) * (1.0 / D)
    r = lax.rsqrt(_chain_sum(load, lambda v: (v - m) * (v - m)) * (1.0 / D) + EPS)
    return load(0, D) * r - m * r


def _prep_wqkv(c, wqkv_ref, wq_ref, t1_ref):
    n = min(256, D - 256 * c)
    wp = pltpu.bitcast(wqkv_ref[256 * c:256 * c + n, :], u32)
    if n < 256:
        wp = cat0(wp, jnp.zeros(((256 - n) // 2, 3 * D), u32))
    t1_ref[c] = wp.T

    def rows(t, d):
        return t1_ref[c, pl.ds(t * D + d, H, stride=DH), :]

    parts = []
    for t in range(3):
        parts += [rows(t, d) for d in range(16)]
    parts += [rows(0, 16), rows(0, 17), rows(2, 16), rows(2, 17)]
    parts += [rows(1, 16), rows(1, 17), jnp.zeros((64, 128), u32)]
    wq_ref[128 * c:128 * c + n // 2, :] = cat0(*parts).T[:n // 2]


def _prep_wo(wo_ref, wot_ref, t2_ref):
    wo = cat1(wo_ref[...].astype(f32), jnp.zeros((D, 64), f32))
    for c in range(5):
        t2_ref[c] = wo[:, c * 128:(c + 1) * 128]
    for c in range(5):
        parts = [t2_ref[c, pl.ds(d, H, stride=DH), :] for d in range(16)]
        parts += [jnp.zeros((64, 128), f32)]
        parts += [t2_ref[c, pl.ds(d, H, stride=DH), :] for d in (16, 17)]
        wot_ref[64 * c:64 * c + 64, :] = pkt(cat0(*parts))


def _attn_lhs(s, x_ref, wq_ref):
    hf = TA // 2
    item = s % NA
    z = _ln_t(lambda r, n: x_ref[item, r:r + n, :])
    z1, z2 = z[:, :hf], z[:, hf:]
    p1 = tb(cat0(z1[:448], z1[448:512] - z2[448:512]))
    p2 = tb(cat0(z2[:448], z2[512:] - z1[512:]))
    ps = tb(cat0(z2[448:512], z1[512:]))
    return p1, p2, dot(ps, up(wq_ref[224:, :]))


def _attn_proj(s, j, lhs, wq_ref, qkv_ref):
    item = s % NA
    t0 = pl.multiple_of(item * TA, TA)
    p1, p2, sh = lhs
    nb = TA // 2 // SB
    r = slice((j % nb) * SB, (j % nb + 1) * SB)
    if j < nb:
        y = dot(p1[r], up(wq_ref[:256, :])) + sh[r]
    else:
        y = dot(p2[r], up(cat0(wq_ref[:224, :], wq_ref[256:, :]))) + sh[r]
    for c in range(14):
        qkv_ref[c, pl.ds(t0 + (HALO + j * SB), SB), :] = y[:, c * 128:(c + 1) * 128]
    if j == 0:
        hrow = pl.multiple_of(jnp.where(item == 0, 0, S + HALO), HALO)
        for c in range(4, 14):
            qkv_ref[c, pl.ds(hrow, HALO), :] = jnp.broadcast_to(y[0:1, c * 128:(c + 1) * 128], (HALO, 128))


def _attn_core(s, j, qkv_ref):
    t0 = pl.multiple_of((s % NA) * TA, TA)
    qi = (0, 1, 2, 3, 12)
    ki = (4, 5, 6, 7, 13)
    vi = (8, 9, 10, 11, 12)
    att = []
    for b in range(SB // RB):
        r0 = t0 + (j * SB + b * RB + HALO)
        q = [qkv_ref[c, pl.ds(r0, RB), :] for c in qi]
        ls = []
        for w in range(W):
            acc = None
            for c in range(5):
                t = q[c] * qkv_ref[ki[c], pl.ds(r0 - DIL * w, RB), :]
                acc = t if acc is None else acc + t
            acc = acc + pltpu.roll(acc, 64, 1)
            acc = acc + pltpu.roll(acc, 32, 1)
            if w > 0 and j == 0 and b == 0:
                pos = t0 + lax.broadcasted_iota(i32, (HALO, 128), 0)
                top = jnp.where(pos >= DIL * w, acc[:HALO], NEG)
                acc = top if RB == HALO else cat0(top, acc[HALO:])
            ls.append(acc)
        m = functools.reduce(jnp.maximum, ls)
        pr = [jnp.exp2((l - m) * EXP2_C) for l in ls]
        inv = 1.0 / functools.reduce(jnp.add, pr)
        outs = []
        for c in range(5):
            acc = None
            for w in range(W):
                t = pr[w] * qkv_ref[vi[c], pl.ds(r0 - DIL * w, RB), :]
                acc = t if acc is None else acc + t
            outs.append(acc * inv)
        att.append(cat1(*outs))
    return cat0(*att)


def _attn_post(s, att, x_ref, wot_ref, lm_ref):
    item = s % NA
    hf = TA // 2
    xt = x_ref[item] + dnt(up(wot_ref[:D // 2, :]), att.astype(bf16))
    x_ref[item] = xt
    m = _chain_sum(lambda r, n: xt[r:r + n], lambda v: v) * (1.0 / D)
    z = _ln_t(lambda r, n: x_ref[item, r:r + n, :], m)
    a11, a12, r1 = z[:256, :hf], z[256:512, :hf], z[512:, :hf]
    a21, a22, r2 = z[:256, hf:], z[256:512, hf:], z[512:, hf:]
    par = (s // LAG) % 2
    sub = s % LAG
    for n, v in enumerate((a11 + a22, a11, a22)):
        lm_ref.at[par, sub, n][...] = pkt(v)
    lo = lax.broadcasted_iota(i32, (64, hf), 1) < 64
    sh = []
    for n, (zm, zc) in enumerate(((a21 + a22, r2), (a11 + a12, r1), (a21 - a11, r2), (a12 - a22, r1))):
        zb = zm[192:]
        zbr = pltpu.roll(zb, 64, 1)
        zcr = pltpu.roll(zc, 64, 1)
        lm_ref.at[par, sub, 3 + n][...] = pkt(cat0(zm[:192], jnp.where(lo, zb - zbr, zc - zcr)))
        sh.append((zb, zbr, zc, zcr))
    ps = []
    for n in (0, 2):
        (_, zbr0, zc0, _), (zb1, _, _, zcr1) = sh[n], sh[n + 1]
        ps += [jnp.where(lo, zbr0, zb1), jnp.where(lo, zc0, zcr1)]
    lm_ref.at[par, sub, 7][...] = pkt(cat0(*ps))


def _load_lhs(f, lm_ref):
    par = (f // LAG) % 2
    q8 = TA // 8

    def ld(n, rows, cols):
        return up(cat0(*[lm_ref[par, a, n, rows, cols] for a in range(LAG)]))

    full, top, bot = slice(None), slice(0, q8), slice(q8, 2 * q8)
    lm = [ld(n, full, full) for n in range(3)]
    lp = [ld(3 + n // 2, (top, bot)[n % 2], full) for n in range(8)]
    ls = [ld(7, (top, bot)[n % 2], slice(128 * (n // 2), 128 * (n // 2) + 128)) for n in range(4)]
    return lm, lp, ls


def _pair(ref, r, ck, o, w):
    rows = pl.ds(pl.multiple_of(r, 32), 32)
    c = pl.multiple_of(ck * CW + o, 128)
    return (ref[rows, pl.ds(c, w)].astype(f32),
            ref[rows, pl.ds(pl.multiple_of(c + FH, 128), w)].astype(f32))


_PIECES = ((0, 256), (256, 128))


def _combine_proj(c0, w_ref, c_ref):
    def main(j, carry):
        r = j * 32
        rows = pl.ds(pl.multiple_of(j * 16, 16), 16)
        for k in range(CPI):
            for o, w in _PIECES:
                (b11, b12), (b21, b22) = _pair(w_ref, r, c0 + k, o, w), _pair(w_ref, r + 256, c0 + k, o, w)
                for n, v in enumerate((b11 + b22, b12 - b22, b21 - b11, b11, b22, b11 + b12, b21 + b22)):
                    c_ref.at[c0 + k, n][rows, o:o + w] = pkb(v)
        return carry

    def rem(j, carry):
        rows = pl.ds(pl.multiple_of(128 + j * 16, 16), 16)
        for k in range(CPI):
            r1, r2 = _pair(w_ref, 512 + j * 32, c0 + k, 0, CW)
            rs = pkb(r1 + r2)
            for n, v in ((3, pkb(r1)), (4, pkb(r2)), (5, rs), (6, rs)):
                c_ref.at[c0 + k, n][rows, :] = v
        return carry

    lax.fori_loop(0, 8, main, 0)
    lax.fori_loop(0, 2, rem, 0)


def _combine_down(c0, wdt_ref, cd_ref):
    def body(j, carry):
        r = j * 32
        rows = pl.ds(pl.multiple_of(j * 16, 16), 16)
        for k in range(CPI):
            for o, w in _PIECES:
                (a11, a12), (a21, a22) = _pair(wdt_ref, r, c0 + k, o, w), _pair(wdt_ref, r + 288, c0 + k, o, w)
                for n, v in enumerate((a11 + a22, a21 + a22, a11, a22, a11 + a12, a21 - a11, a12 - a22)):
                    cd_ref.at[c0 + k, n][rows, o:o + w] = pkb(v)
        return carry

    lax.fori_loop(0, 9, body, 0)


def _wload(c_ref, c0, nck, n, *rows):
    return up(cat1(*[cat0(*[c_ref[c0 + k, n, a:b, :] for a, b in rows]) for k in range(nck)]))


def _ffn_proj(c0, nck, lhs, c_ref):
    lm, lp, ls = lhs
    q4 = TA // 4
    wl = functools.partial(_wload, c_ref, c0, nck)

    def share(n):
        s = dot(ls[n], wl(3 + n, (96, 160)))
        c1 = dot(lp[2 * n], wl(3 + n, (0, 128))) + s
        c2 = dot(lp[2 * n + 1], wl(3 + n, (0, 96), (128, 160))) + s
        parts = []
        for a in range(LAG):
            parts += [c1[a * q4:(a + 1) * q4], c2[a * q4:(a + 1) * q4]]
        return cat0(*parts)

    m1 = dot(lm[0], wl(0, (0, 128)))
    m3 = dot(lm[1], wl(1, (0, 128)))
    m4 = dot(lm[2], wl(2, (0, 128)))
    m2 = share(0)
    m5 = share(1)
    m6 = share(2)
    m7 = share(3)
    return m1 + m4 - m5 + m7, m3 + m5, m2 + m4, m1 - m2 + m3 + m6


def _ffn_down(f, c0, nck, hs, cd_ref, x_ref, ob_ref, mid=lambda k: None):
    b11, b21, b12, b22 = hs
    rhs = (lambda: b11 + b22, lambda: b11, lambda: b12 - b22, lambda: b21 - b11,
           lambda: b22, lambda: b11 + b12, lambda: b21 + b22)
    ms = []
    for n in range(7):
        mid(n)
        ms.append(dnt(_wload(cd_ref, c0, nck, n, (0, 144)), rhs[n]().astype(bf16)))
    m1, m2, m3, m4, m5, m6, m7 = ms
    tok1 = cat0(m1 + m4 - m5 + m7, m2 + m4)
    tok2 = cat0(m3 + m5, m1 - m2 + m3 + m6)
    hf = TA // 2
    tile = (f // LAG) % (S // TF)
    for a in range(LAG):
        it = tile * LAG + a
        xn = x_ref[it] + cat1(tok1[:, a * hf:(a + 1) * hf], tok2[:, a * hf:(a + 1) * hf])
        x_ref[it] = xn
        ob_ref[it] = xn.astype(bf16)


def _kernel(xt_hbm, wqkv_hbm, wo_hbm, wg_hbm, wu_hbm, wdt_hbm, o_hbm,
            xb_ref, wqkv_ref, wo_ref, wg_ref, wu_ref, wdt_ref,
            cg_ref, cu_ref, cd_ref, wq_ref, wot_ref, t1_ref, t2_ref, x_ref, qkv_ref,
            lm_ref, ob_ref, sem_in, sem_w, sem_out):
    def cp_wqkv(c):
        rows = pl.ds(256 * c, min(256, D - 256 * c))
        return pltpu.make_async_copy(wqkv_hbm.at[rows], wqkv_ref.at[rows], sem_in.at[c])

    cp_x0 = pltpu.make_async_copy(xt_hbm.at[:, pl.ds(0, TF)], xb_ref.at[:, pl.ds(0, TF)], sem_in.at[3])
    cp_wo = pltpu.make_async_copy(wo_hbm, wo_ref, sem_in.at[4])
    cp_x1 = pltpu.make_async_copy(xt_hbm.at[:, pl.ds(TF, S - TF)], xb_ref.at[:, pl.ds(TF, S - TF)], sem_in.at[5])

    def cp_w(half, n):
        src, dst = ((wg_hbm, wg_ref), (wu_hbm, wu_ref), (wdt_hbm, wdt_ref))[n // 2]
        sl = pl.ds((n % 2) * FH + half * CPI * CW, CPI * CW)
        return pltpu.make_async_copy(src.at[:, sl], dst.at[:, sl], sem_w.at[half * 6 + n])

    def cp_out(it):
        o = it * TA
        sl = pl.ds(o if isinstance(o, int) else pl.multiple_of(o, TA), TA)
        return pltpu.make_async_copy(ob_ref.at[it], o_hbm.at[:, sl], sem_out.at[it])

    for c in range(3):
        cp_wqkv(c).start()
    cp_wqkv(0).wait()
    cp_x0.start()
    cp_wo.start()
    _prep_wqkv(0, wqkv_ref, wq_ref, t1_ref)
    cp_wqkv(1).wait()
    _prep_wqkv(1, wqkv_ref, wq_ref, t1_ref)
    cp_wqkv(2).wait()
    for n in range(6):
        cp_w(0, n).start()
    _prep_wqkv(2, wqkv_ref, wq_ref, t1_ref)
    cp_x0.wait()
    cp_wo.wait()
    for a in range(LAG):
        x_ref[a] = xb_ref[:, a * TA:(a + 1) * TA].astype(f32)
    _prep_wo(wo_ref, wot_ref, t2_ref)

    def pro(s, carry):
        alhs = _attn_lhs(s, x_ref, wq_ref)
        att = []
        for j in range(TA // SB):
            _attn_proj(s, j, alhs, wq_ref, qkv_ref)
            att.append(_attn_core(s, j, qkv_ref))
        _attn_post(s, cat0(*att), x_ref, wot_ref, lm_ref)
        return carry

    lax.fori_loop(0, LAG, pro, 0)
    cp_x1.start()

    def wait_weights(f):
        @pl.when(f < LAG)
        def _():
            for m, (w_ref, c_ref, fn) in enumerate(((wg_ref, cg_ref, _combine_proj), (wu_ref, cu_ref, _combine_proj),
                                                    (wdt_ref, cd_ref, _combine_down))):
                for half in range(LAG):
                    @pl.when(f == half)
                    def _():
                        cp_w(half, 2 * m).wait()
                        cp_w(half, 2 * m + 1).wait()
                fn(f * CPI, w_ref, c_ref)

        @pl.when(f == 0)
        def _():
            cp_x1.wait()
            for n in range(6):
                cp_w(1, n).start()
            for a in range(LAG, NA):
                x_ref[a] = xb_ref[:, a * TA:(a + 1) * TA].astype(f32)

    def start_out(f):
        @pl.when(jnp.logical_and(f >= NA, f % LAG == LAG - 1))
        def _():
            for a in range(LAG):
                cp_out(f - NA - (LAG - 1) + a).start()

    def fused(s, carry):
        f = s - LAG
        wait_weights(f)
        c0 = (f % LAG) * CPI
        lhs = _load_lhs(f, lm_ref)
        g = _ffn_proj(c0, CPI, lhs, cg_ref)
        u = _ffn_proj(c0, CPI, lhs, cu_ref)
        alhs = _attn_lhs(s, x_ref, wq_ref)
        hs = [a * b for a, b in zip(g, u)]
        att = []

        def mid(k):
            if k < TA // SB:
                _attn_proj(s, k, alhs, wq_ref, qkv_ref)
                att.append(_attn_core(s, k, qkv_ref))
            elif k == 5:
                _attn_post(s, cat0(*att), x_ref, wot_ref, lm_ref)

        _ffn_down(f, c0, CPI, hs, cd_ref, x_ref, ob_ref, mid=mid)
        start_out(f)
        return carry

    lax.fori_loop(LAG, NSTEP, fused, 0)

    def epi(c, carry):
        f = NSTEP - 1
        lhs = _load_lhs(f, lm_ref)
        hs = [a * b for a, b in zip(_ffn_proj(c, 1, lhs, cg_ref), _ffn_proj(c, 1, lhs, cu_ref))]
        _ffn_down(f, c, 1, hs, cd_ref, x_ref, ob_ref)
        return carry

    lax.fori_loop(0, NCK, epi, 0)
    for it in range(NA - LAG, NA):
        cp_out(it).start()
    for it in range(NA):
        cp_out(it).wait()


@jax.jit
def pallas_interleave_layers__sliding_local_dilated__glu_gated_bilinear__prompt_kernel(
    A_x, A_wqkv, A_wo, B_x, B_w_gate, B_w_up, B_w_down):
    xt = A_x[0].T
    wdt = B_w_down.T
    hbm = pl.BlockSpec(memory_space=pl.ANY)
    out_t = pl.pallas_call(
        _kernel,
        in_specs=[hbm] * 6,
        out_specs=hbm,
        out_shape=jax.ShapeDtypeStruct((D, S), bf16),
        scratch_shapes=[
            pltpu.VMEM((D, S), bf16),
            pltpu.VMEM((D, 3 * D), bf16),
            pltpu.VMEM((D, D), bf16),
            pltpu.VMEM((D, F), bf16),
            pltpu.VMEM((D, F), bf16),
            pltpu.VMEM((D, F), bf16),
            pltpu.VMEM((NCK, 7, 160, CW), u32),
            pltpu.VMEM((NCK, 7, 160, CW), u32),
            pltpu.VMEM((NCK, 8, 144, CW), u32),
            pltpu.VMEM((D // 2, NQ), u32),
            pltpu.VMEM((320, 640), u32),
            pltpu.VMEM((3, 3 * D, 128), u32),
            pltpu.VMEM((5, D, 128), f32),
            pltpu.VMEM((NA, D, TA), f32),
            pltpu.VMEM((14, QROWS, 128), f32),
            pltpu.VMEM((2, LAG, 8, TA // 4, 256), u32),
            pltpu.VMEM((NA, D, TA), bf16),
            pltpu.SemaphoreType.DMA((6,)),
            pltpu.SemaphoreType.DMA((6 * LAG,)),
            pltpu.SemaphoreType.DMA((NA,)),
        ],
        compiler_params=pltpu.CompilerParams(vmem_limit_bytes=110 * 1024 * 1024),
    )(xt, A_wqkv, A_wo, B_w_gate, B_w_up, wdt)
    return out_t.T[None]
```

```python
import functools
import math

import jax
import jax.numpy as jnp
from jax import lax
import jax.experimental.pallas as pl
import jax.experimental.pallas.tpu as pltpu

S, D, F = 2048, 576, 4608
H, DH, W, DIL = 32, 18, 8, 2
NQ = 14 * 128
HALO = 16
QROWS = S + 2 * HALO + 8
TA = 256
TF = 512
FH = F // 2
LAG = TF // TA
EVERY = 6
STAGES = {0: (0, 1), 1: (2,), 2: (3,)}
KPOST, DPOST = 4, 7
LEAD = 2
NCH = 2
RB = 32
SB = 64
NA = S // TA
NSTEP = 2 * NA
EPS = 1e-5
bf16, f32, u32, i32 = jnp.bfloat16, jnp.float32, jnp.uint32, jnp.int32
NT = (((1,), (1,)), ((), ()))
SCALE = DH ** -0.5
EXP2_C = SCALE * math.log2(math.e)
NEG = -1e9 / SCALE

ORD = (0, 2, 3, 1, 4, 5, 6)
SPEC = {1: (1, (0,)), 4: (0, (1,)), 5: (1, (0, 1)), 6: (0, (0, 1))}
SETS = ((0,), (1,), (0, 1))
SIDX = {n: k for k, n in enumerate(SPEC)}

dot = functools.partial(jnp.dot, preferred_element_type=f32)


def dnt(a, b):
    return lax.dot_general(a, b, NT, preferred_element_type=f32)


def cat0(*xs):
    return xs[0] if len(xs) == 1 else jnp.concatenate(xs, axis=0)


def cat1(*xs):
    return xs[0] if len(xs) == 1 else jnp.concatenate(xs, axis=1)


def tb(x):
    return x.T.astype(bf16)


def pkb(x):
    return pltpu.bitcast(x.astype(bf16), u32)


def pkt(x):
    return pltpu.bitcast(tb(x), u32)


def up(x):
    return pltpu.bitcast(x, bf16)


def _chain_sum(load, fn):
    acc = None
    for r in range(0, D, 8 * NCH):
        t = fn(load(r, 8 * NCH))
        acc = t if acc is None else acc + t
    return jnp.sum(acc, axis=0, keepdims=True)


def _ln_t(load, m=None):
    if m is None:
        m = _chain_sum(load, lambda v: v) * (1.0 / D)
    r = lax.rsqrt(_chain_sum(load, lambda v: (v - m) * (v - m)) * (1.0 / D) + EPS)
    return load(0, D) * r - m * r


def _prep_wqkv(c, wqkv_ref, wq_ref, t1_ref):
    n = min(256, D - 256 * c)
    wp = pltpu.bitcast(wqkv_ref[256 * c:256 * c + n, :], u32)
    if n < 256:
        wp = cat0(wp, jnp.zeros(((256 - n) // 2, 3 * D), u32))
    t1_ref[c] = wp.T

    def rows(t, d):
        return t1_ref[c, pl.ds(t * D + d, H, stride=DH), :]

    parts = []
    for t in range(3):
        parts += [rows(t, d) for d in range(16)]
    parts += [rows(0, 16), rows(0, 17), rows(2, 16), rows(2, 17)]
    parts += [rows(1, 16), rows(1, 17), jnp.zeros((64, 128), u32)]
    wq_ref[128 * c:128 * c + n // 2, :] = cat0(*parts).T[:n // 2]


def _prep_wo(wo_ref, wot_ref, t2_ref):
    wo = cat1(wo_ref[...].astype(f32), jnp.zeros((D, 64), f32))
    for c in range(5):
        t2_ref[c] = wo[:, c * 128:(c + 1) * 128]
    for c in range(5):
        parts = [t2_ref[c, pl.ds(d, H, stride=DH), :] for d in range(16)]
        parts += [jnp.zeros((64, 128), f32)]
        parts += [t2_ref[c, pl.ds(d, H, stride=DH), :] for d in (16, 17)]
        wot_ref[64 * c:64 * c + 64, :] = pkt(cat0(*parts))


def _attn_lhs(s, x_ref, wq_ref, pa, pa_ld):
    hf = TA // 2
    item = s % NA
    z = _ln_t(lambda r, n: x_ref[item, r:r + n, :])
    z1, z2 = z[:, :hf], z[:, hf:]
    pa.at[0][...] = pkt(cat0(z1[:448], z1[448:512] - z2[448:512]))
    pa.at[1][...] = pkt(cat0(z2[:448], z2[512:] - z1[512:]))
    pa.at[2][:, :128] = pkt(cat0(z2[448:512], z1[512:]))
    return dot(up(pa_ld[2, :, :128]), up(wq_ref[224:, :]))


def _attn_proj(s, j, sh, pa, wq_ref, qkv_ref):
    item = s % NA
    t0 = pl.multiple_of(item * TA, TA)
    nb = TA // 2 // SB
    r = (j % nb) * SB
    p = up(pa[j // nb, r // 2:(r + SB) // 2, :])
    if j < nb:
        y = dot(p, up(wq_ref[:256, :])) + sh[r:r + SB]
    else:
        y = dot(p, up(cat0(wq_ref[:224, :], wq_ref[256:, :]))) + sh[r:r + SB]
    for c in range(14):
        qkv_ref[c, pl.ds(t0 + (HALO + j * SB), SB), :] = y[:, c * 128:(c + 1) * 128]
    if j == 0:
        hrow = pl.multiple_of(jnp.where(item == 0, 0, S + HALO), HALO)
        for c in range(4, 14):
            qkv_ref[c, pl.ds(hrow, HALO), :] = jnp.broadcast_to(y[0:1, c * 128:(c + 1) * 128], (HALO, 128))


def _attn_core(s, j, qkv_ref, at):
    t0 = pl.multiple_of((s % NA) * TA, TA)
    qi = (0, 1, 2, 3, 12)
    ki = (4, 5, 6, 7, 13)
    vi = (8, 9, 10, 11, 12)
    for b in range(SB // RB):
        r0 = t0 + (j * SB + b * RB + HALO)
        q = [qkv_ref[c, pl.ds(r0, RB), :] for c in qi]
        ls = []
        for w in range(W):
            acc = None
            for c in range(5):
                t = q[c] * qkv_ref[ki[c], pl.ds(r0 - DIL * w, RB), :]
                acc = t if acc is None else acc + t
            acc = acc + pltpu.roll(acc, 64, 1)
            acc = acc + pltpu.roll(acc, 32, 1)
            if w > 0 and j == 0 and b == 0:
                pos = t0 + lax.broadcasted_iota(i32, (HALO, 128), 0)
                top = jnp.where(pos >= DIL * w, acc[:HALO], NEG)
                acc = top if RB == HALO else cat0(top, acc[HALO:])
            ls.append(acc)
        m = functools.reduce(jnp.maximum, ls)
        pr = [jnp.exp2((l - m) * EXP2_C) for l in ls]
        inv = 1.0 / functools.reduce(jnp.add, pr)
        o = (j * SB + b * RB) // 2
        for c in range(5):
            acc = None
            for w in range(W):
                t = pr[w] * qkv_ref[vi[c], pl.ds(r0 - DIL * w, RB), :]
                acc = t if acc is None else acc + t
            at[o:o + RB // 2, 128 * c:128 * c + 128] = pkb(acc * inv)


def lhs7(a11, a12, a21, a22):
    return (lambda: a11 + a22, lambda: a21 + a22, lambda: a11, lambda: a22,
            lambda: a11 + a12, lambda: a21 - a11, lambda: a12 - a22)


def rhs7(b11, b12, b21, b22):
    return (lambda: b11 + b22, lambda: b11, lambda: b12 - b22, lambda: b21 - b11,
            lambda: b22, lambda: b11 + b12, lambda: b21 + b22)


def out4(m):
    m1, m2, m3, m4, m5, m6, m7 = m
    return [[m1 + m4 - m5 + m7, m3 + m5], [m2 + m4, m1 + m3 - m2 + m6]]


def unit(u, rows, off=0, n=None):
    off = rows * (u // 2) + off
    n = rows if n is None else n
    r = slice(off, off + n) if isinstance(off, int) else pl.ds(pl.multiple_of(off, 8), n)
    return r, slice(128 * (u % 2), 128 * (u % 2) + 128)


def _attn_post(s, at, x_ref, wot_ref, lm_ref):
    item = s % NA
    xt = x_ref[item] + dnt(up(wot_ref[:D // 2, :]), up(at[...]))
    x_ref[item] = xt
    m = _chain_sum(lambda r, n: xt[r:r + n], lambda v: v) * (1.0 / D)
    z = _ln_t(lambda r, n: x_ref[item, r:r + n, :], m)
    zt = cat0(z, z[512:]).T
    dst = lm_ref.at[(s // LAG) % 2, s % LAG]
    lo = lax.broadcasted_iota(i32, (16, 128), 1) < 64

    def step(r, n, gate):
        def blk(q, i, k):
            o = 64 * i + 32 * q + r
            return zt[o:o + 16, 128 * k:128 * k + 128]

        g11, g22 = (gate, lambda v: v) if n in (0, 2, 4, 5) else (lambda v: v, gate)
        inner = [lhs7(*[lhs7(g11(blk(q, i, k)), blk(q, i, 2 + k), blk(q, 2 + i, k), g22(blk(q, 2 + i, 2 + k)))[n]()
                        for i in range(2) for k in range(2)]) for q in range(2)]
        for l in range(7):
            x1, x2 = inner[0][l](), inner[1][l]()
            if n in SPEC and l in SPEC:
                i = 2 * SPEC[n][0] + SPEC[l][0]
                r1, r2 = blk(0, i, 4), blk(1, i, 4)
                dst[unit(98 + 4 * SIDX[n] + SIDX[l], 16, r // 2, 8)] = pkb(jnp.where(lo, r1, x2))
                x1, x2 = jnp.where(lo, x1, x1 - x2), jnp.where(lo, x2, r2 - r1)
            dst[unit(2 * (7 * n + l), 16, r // 2, 8)] = pkb(x1)
            dst[unit(2 * (7 * n + l) + 1, 16, r // 2, 8)] = pkb(x2)

    return [functools.partial(step, r, n) for r in (0, 16) for n in range(7)]


class Pacer:
    def __init__(self, live):
        self.live, self.todo, self.wait = live, [], 0

    def add(self, steps, every, delay=0):
        if not self.todo:
            self.wait = delay
        self.todo += [(st, every) for st in steps]

    def tick(self, p):
        self.wait -= 1
        if self.todo and self.wait <= 0:
            st, self.wait = self.todo.pop(0)
            tok = p[:16, :128]
            st(lambda v: tok if v is None else jnp.where(self.live, v, tok))

    def flush(self):
        while self.todo:
            self.todo.pop(0)[0](lambda v: v)


def wunit(p, part, off=0, n=32):
    if part == 2:
        p, part = (49, p) if p < 2 else (50 + p % 2, p // 2 - 1)
    return unit(p, 64, 32 * part + off, n)


def _row(ref, r, c, n):
    c = 128 * c if isinstance(c, int) else pl.multiple_of(128 * c, 128)
    r = r if isinstance(r, int) else pl.multiple_of(r, 16)
    v = pltpu.bitcast(ref[pl.ds(r, 16), pl.ds(c, 128 * n)], u32)
    return [v[:, 128 * k:128 * k + 128] for k in range(n)]


def unp(v):
    return up(v).astype(f32)


class Chain:
    def __init__(self, live):
        self.live, self.tok = live, None

    def stage(self, blocks, emit):
        tok, self.tok = self.tok, None
        for k, (idx, v) in enumerate(emit([unp(v if tok is None else jnp.where(self.live, v, tok)) for v in blocks])):
            v = pkb(v)
            idx[0][idx[1]] = v
            if k <= LEAD:
                self.tok = v

    def two_level(self, fn, blk, where):
        quad = lambda a, b: [blk[2 * a + i][2 * b + j] for i in range(2) for j in range(2)]
        got = {}

        def emit(keys, ns, vals):
            for k, key in enumerate(keys):
                got[key] = vals[4 * k:4 * k + 4]
            for n in ns:
                q = [got.get(c, (None,) * 4) for c in ((0, 0), (0, 1), (1, 0), (1, 1))]
                inner = fn(*[fn(*[c[x] for c in q])[n]() for x in range(4)])
                for l in range(7):
                    yield where(7 * n + l), inner[l]()

        plan = ((1, 4, 0), (5, 2), (3, 6)) if fn is rhs7 else ((2, 3, 0), (4, 6), (1, 5))
        for keys, ns in zip((((0, 0), (1, 1)), ((0, 1),), ((1, 0),)), plan):
            self.stage(sum((quad(*k) for k in keys), []), functools.partial(emit, keys, ns))


def _shift(ref, off, most):
    return ref.at[pl.ds(off if isinstance(off, int) else pl.multiple_of(off, 8), ref.shape[0] - most)]


def _combine_proj(half, live, wg_ref, wu_ref, c_ref):
    lo = lax.broadcasted_iota(i32, (8, 128), 1) < 64

    def row(r, tile):
        if tile < 8:
            return _row((wg_ref, wu_ref)[tile % 2], r, 4 * (tile // 2), 4)
        out = []
        for g, u in zip(_row(wg_ref, r, 16, 2), _row(wu_ref, r, 16, 2)):
            w = pltpu.roll(jnp.where(lo, u, g), 64, 1)
            out += [jnp.where(lo, g, w), jnp.where(lo, w, u)]
        return out

    def main(j, carry):
        ch = Chain(live)
        for tile in range(9):
            dst = _shift(c_ref.at[half * 9 + tile], 8 * j, 56)
            ch.two_level(rhs7, [row(128 * k + 16 * j, tile) for k in range(4)], lambda p: (dst, wunit(p, 0, 0, 8)))
        return carry

    def rem(j, carry):
        ch = Chain(live)
        for tile in range(9):
            dst = _shift(c_ref.at[half * 9 + tile], 8 * j, 24)

            def emit(r):
                for a, (x, y) in enumerate(((r[0], r[1]), (r[2], r[3]), (r[0] + r[2], r[1] + r[3]))):
                    for b, v in enumerate((x, y, x + y)):
                        yield (dst, wunit(3 * a + b, 2, 0, 8)), v

            ch.stage(row(512 + 16 * j, tile), emit)
        return carry

    lax.fori_loop(0, 8, main, 0)
    lax.fori_loop(0, 4, rem, 0)


def _down_unit(ch, j, w_ref, c, dst):
    dst = _shift(dst, 8 * j, 64)
    ch.two_level(lhs7, [_row(w_ref, 144 * k + 16 * j, c, 4) for k in range(4)], lambda p: (dst, unit(p, 72, 0, 8)))


def _combine_down(half, live, wdt_ref, cd_ref, cr_ref):
    def body(j, carry):
        ch = Chain(live)
        for t in range(4):
            _down_unit(ch, j, wdt_ref, 4 * t, cd_ref.at[1 + half * 4 + t])
        dst = _shift(cr_ref.at[half], 8 * j, 64)
        for c in range(2):
            r = 144 * c + 16 * j
            ch.stage(_row(wdt_ref, r, 16, 2) + _row(wdt_ref, 288 + r, 16, 2),
                     lambda a: [((dst, unit(n, 144, 72 * c, 8)), lhs7(*a)[n]()) for n in range(7)])
        return carry

    lax.fori_loop(0, 9, body, 0)


def _proj_pass(lm, w, q, sh, tick):
    def lhs(u):
        return up(cat0(*[lm.at[a][unit(u, 16)] for a in range(LAG)]))

    def wts(a, b):
        return up(cat0(w[wunit(*a)], w[wunit(*b)]))

    def prod(n, l):
        p = 7 * n + l
        if n in SPEC and l in SPEC:
            wr = (3 * SETS.index(SPEC[n][1]) + SETS.index(SPEC[l][1]), 2)
            if q == 0:
                sh[p] = dot(lhs(98 + 4 * SIDX[n] + SIDX[l]), wts(wr, (p, 1)))
            return dot(lhs(2 * p + q), wts((p, 0), wr if q else (p, 1))) + sh[p]
        return dot(lhs(2 * p + q), wts((p, 0), (p, 1)))

    ms = [None] * 7
    for n in ORD:
        p = [None] * 7
        for l in ORD:
            p[l] = prod(n, l)
            tick(p[l])
        ms[n] = out4(p)
    return ms


def _col(ms, ii, ji, jo, rows, gate):
    m1, m2, m3, m4, m5, m6, m7 = [m[ii][ji][rows] for m in ms]
    if jo == 0:
        a = gate(m4)
        return a + m1 - m5 + m7, a + m2
    a = gate(m3)
    return a + m5, a + m1 - m2 + m6


def _mix(a, b):
    lo = lax.broadcasted_iota(i32, a.shape, 1) < 64
    return jnp.where(lo, a, b) * pltpu.roll(jnp.where(lo, b, a), 64, 1)


def _build_steps(mg, mu, t, q, rb, merged=False):
    def step(e, r, blk, k, ns, gate):
        rows = slice(32 * k[1] + r, 32 * k[1] + r + 16)
        blk[k] = []
        for ki in range(2):
            if merged:
                a, b = [_col((mg, mu)[k[0]], e, ji, ki, rows, gate) for ji in range(2)]
                blk[k] += [_mix(a[0], b[0]), _mix(a[1], b[1])]
            else:
                g, u = _col(mg, e, ki, k[0], rows, gate), _col(mu, e, ki, k[0], rows, gate)
                blk[k] += [g[0] * u[0], g[1] * u[1]]
        o = 32 * e + 16 * q + r // 2
        for n in ns:
            quad = [blk.get(c, (None,) * 4) for c in ((0, 0), (0, 1), (1, 0), (1, 1))]
            inner = rhs7(*[rhs7(*[c[x] for c in quad])[n]() for x in range(4)])
            for l in range(7):
                rb.at[7 * n + l][o:o + 8, 128 * t:128 * t + 128] = pkb(inner[l]())

    steps = []
    for e in range(2):
        for r in (0, 16):
            blk = {}
            for k, ns in (((0, 0), (1,)), ((1, 1), (4, 0)), ((0, 1), (5, 2)), ((1, 0), (3, 6))):
                steps.append(functools.partial(step, e, r, blk, k, ns))
    return steps


def _build_rem(ms, q, rb):
    for ii in range(2):
        c = [[_col(ms, ii, ji, jo, slice(None), lambda v: v) for ji in range(2)] for jo in range(2)]
        for io in range(2):
            h = [_mix(a[io], b[io]) for a, b in c]
            ops = rhs7(h[0][:32], h[0][32:], h[1][:32], h[1][32:])
            for n in range(7):
                o, cc = 32 * ii + 16 * q, 256 * (n % 2) + 128 * io
                rb.at[49 + n // 2][o:o + 16, cc:cc + 128] = pkb(ops[n]())


def _ffn_pos(lm, wa, wb, t, pc, rb, every, merged=False, early=lambda: None):
    sa, sb = {}, {}
    for q in range(2):
        g = _proj_pass(lm, wa, q, sa, pc.tick)
        u = _proj_pass(lm, wb, q, sb, pc.tick)
        pc.add(_build_steps(g, u, t, q, rb, merged), every[q], 4)
        if q == 0:
            early()


def _ffn_down(tile, wts, rhs, rem, pc, x_ref, mid=lambda k: None):
    ms = [None] * 7

    def rdot(n):
        r = dnt(*rem(n))
        pc.tick(r)
        return r

    def group(n, base):
        if rem and n != ORD[0]:
            base = rdot(n) if base is None else base + rdot(n)
        p = [None] * 7
        for l in ORD:
            p[l] = dnt(up(wts(7 * n + l)), up(rhs(7 * n + l)))
            pc.tick(p[l])
        m1, m2, m3, m4, m5, m6, m7 = p
        if base is None:
            m = out4(p)
        else:
            b = [[base[144 * i:144 * i + 144, 128 * j:128 * j + 128] for j in range(2)] for i in range(2)]
            m = [[b[0][0] + m1 + m4 - m5 + m7, b[0][1] + m3 + m5],
                 [b[1][0] + m4 + m2, b[1][1] + m1 + m3 - m2 + m6]]
        base = cat0(cat1(*m[0]), cat1(*m[1]))
        if rem and n == ORD[0]:
            base = base + rdot(n)
        return base

    def xs(io, a):
        return x_ref.at[tile * LAG + a, 288 * io:288 * io + 288, :]

    for k, n in enumerate(ORD):
        mid(k)
        if n == 5:
            xs(1, 1)[...] = group(n, xs(1, 1)[...] + ms[0] + ms[2] - ms[1])
        elif n == 6:
            xs(0, 0)[...] = group(n, xs(0, 0)[...] + ms[0] + ms[3] - ms[4])
        else:
            ms[n] = group(n, None)
            if n == 1:
                xs(1, 0)[...] = xs(1, 0)[...] + ms[3] + ms[1]
            elif n == 4:
                xs(0, 1)[...] = xs(0, 1)[...] + ms[2] + ms[4]
    pc.flush()


def _kernel(xt_hbm, wqkv_hbm, wo_hbm, wg_hbm, wu_hbm, wdt_hbm, o_hbm,
            xb_ref, wqkv_ref, wo_ref, wg_ref, wu_ref, wdt_ref, wm_ref,
            cgu_ref, cd_ref, cr_ref, wq_ref, wot_ref, t1_ref, t2_ref, x_ref,
            lm_ref, rb_ref, pa_ref, at_ref, ob_ref, qkv_ref, one_ref, sem_in, sem_w, sem_out):
    def cp_wqkv(c):
        rows = pl.ds(256 * c, min(256, D - 256 * c))
        return pltpu.make_async_copy(wqkv_hbm.at[rows], wqkv_ref.at[rows], sem_in.at[c])

    cp_x0 = pltpu.make_async_copy(xt_hbm.at[:, pl.ds(0, TF)], xb_ref.at[:, pl.ds(0, TF)], sem_in.at[3])
    cp_wo = pltpu.make_async_copy(wo_hbm, wo_ref, sem_in.at[4])
    cp_x1 = pltpu.make_async_copy(xt_hbm.at[:, pl.ds(TF, S - TF)], xb_ref.at[:, pl.ds(TF, S - TF)], sem_in.at[5])

    def cp_w(half, n):
        src, dst = ((wg_hbm, wg_ref), (wu_hbm, wu_ref), (wdt_hbm, wdt_ref))[n]
        return pltpu.make_async_copy(src.at[:, pl.ds(half * FH, FH)], dst, sem_w.at[half * 3 + n])

    def cp_m(half):
        return pltpu.make_async_copy(wdt_hbm.at[:, pl.ds(half * FH + 2048, 256)],
                                     wm_ref.at[:, pl.ds(half * 256, 256)], sem_w.at[3 * LAG + half])

    def cp_out(it):
        o = it * TA
        sl = pl.ds(o if isinstance(o, int) else pl.multiple_of(o, TA), TA)
        return pltpu.make_async_copy(ob_ref.at[it], o_hbm.at[:, sl], sem_out.at[it])

    for c in range(3):
        cp_wqkv(c).start()
    one_ref[0] = 1
    cp_wqkv(0).wait()
    cp_x0.start()
    cp_wo.start()
    _prep_wqkv(0, wqkv_ref, wq_ref, t1_ref)
    cp_wqkv(1).wait()
    _prep_wqkv(1, wqkv_ref, wq_ref, t1_ref)
    cp_wqkv(2).wait()
    for n in range(3):
        cp_w(0, n).start()
    _prep_wqkv(2, wqkv_ref, wq_ref, t1_ref)
    cp_x0.wait()
    cp_wo.wait()
    for a in range(LAG):
        x_ref[a] = xb_ref[:, a * TA:(a + 1) * TA].astype(f32)
    _prep_wo(wo_ref, wot_ref, t2_ref)

    def flags():
        one = one_ref[0]
        return Pacer(jnp.full((16, 128), one, i32) > 0), one - 1

    def pro(s, carry):
        pc, z = flags()
        sh = _attn_lhs(s, x_ref, wq_ref, pa_ref.at[0], pa_ref.at[0])
        for j in range(TA // SB):
            _attn_proj(s, j, sh, pa_ref.at[0], wq_ref, qkv_ref)
            _attn_core(s, j, qkv_ref, at_ref.at[0])
        pc.add(_attn_post(s, at_ref.at[z], x_ref, wot_ref, lm_ref), 1)
        pc.flush()
        return carry

    lax.fori_loop(0, LAG, pro, 0)
    cp_x1.start()

    def wait_w(f, ns):
        for half in range(LAG):
            @pl.when(f == half)
            def _():
                for n in ns:
                    cp_w(half, n).wait()

    def wait_weights(f):
        @pl.when(f < LAG)
        def _():
            live = jnp.full((8, 128), one_ref[0], i32) > 0
            wait_w(f, (0, 1))
            _combine_proj(f, live, wg_ref, wu_ref, cgu_ref)
            wait_w(f, (2,))
            _combine_down(f, live, wdt_ref, cd_ref, cr_ref)

        @pl.when(f == 0)
        def _():
            cp_x1.wait()
            for n in range(3):
                cp_w(1, n).start()
            for half in range(LAG):
                cp_m(half).start()
            for a in range(LAG, NA):
                x_ref[a] = xb_ref[:, a * TA:(a + 1) * TA].astype(f32)

    def emit(it):
        ob_ref[it] = x_ref[it].astype(bf16)
        cp_out(it).start()

    def start_out(f):
        @pl.when(jnp.logical_and(f >= NA, f % LAG == LAG - 1))
        def _():
            for a in range(LAG):
                emit(f - NA - (LAG - 1) + a)

    def fused(s, carry):
        f = s - LAG
        wait_weights(f)
        pc, z = flags()
        half = f % LAG
        lm, rb, rbl = lm_ref.at[(f // LAG) % 2], rb_ref.at[0], rb_ref.at[z]
        sh = []

        def early():
            sh.append(_attn_lhs(s, x_ref, wq_ref, pa_ref.at[0], pa_ref.at[z]))

        for t in range(4):
            _ffn_pos(lm, cgu_ref.at[half * 9 + 2 * t], cgu_ref.at[half * 9 + 2 * t + 1], t, pc, rb,
                     (EVERY, EVERY), early=early if t == 0 else lambda: None)
        sm = {}
        for q in range(2):
            _build_rem(_proj_pass(lm, cgu_ref.at[half * 9 + 8], q, sm, pc.tick), q, rb)
        pc.flush()

        def mid(k):
            for j in STAGES.get(k, ()):
                _attn_proj(s, j, sh[0], pa_ref.at[z], wq_ref, qkv_ref)
                _attn_core(s, j, qkv_ref, at_ref.at[0])
            if k == KPOST:
                pc.add(_attn_post(s, at_ref.at[z], x_ref, wot_ref, lm_ref), 1, DPOST)

        def rem(n):
            cc = 256 * (n % 2)
            return (up(cr_ref.at[half][unit(n, 144)]),
                    up(cat0(rbl[49 + n // 2, :, cc:cc + 128], rbl[49 + n // 2, :, cc + 128:cc + 256])))

        _ffn_down((f // LAG) % (S // TF),
                  lambda p: cat1(*[cd_ref.at[1 + half * 4 + t][unit(p, 72)] for t in range(4)]),
                  lambda p: rbl[p], rem, pc, x_ref, mid=mid)
        start_out(f)
        return carry

    lax.fori_loop(LAG, NSTEP, fused, 0)

    last, lm, rb = S // TF - 1, lm_ref.at[(NSTEP // LAG - 1) % 2], rb_ref.at[0]
    for half in range(LAG):
        cp_m(half).wait()
    pc, _ = flags()
    ch = Chain(pc.live[:8])

    def ninth(j, gate):
        ch.tok = pltpu.bitcast(gate(None)[:8], u32)
        _down_unit(ch, j, wm_ref, 0, cd_ref.at[0])

    pc.add([functools.partial(ninth, j) for j in range(9)], 10, 4)
    _ffn_pos(lm, cgu_ref.at[8], cgu_ref.at[17], 0, pc, rb, (EVERY, EVERY), merged=True)
    pc.flush()

    def epi(c, carry):
        pc, _ = flags()
        ops = [rb[p, :, :128] for p in range(49)]
        w = 2 * c + c // 4
        _ffn_pos(lm, cgu_ref.at[w], cgu_ref.at[w + 1], 0, pc, rb, (EVERY, 3))
        _ffn_down(last, lambda p: cd_ref.at[c][unit(p, 72)], lambda p: ops[p], None, pc, x_ref)
        return carry

    lax.fori_loop(0, 8, epi, 0)
    _ffn_down(last, lambda p: cd_ref.at[8][unit(p, 72)], lambda p: rb[p, :, :128], None, pc, x_ref)
    for it in range(NA - LAG, NA):
        emit(it)
    for it in range(NA):
        cp_out(it).wait()


@jax.jit
def pallas_interleave_layers__sliding_local_dilated__glu_gated_bilinear__prompt_kernel(
    A_x, A_wqkv, A_wo, B_x, B_w_gate, B_w_up, B_w_down):
    xt = A_x[0].T
    wdt = B_w_down.T
    hbm = pl.BlockSpec(memory_space=pl.ANY)
    out_t = pl.pallas_call(
        _kernel,
        in_specs=[hbm] * 6,
        out_specs=hbm,
        out_shape=jax.ShapeDtypeStruct((D, S), bf16),
        scratch_shapes=[
            pltpu.VMEM((D, S), bf16),
            pltpu.VMEM((D, 3 * D), bf16),
            pltpu.VMEM((D, D), bf16),
            pltpu.VMEM((D, FH), bf16),
            pltpu.VMEM((D, FH), bf16),
            pltpu.VMEM((D, FH), bf16),
            pltpu.VMEM((D, 512), bf16),
            pltpu.VMEM((18, 54 * 32, 256), u32),
            pltpu.VMEM((9, 25 * 72 + 8, 256), u32),
            pltpu.VMEM((2, 4 * 144, 256), u32),
            pltpu.VMEM((D // 2, NQ), u32),
            pltpu.VMEM((320, 640), u32),
            pltpu.VMEM((3, 3 * D, 128), u32),
            pltpu.VMEM((5, D, 128), f32),
            pltpu.VMEM((NA, D, TA), f32),
            pltpu.VMEM((2, LAG, 57 * 16, 256), u32),
            pltpu.VMEM((1, 53, 64, 512), u32),
            pltpu.VMEM((1, 3, TA // 4, 512), u32),
            pltpu.VMEM((1, TA // 2, 640), u32),
            pltpu.VMEM((NA, D, TA), bf16),
            pltpu.VMEM((14, QROWS, 128), f32),
            pltpu.SMEM((1,), i32),
            pltpu.SemaphoreType.DMA((6,)),
            pltpu.SemaphoreType.DMA((4 * LAG,)),
            pltpu.SemaphoreType.DMA((NA,)),
        ],
        compiler_params=pltpu.CompilerParams(vmem_limit_bytes=116 * 1024 * 1024),
    )(xt, A_wqkv, A_wo, B_w_gate, B_w_up, wdt)
    return out_t.T[None]
```

```python
import functools
import math

import jax
import jax.numpy as jnp
from jax import lax
import jax.experimental.pallas as pl
import jax.experimental.pallas.tpu as pltpu

S, D, F = 2048, 576, 4608
H, DH, W, DIL = 32, 18, 8, 2
NQ = 14 * 128
NH = NQ // 2
HALO = 16
QROWS = S + 2 * HALO + 8
TA = 256
TF = 512
FH = F // 2
LAG = TF // TA
EVERY = 6
KPOST, DPOST, DLHS = 5, 1, 110
SUB, ELN, EPOST = 3, 1, 2
C1, C2 = (6, 7), 3
EREM = 5
LEAD = 2
NCH = 2
RB = 16
NA = S // TA
NSTEP = 2 * NA
EPS = 1e-5
bf16, f32, u32, i32 = jnp.bfloat16, jnp.float32, jnp.uint32, jnp.int32
NT = (((1,), (1,)), ((), ()))
SCALE = DH ** -0.5
EXP2_C = SCALE * math.log2(math.e)
NEG = -1e9 / SCALE

ORD = (0, 2, 3, 1, 4, 5, 6)
SPEC = {1: (1, (0,)), 4: (0, (1,)), 5: (1, (0, 1)), 6: (0, (0, 1))}
SETS = ((0,), (1,), (0, 1))
QSUM = (0, 2, 3, 5, 6)
SIDX = {n: k for k, n in enumerate(SPEC)}

dot = functools.partial(jnp.dot, preferred_element_type=f32)


def dnt(a, b):
    return lax.dot_general(a, b, NT, preferred_element_type=f32)


def cat0(*xs):
    return xs[0] if len(xs) == 1 else jnp.concatenate(xs, axis=0)


def cat1(*xs):
    return xs[0] if len(xs) == 1 else jnp.concatenate(xs, axis=1)


def tb(x):
    return x.T.astype(bf16)


def pkb(x):
    return pltpu.bitcast(x.astype(bf16), u32)


def pkt(x):
    return pltpu.bitcast(tb(x), u32)


def up(x):
    return pltpu.bitcast(x, bf16)


def _chain_sum(load, fn):
    acc = None
    for r in range(0, D, 8 * NCH):
        t = fn(load(r, 8 * NCH))
        acc = t if acc is None else acc + t
    return jnp.sum(acc, axis=0, keepdims=True)


def _ln_t(load, m=None):
    if m is None:
        m = _chain_sum(load, lambda v: v) * (1.0 / D)
    r = lax.rsqrt(_chain_sum(load, lambda v: (v - m) * (v - m)) * (1.0 / D) + EPS)
    return load(0, D) * r - m * r


def _ln_steps(load, m, out):
    st = {}

    def wide(gate, v):
        v = jnp.broadcast_to(v, (16, TA))
        return cat1(gate(v[:, :128]), gate(v[:, 128:]))

    def var(r0, gate):
        mg = wide(gate, m)
        for r in range(r0, r0 + 96, 16):
            d = load(r, 16) - mg
            st["acc"] = d * d if r == 0 else st["acc"] + d * d

    def norm(c, gate):
        if c == 0:
            st["r"] = lax.rsqrt(jnp.sum(st["acc"], axis=0, keepdims=True) * (1.0 / D) + EPS)
            st["mr"] = jnp.broadcast_to(m * st["r"], (16, TA))
        rg = wide(gate, st["r"])
        z = [load(r, 16) * rg - st["mr"] for r in range(128 * c, min(128 * c + 128, D), 16)]
        out.append(cat0(*(z if c < 4 else z + z)).T)

    return [functools.partial(var, r) for r in range(0, D, 96)] + [functools.partial(norm, c) for c in range(5)]


def _prep_wqkv(c, wqkv_ref, wq_ref, t1_ref):
    n = min(256, D - 256 * c)
    wp = pltpu.bitcast(wqkv_ref[256 * c:256 * c + n, :], u32)
    if n < 256:
        wp = cat0(wp, jnp.zeros(((256 - n) // 2, 3 * D), u32))
    t1_ref[c] = wp.T

    def rows(t, d):
        return t1_ref[c, pl.ds(t * D + d, H, stride=DH), :]

    parts = []
    for t in range(3):
        parts += [rows(t, d) for d in range(16)]
    parts += [rows(0, 16), rows(0, 17), rows(2, 16), rows(2, 17)]
    parts += [rows(1, 16), rows(1, 17), jnp.zeros((64, 128), u32)]
    wq_ref[128 * c:128 * c + n // 2, :] = cat0(*parts).T[:n // 2]


def _share_lhs(blk, rows, dst):
    lo = lax.broadcasted_iota(i32, (2 * rows, 128), 1) < 64
    for c in range(2):
        ops = [lhs7(blk(q, 0, c), blk(q, 0, 2 + c), blk(q, 1, c), blk(q, 1, 2 + c)) for q in range(2)]
        for n in range(7):
            x1, x2 = ops[0][n](), ops[1][n]()
            if c == 1 and n in SPEC:
                r1, r2 = blk(0, SPEC[n][0], 4), blk(1, SPEC[n][0], 4)
                dst[unit(28 + SIDX[n], rows)] = pkb(jnp.where(lo, r1, x2))
                x1, x2 = jnp.where(lo, x1, x1 - x2), jnp.where(lo, x2, r2 - r1)
            dst[unit(4 * n + c, rows)] = pkb(x1)
            dst[unit(4 * n + 2 + c, rows)] = pkb(x2)


def _prep_wo(wo_ref, cw_ref, t2_ref):
    wo = cat1(wo_ref[...].astype(f32), jnp.zeros((D, 64), f32))
    for c in range(5):
        t2_ref[c] = wo[:, c * 128:(c + 1) * 128]
    wt = []
    for c in range(5):
        wt.append(cat0(*[t2_ref[c, pl.ds(d, H, stride=DH), :] for d in tuple(range(18)) + (16, 17)]).T)
    wt = cat0(*wt)
    _share_lhs(lambda q, i, c: wt[288 * i + 144 * q:288 * i + 144 * q + 144, 128 * c:128 * c + 128], 72, cw_ref)


def _prep_wq(live, wq_ref, cq_ref):
    def body(j, carry):
        ch = Chain(live)
        src, dst = _shift(wq_ref, 32 * j, 96), _shift(cq_ref, 32 * j, 96)
        todo = [(r, 128 * t) for r in range(0, 32, 8) for t in range(7)]
        for g in range(0, 28, 2):
            grp = todo[g:g + 2]
            ch.stage([src[r + k:r + k + 8, c + o:c + o + 128] for r, c in grp for k in (0, 128) for o in (0, NH)],
                     lambda v: [((dst, (slice(128 * k + r, 128 * k + r + 8), slice(c, c + 128))),
                                 rhs7(*v[4 * i:4 * i + 4])[n]())
                                for i, (r, c) in enumerate(grp) for k, n in enumerate(QSUM)], 0)
        return carry

    lax.fori_loop(0, 4, body, 0)
    cq_ref[640:, :] = pkb(unp(wq_ref[256:, :NH]) + unp(wq_ref[256:, NH:]))


def _attn_lhs(s, x_ref, pa):
    item = s % NA
    z = _ln_t(lambda r, n: x_ref[item, r:r + n, :])
    zt = cat0(z, z[512:]).T
    _share_lhs(lambda q, i, c: zt[128 * q + 64 * i:128 * q + 64 * i + 64, 128 * c:128 * c + 128], 32, pa)


def _attn_proj(s, q, sh, pc, pa, wq_ref, cq_ref, qkv_ref):
    item = s % NA
    t0 = pl.multiple_of(item * TA, TA)
    lo = lax.broadcasted_iota(i32, (64, 128), 1) < 64
    for t in range(7):
        def wts(n, r, k):
            c = 128 * t
            if n in QSUM:
                return cq_ref[128 * QSUM.index(n) + r:128 * QSUM.index(n) + r + k, c:c + 128]
            return wq_ref[r:r + k, c:c + 128] if n == 1 else wq_ref[128 + r:128 + r + k, NH + c:NH + c + 128]

        def wrem(n):
            c = 128 * t + (NH if n == 4 else 0)
            return (wq_ref[256:, c:c + 128] if n in (1, 4) else cq_ref[640:, c:c + 128])

        p = [None] * 7
        for n in ORD:
            x = pc.pre(pa[64 * n + 32 * q:64 * n + 32 * q + 32, :])
            if n in SPEC:
                if q == 0:
                    sh[t, n] = dot(up(pa[unit(28 + SIDX[n], 32)]), up(cat0(wrem(n), wts(n, 96, 32))))
                w = cat0(wts(n, 0, 96), wrem(n)) if q else wts(n, 0, 128)
                p[n] = dot(up(x), up(w)) + sh[t, n]
            else:
                p[n] = dot(up(x), up(wts(n, 0, 128)))
            pc.tick(p[n])
        y = out4(p)
        for i in range(2):
            for j in range(2):
                c, v = t + 7 * j, y[i][j]
                if c == 13:
                    v = jnp.where(lo, v, 0.0)
                qkv_ref[c, pl.ds(t0 + (HALO + 128 * q + 64 * i), 64), :] = v
                if q == 0 and i == 0 and c >= 4:
                    hrow = pl.multiple_of(jnp.where(item == 0, 0, S + HALO), HALO)
                    qkv_ref[c, pl.ds(hrow, HALO), :] = jnp.broadcast_to(v[0:1], (HALO, 128))


def _attn_core(s, b, qkv_ref, gate):
    t0 = pl.multiple_of((s % NA) * TA, TA)
    qi = (0, 1, 2, 3, 12)
    ki = (4, 5, 6, 7, 13)
    vi = (8, 9, 10, 11, 12)
    r0 = t0 + (b * RB + HALO)
    q = [cat0(*[gate(qkv_ref[c, pl.ds(r0 + r, 16), :]) for r in range(0, RB, 16)]) for c in qi]
    ls = []
    for w in range(W):
        acc = None
        for c in range(5):
            t = q[c] * qkv_ref[ki[c], pl.ds(r0 - DIL * w, RB), :]
            acc = t if acc is None else acc + t
        acc = acc + pltpu.roll(acc, 64, 1)
        acc = acc + pltpu.roll(acc, 32, 1)
        if w > 0 and b == 0:
            pos = t0 + lax.broadcasted_iota(i32, (HALO, 128), 0)
            top = jnp.where(pos >= DIL * w, acc[:HALO], NEG)
            acc = top if RB == HALO else cat0(top, acc[HALO:])
        ls.append(acc)
    m = functools.reduce(jnp.maximum, ls)
    pr = [jnp.exp2((l - m) * EXP2_C) for l in ls]
    inv = 1.0 / functools.reduce(jnp.add, pr)
    out = []
    for c in range(5):
        acc = None
        for w in range(W):
            t = pr[w] * qkv_ref[vi[c], pl.ds(r0 - DIL * w, RB), :]
            acc = t if acc is None else acc + t
        out.append(acc * inv)
    return out


def _attn_rhs(b, a0, a1, at):
    lo = lax.broadcasted_iota(i32, (RB, 128), 1) < 64
    rem = (a0[4], a1[4], a0[4] + a1[4])
    rem = [(r, pltpu.roll(r, 64, 1)) for r in rem]
    for c in range(2):
        ops = rhs7(a0[c], a1[c], a0[2 + c], a1[2 + c])
        for n in range(7):
            v = ops[n]()
            at[unit(2 * n + c, 64, b * RB // 2, RB // 2)] = pkb(v)
            if c == 1 and n in SPEC:
                hi, low = rem[SETS.index(SPEC[n][1])]
                at[unit(14 + 2 * SIDX[n], 64, b * RB // 2, RB // 2)] = pkb(jnp.where(lo, v, hi))
                at[unit(15 + 2 * SIDX[n], 64, b * RB // 2, RB // 2)] = pkb(jnp.where(lo, low, v))


def lhs7(a11, a12, a21, a22):
    return (lambda: a11 + a22, lambda: a21 + a22, lambda: a11, lambda: a22,
            lambda: a11 + a12, lambda: a21 - a11, lambda: a12 - a22)


def rhs7(b11, b12, b21, b22):
    return (lambda: b11 + b22, lambda: b11, lambda: b12 - b22, lambda: b21 - b11,
            lambda: b22, lambda: b11 + b12, lambda: b21 + b22)


def out4(m):
    m1, m2, m3, m4, m5, m6, m7 = m
    return [[m1 + m4 - m5 + m7, m3 + m5], [m2 + m4, m1 + m3 - m2 + m6]]


def unit(u, rows, off=0, n=None):
    off = rows * (u // 2) + off
    n = rows if n is None else n
    r = slice(off, off + n) if isinstance(off, int) else pl.ds(pl.multiple_of(off, 8), n)
    return r, slice(128 * (u % 2), 128 * (u % 2) + 128)


def _attn_post(s, pc, at, x_ref, cw_ref, lm_ref):
    item = s % NA
    sh, y = {}, []
    for q in range(2):
        p = [None] * 7
        for n in ORD:
            w = up(cw_ref[144 * n + 72 * q:144 * n + 72 * q + 72, :])
            if n in SPEC:
                if q == 0:
                    sh[n] = dnt(up(cw_ref[unit(28 + SIDX[n], 72)]), up(at[unit(15 + 2 * SIDX[n], 64)]))
                last = at[unit(14 + 2 * SIDX[n] if q else 2 * n + 1, 64)]
                p[n] = dnt(w, up(cat1(at[unit(2 * n, 64)], last))) + sh[n]
            else:
                p[n] = dnt(w, up(at[64 * n:64 * n + 64, :]))
            pc.tick(p[n])
        y.append(out4(p))
    xt = x_ref[item] + cat0(*[cat1(*y[q][i]) for i in range(2) for q in range(2)])
    x_ref[item] = xt
    m = _chain_sum(lambda r, n: xt[r:r + n], lambda v: v) * (1.0 / D)
    zt = []
    dst = lm_ref.at[(s // LAG) % 2, s % LAG]
    lo = lax.broadcasted_iota(i32, (16, 128), 1) < 64

    def step(r, n, gate):
        def blk(q, i, k):
            o = 64 * i + 32 * q + r
            return zt[k][o:o + 16]

        g11, g22 = (gate, lambda v: v) if n in (0, 2, 4, 5) else (lambda v: v, gate)
        inner = [lhs7(*[lhs7(g11(blk(q, i, k)), blk(q, i, 2 + k), blk(q, 2 + i, k), g22(blk(q, 2 + i, 2 + k)))[n]()
                        for i in range(2) for k in range(2)]) for q in range(2)]
        for l in range(7):
            x1, x2 = inner[0][l](), inner[1][l]()
            if n in SPEC and l in SPEC:
                i = 2 * SPEC[n][0] + SPEC[l][0]
                r1, r2 = blk(0, i, 4), blk(1, i, 4)
                dst[unit(98 + 4 * SIDX[n] + SIDX[l], 16, r // 2, 8)] = pkb(jnp.where(lo, r1, x2))
                x1, x2 = jnp.where(lo, x1, x1 - x2), jnp.where(lo, x2, r2 - r1)
            dst[unit(2 * (7 * n + l), 16, r // 2, 8)] = pkb(x1)
            dst[unit(2 * (7 * n + l) + 1, 16, r // 2, 8)] = pkb(x2)

    return (_ln_steps(lambda r, n: x_ref[item, r:r + n, :], m, zt),
            [functools.partial(step, r, n) for r in (0, 16) for n in range(7)])


class Pacer:
    def __init__(self, live):
        self.live, self.todo, self.wait, self.due, self.sub = live, [], 0, [], 1

    def add(self, steps, every, delay=0):
        if not self.todo:
            self.wait = delay
        self.todo += [(st, every) for st in steps]

    def tick(self, p):
        for k in range(self.sub):
            self.wait -= 1
            if self.todo and self.wait <= 0:
                st, self.wait = self.todo.pop(0)
                o = p.shape[0] // self.sub * k
                tok = p[o:o + 16, :128]
                st(lambda v: tok if v is None else jnp.where(self.live, v, tok))

    def by(self, count, load):
        self.due.append([count, load()])

    def pre(self, w):
        for d in self.due:
            d[0] -= 1
        while self.due and self.due[0][0] <= 0:
            v = jnp.where(self.live[:8], w[:8, :128], self.due.pop(0)[1])
            w = cat0(cat1(v, w[:8, 128:]) if w.shape[1] > 128 else v, w[8:])
        return w

    def flush(self):
        while self.todo:
            self.todo.pop(0)[0](lambda v: v)


def wunit(p, part, off=0, n=32):
    if part == 2:
        p, part = (49, p) if p < 2 else (50 + p % 2, p // 2 - 1)
    return unit(p, 64, 32 * part + off, n)


def _row(ref, r, c, n):
    c = 128 * c if isinstance(c, int) else pl.multiple_of(128 * c, 128)
    r = r if isinstance(r, int) else pl.multiple_of(r, 16)
    v = pltpu.bitcast(ref[pl.ds(r, 16), pl.ds(c, 128 * n)], u32)
    return [v[:, 128 * k:128 * k + 128] for k in range(n)]


def unp(v):
    return up(v).astype(f32)


class Chain:
    def __init__(self, live):
        self.live, self.tok = live, None

    def stage(self, blocks, emit, lead=LEAD):
        tok, self.tok = self.tok, None
        for k, (idx, v) in enumerate(emit([unp(v if tok is None else jnp.where(self.live, v, tok)) for v in blocks])):
            v = pkb(v)
            idx[0][idx[1]] = v
            if k <= lead:
                self.tok = v

    def two_level(self, fn, blk, where):
        quad = lambda a, b: [blk[2 * a + i][2 * b + j] for i in range(2) for j in range(2)]
        got = {}

        def emit(keys, ns, vals):
            for k, key in enumerate(keys):
                got[key] = vals[4 * k:4 * k + 4]
            for n in ns:
                q = [got.get(c, (None,) * 4) for c in ((0, 0), (0, 1), (1, 0), (1, 1))]
                inner = fn(*[fn(*[c[x] for c in q])[n]() for x in range(4)])
                for l in range(7):
                    yield where(7 * n + l), inner[l]()

        plan = ((1, 4, 0), (5, 2), (3, 6)) if fn is rhs7 else ((2, 3, 0), (4, 6), (1, 5))
        for keys, ns in zip((((0, 0), (1, 1)), ((0, 1),), ((1, 0),)), plan):
            self.stage(sum((quad(*k) for k in keys), []), functools.partial(emit, keys, ns))


def _shift(ref, off, most):
    return ref.at[pl.ds(off if isinstance(off, int) else pl.multiple_of(off, 8), ref.shape[0] - most)]


def _combine_proj(half, live, wg_ref, wu_ref, c_ref):
    lo = lax.broadcasted_iota(i32, (8, 128), 1) < 64

    def row(r, tile):
        if tile < 8:
            return _row((wg_ref, wu_ref)[tile % 2], r, 4 * (tile // 2), 4)
        out = []
        for g, u in zip(_row(wg_ref, r, 16, 2), _row(wu_ref, r, 16, 2)):
            w = pltpu.roll(jnp.where(lo, u, g), 64, 1)
            out += [jnp.where(lo, g, w), jnp.where(lo, w, u)]
        return out

    def main(j, carry):
        ch = Chain(live)
        for tile in range(9):
            dst = _shift(c_ref.at[half * 9 + tile], 8 * j, 56)
            ch.two_level(rhs7, [row(128 * k + 16 * j, tile) for k in range(4)], lambda p: (dst, wunit(p, 0, 0, 8)))
        return carry

    def rem(j, carry):
        ch = Chain(live)
        for tile in range(9):
            dst = _shift(c_ref.at[half * 9 + tile], 8 * j, 24)

            def emit(r):
                for a, (x, y) in enumerate(((r[0], r[1]), (r[2], r[3]), (r[0] + r[2], r[1] + r[3]))):
                    for b, v in enumerate((x, y, x + y)):
                        yield (dst, wunit(3 * a + b, 2, 0, 8)), v

            ch.stage(row(512 + 16 * j, tile), emit)
        return carry

    lax.fori_loop(0, 8, main, 0)
    lax.fori_loop(0, 4, rem, 0)


def _down_unit(ch, j, w_ref, c, dst):
    dst = _shift(dst, 8 * j, 64)
    ch.two_level(lhs7, [_row(w_ref, 144 * k + 16 * j, c, 4) for k in range(4)], lambda p: (dst, unit(p, 72, 0, 8)))


def _combine_down(half, live, wdt_ref, cd_ref, cr_ref):
    def body(j, carry):
        ch = Chain(live)
        for t in range(4):
            _down_unit(ch, j, wdt_ref, 4 * t, cd_ref.at[1 + half * 4 + t])
        dst = _shift(cr_ref.at[half], 8 * j, 64)
        for c in range(2):
            r = 144 * c + 16 * j
            ch.stage(_row(wdt_ref, r, 16, 2) + _row(wdt_ref, 288 + r, 16, 2),
                     lambda a: [((dst, unit(n, 144, 72 * c, 8)), lhs7(*a)[n]()) for n in range(7)])
        return carry

    lax.fori_loop(0, 9, body, 0)


def _proj_pass(lm, w, q, sh, pc):
    def lhs(u):
        return up(pc.pre(cat0(*[lm.at[a][unit(u, 16)] for a in range(LAG)])))

    def wts(a, b):
        return up(cat0(w[wunit(*a)], w[wunit(*b)]))

    def prod(n, l):
        p = 7 * n + l
        if n in SPEC and l in SPEC:
            wr = (3 * SETS.index(SPEC[n][1]) + SETS.index(SPEC[l][1]), 2)
            if q == 0:
                sh[p] = dot(lhs(98 + 4 * SIDX[n] + SIDX[l]), wts(wr, (p, 1)))
            return dot(lhs(2 * p + q), wts((p, 0), wr if q else (p, 1))) + sh[p]
        return dot(lhs(2 * p + q), wts((p, 0), (p, 1)))

    ms = [None] * 7
    for n in ORD:
        p = [None] * 7
        for l in ORD:
            p[l] = prod(n, l)
            pc.tick(p[l])
        ms[n] = out4(p)
    return ms


def _col(ms, ii, ji, jo, rows, gate):
    m1, m2, m3, m4, m5, m6, m7 = [m[ii][ji][rows] for m in ms]
    if jo == 0:
        a = gate(m4)
        return a + m1 - m5 + m7, a + m2
    a = gate(m3)
    return a + m5, a + m1 - m2 + m6


def _mix(a, b):
    lo = lax.broadcasted_iota(i32, a.shape, 1) < 64
    return jnp.where(lo, a, b) * pltpu.roll(jnp.where(lo, b, a), 64, 1)


def _build_steps(mg, mu, t, q, rb, merged=False):
    def step(e, r, blk, k, ns, gate):
        rows = slice(32 * k[1] + r, 32 * k[1] + r + 16)
        blk[k] = []
        for ki in range(2):
            if merged:
                a, b = [_col((mg, mu)[k[0]], e, ji, ki, rows, gate) for ji in range(2)]
                blk[k] += [_mix(a[0], b[0]), _mix(a[1], b[1])]
            else:
                g, u = _col(mg, e, ki, k[0], rows, gate), _col(mu, e, ki, k[0], rows, gate)
                blk[k] += [g[0] * u[0], g[1] * u[1]]
        o = 32 * e + 16 * q + r // 2
        for n in ns:
            quad = [blk.get(c, (None,) * 4) for c in ((0, 0), (0, 1), (1, 0), (1, 1))]
            inner = rhs7(*[rhs7(*[c[x] for c in quad])[n]() for x in range(4)])
            for l in range(7):
                rb.at[7 * n + l][o:o + 8, 128 * t:128 * t + 128] = pkb(inner[l]())

    steps = []
    for e in range(2):
        for r in (0, 16):
            blk = {}
            for k, ns in (((0, 0), (1,)), ((1, 1), (4, 0)), ((0, 1), (5, 2)), ((1, 0), (3, 6))):
                steps.append(functools.partial(step, e, r, blk, k, ns))
    return steps


def _rem_steps(ms, q, rb):
    def step(ii, r, gate):
        h = []
        for jo in range(2):
            for item in range(2):
                rows = slice(32 * item + r, 32 * item + r + 16)
                a, b = [_col(ms, ii, ji, jo, rows, gate) for ji in range(2)]
                h.append([_mix(a[io], b[io]) for io in range(2)])
        for io in range(2):
            ops = rhs7(*[v[io] for v in h])
            for n in range(7):
                o, cc = 32 * ii + 16 * q + r // 2, 256 * (n % 2) + 128 * io
                rb.at[49 + n // 2][o:o + 8, cc:cc + 128] = pkb(ops[n]())

    return [functools.partial(step, ii, r) for ii in range(2) for r in (0, 16)]


def _ffn_pos(lm, wa, wb, t, pc, rb, every, merged=False):
    sa, sb = {}, {}
    for q in range(2):
        g = _proj_pass(lm, wa, q, sa, pc)
        u = _proj_pass(lm, wb, q, sb, pc)
        pc.add(_build_steps(g, u, t, q, rb, merged), every[q], 4)


def _ffn_down(tile, wts, rhs, rem, pc, x_ref, mid=lambda k: None):
    ms = [None] * 7

    def rdot(n):
        r = dnt(*rem(n))
        pc.tick(r)
        return r

    def group(n, base):
        if rem and n != ORD[0]:
            base = rdot(n) if base is None else base + rdot(n)
        p = [None] * 7
        for l in ORD:
            p[l] = dnt(up(pc.pre(wts(7 * n + l))), up(rhs(7 * n + l)))
            pc.tick(p[l])
        m1, m2, m3, m4, m5, m6, m7 = p
        if base is None:
            m = out4(p)
        else:
            b = [[base[144 * i:144 * i + 144, 128 * j:128 * j + 128] for j in range(2)] for i in range(2)]
            m = [[b[0][0] + m1 + m4 - m5 + m7, b[0][1] + m3 + m5],
                 [b[1][0] + m4 + m2, b[1][1] + m1 + m3 - m2 + m6]]
        base = cat0(cat1(*m[0]), cat1(*m[1]))
        if rem and n == ORD[0]:
            base = base + rdot(n)
        return base

    def xs(io, a):
        return x_ref.at[tile * LAG + a, 288 * io:288 * io + 288, :]

    for k, n in enumerate(ORD):
        mid(k)
        if n == 5:
            xs(1, 1)[...] = group(n, xs(1, 1)[...] + ms[0] + ms[2] - ms[1])
        elif n == 6:
            xs(0, 0)[...] = group(n, xs(0, 0)[...] + ms[0] + ms[3] - ms[4])
        else:
            ms[n] = group(n, None)
            if n == 1:
                xs(1, 0)[...] = xs(1, 0)[...] + ms[3] + ms[1]
            elif n == 4:
                xs(0, 1)[...] = xs(0, 1)[...] + ms[2] + ms[4]
    pc.flush()


def _kernel(xt_hbm, wqkv_hbm, wo_hbm, wg_hbm, wu_hbm, wdt_hbm, o_hbm,
            xb_ref, wqkv_ref, wo_ref, wg_ref, wu_ref, wdt_ref, wm_ref,
            cgu_ref, cd_ref, cr_ref, wq_ref, cq_ref, cw_ref, t1_ref, t2_ref, x_ref,
            lm_ref, rb_ref, pa_ref, at_ref, ob_ref, qkv_ref, one_ref, sem_in, sem_w, sem_out):
    def cp_wqkv(c):
        rows = pl.ds(256 * c, min(256, D - 256 * c))
        return pltpu.make_async_copy(wqkv_hbm.at[rows], wqkv_ref.at[rows], sem_in.at[c])

    cp_x0 = pltpu.make_async_copy(xt_hbm.at[:, pl.ds(0, TF)], xb_ref.at[:, pl.ds(0, TF)], sem_in.at[3])
    cp_wo = pltpu.make_async_copy(wo_hbm, wo_ref, sem_in.at[4])
    cp_x1 = pltpu.make_async_copy(xt_hbm.at[:, pl.ds(TF, S - TF)], xb_ref.at[:, pl.ds(TF, S - TF)], sem_in.at[5])

    def cp_w(half, n):
        src, dst = ((wg_hbm, wg_ref), (wu_hbm, wu_ref), (wdt_hbm, wdt_ref))[n]
        return pltpu.make_async_copy(src.at[:, pl.ds(half * FH, FH)], dst, sem_w.at[half * 3 + n])

    def cp_m(half):
        return pltpu.make_async_copy(wdt_hbm.at[:, pl.ds(half * FH + 2048, 256)],
                                     wm_ref.at[:, pl.ds(half * 256, 256)], sem_w.at[3 * LAG + half])

    def cp_out(it):
        o = it * TA
        sl = pl.ds(o if isinstance(o, int) else pl.multiple_of(o, TA), TA)
        return pltpu.make_async_copy(ob_ref.at[it], o_hbm.at[:, sl], sem_out.at[it])

    for c in range(3):
        cp_wqkv(c).start()
    one_ref[0] = 1
    cp_wqkv(0).wait()
    cp_x0.start()
    cp_wo.start()
    _prep_wqkv(0, wqkv_ref, wq_ref, t1_ref)
    cp_wqkv(1).wait()
    _prep_wqkv(1, wqkv_ref, wq_ref, t1_ref)
    cp_wqkv(2).wait()
    for n in range(3):
        cp_w(0, n).start()
    _prep_wqkv(2, wqkv_ref, wq_ref, t1_ref)
    cp_x0.wait()
    cp_wo.wait()
    for a in range(LAG):
        x_ref[a] = xb_ref[:, a * TA:(a + 1) * TA].astype(f32)
    _prep_wo(wo_ref, cw_ref, t2_ref)

    def flags():
        one = one_ref[0]
        return Pacer(jnp.full((16, 128), one, i32) > 0), one - 1

    nb = TA // 2 // RB

    def cores(s, att, blocks):
        def step(b, gate):
            att[b] = _attn_core(s, b, qkv_ref, gate)
            if b >= nb:
                _attn_rhs(b - nb, att[b - nb], att[b], at_ref.at[0])
        return [functools.partial(step, b) for b in blocks]

    _prep_wq(flags()[0].live[:8], wq_ref, cq_ref)

    def pro(s, carry):
        pc, z = flags()
        sh, att = {}, {}
        _attn_lhs(s, x_ref, pa_ref.at[0])
        _attn_proj(s, 0, sh, pc, pa_ref.at[0], wq_ref, cq_ref, qkv_ref)
        pc.add(cores(s, att, range(nb)), 40 // nb, 4)
        _attn_proj(s, 1, sh, pc, pa_ref.at[0], wq_ref, cq_ref, qkv_ref)
        pc.add(cores(s, att, range(nb, 2 * nb)), 1)
        pc.flush()
        pc.add(sum(_attn_post(s, pc, at_ref.at[z], x_ref, cw_ref, lm_ref), []), 1)
        pc.flush()
        return carry

    lax.fori_loop(0, LAG, pro, 0)
    cp_x1.start()

    def wait_w(f, ns):
        for half in range(LAG):
            @pl.when(f == half)
            def _():
                for n in ns:
                    cp_w(half, n).wait()

    def wait_weights(f):
        @pl.when(f < LAG)
        def _():
            live = jnp.full((8, 128), one_ref[0], i32) > 0
            wait_w(f, (0, 1))
            _combine_proj(f, live, wg_ref, wu_ref, cgu_ref)
            wait_w(f, (2,))
            _combine_down(f, live, wdt_ref, cd_ref, cr_ref)

        @pl.when(f == 0)
        def _():
            cp_x1.wait()
            for n in range(3):
                cp_w(1, n).start()
            for half in range(LAG):
                cp_m(half).start()
            for a in range(LAG, NA):
                x_ref[a] = xb_ref[:, a * TA:(a + 1) * TA].astype(f32)

    def emit(it):
        ob_ref[it] = x_ref[it].astype(bf16)
        cp_out(it).start()

    def start_out(f):
        @pl.when(jnp.logical_and(f >= NA, f % LAG == LAG - 1))
        def _():
            for a in range(LAG):
                emit(f - NA - (LAG - 1) + a)

    def fused(s, carry):
        f = s - LAG
        wait_weights(f)
        pc, z = flags()
        half = f % LAG
        lm, rb, rbl = lm_ref.at[(f // LAG) % 2], rb_ref.at[0], rb_ref.at[z]
        _attn_lhs(s, x_ref, pa_ref.at[0])
        pc.by(DLHS, lambda: pa_ref[z, :8, :128])
        for t in range(4):
            _ffn_pos(lm, cgu_ref.at[half * 9 + 2 * t], cgu_ref.at[half * 9 + 2 * t + 1], t, pc, rb, (EVERY, EVERY))
        sm, sh, att = {}, {}, {}
        for q in range(2):
            pc.add(_rem_steps(_proj_pass(lm, cgu_ref.at[half * 9 + 8], q, sm, pc), q, rb), EREM)
        _attn_proj(s, 0, sh, pc, pa_ref.at[z], wq_ref, cq_ref, qkv_ref)
        pc.flush()
        pc.add(cores(s, att, range(C1[0])), C1[1], 4)
        _attn_proj(s, 1, sh, pc, pa_ref.at[z], wq_ref, cq_ref, qkv_ref)
        pc.flush()
        pc.add(cores(s, att, range(C1[0], 2 * nb)), C2, 1)

        def mid(k):
            if k == KPOST:
                pc.flush()
                ln, build = _attn_post(s, pc, at_ref.at[z], x_ref, cw_ref, lm_ref)
                pc.sub = SUB
                pc.add(ln, ELN, DPOST)
                pc.add(build, EPOST)

        def rem(n):
            cc = 256 * (n % 2)
            return (up(cr_ref.at[half][unit(n, 144)]),
                    up(cat0(rbl[49 + n // 2, :, cc:cc + 128], rbl[49 + n // 2, :, cc + 128:cc + 256])))

        _ffn_down((f // LAG) % (S // TF),
                  lambda p: cat1(*[cd_ref.at[1 + half * 4 + t][unit(p, 72)] for t in range(4)]),
                  lambda p: rbl[p], rem, pc, x_ref, mid=mid)
        start_out(f)
        return carry

    lax.fori_loop(LAG, NSTEP, fused, 0)

    last, lm, rb = S // TF - 1, lm_ref.at[(NSTEP // LAG - 1) % 2], rb_ref.at[0]
    for half in range(LAG):
        cp_m(half).wait()
    pc, _ = flags()
    ch = Chain(pc.live[:8])

    def ninth(j, gate):
        ch.tok = pltpu.bitcast(gate(None)[:8], u32)
        _down_unit(ch, j, wm_ref, 0, cd_ref.at[0])

    pc.add([functools.partial(ninth, j) for j in range(9)], 10, 4)
    _ffn_pos(lm, cgu_ref.at[8], cgu_ref.at[17], 0, pc, rb, (EVERY, EVERY), merged=True)
    pc.flush()

    def epi(c, carry):
        pc, _ = flags()
        ops = [rb[p, :, :128] for p in range(49)]
        w = 2 * c + c // 4
        _ffn_pos(lm, cgu_ref.at[w], cgu_ref.at[w + 1], 0, pc, rb, (EVERY, 3))
        _ffn_down(last, lambda p: cd_ref.at[c][unit(p, 72)], lambda p: ops[p], None, pc, x_ref)
        return carry

    lax.fori_loop(0, 8, epi, 0)
    _ffn_down(last, lambda p: cd_ref.at[8][unit(p, 72)], lambda p: rb[p, :, :128], None, pc, x_ref)
    for it in range(NA - LAG, NA):
        emit(it)
    for it in range(NA):
        cp_out(it).wait()


@jax.jit
def pallas_interleave_layers__sliding_local_dilated__glu_gated_bilinear__prompt_kernel(
    A_x, A_wqkv, A_wo, B_x, B_w_gate, B_w_up, B_w_down):
    xt = A_x[0].T
    wdt = B_w_down.T
    hbm = pl.BlockSpec(memory_space=pl.ANY)
    out_t = pl.pallas_call(
        _kernel,
        in_specs=[hbm] * 6,
        out_specs=hbm,
        out_shape=jax.ShapeDtypeStruct((D, S), bf16),
        scratch_shapes=[
            pltpu.VMEM((D, S), bf16),
            pltpu.VMEM((D, 3 * D), bf16),
            pltpu.VMEM((D, D), bf16),
            pltpu.VMEM((D, FH), bf16),
            pltpu.VMEM((D, FH), bf16),
            pltpu.VMEM((D, FH), bf16),
            pltpu.VMEM((D, 512), bf16),
            pltpu.VMEM((18, 54 * 32, 256), u32),
            pltpu.VMEM((9, 25 * 72 + 8, 256), u32),
            pltpu.VMEM((2, 4 * 144, 256), u32),
            pltpu.VMEM((D // 2, NQ), u32),
            pltpu.VMEM((672, NH), u32),
            pltpu.VMEM((16 * 72, 256), u32),
            pltpu.VMEM((3, 3 * D, 128), u32),
            pltpu.VMEM((5, D, 128), f32),
            pltpu.VMEM((NA, D, TA), f32),
            pltpu.VMEM((2, LAG, 57 * 16, 256), u32),
            pltpu.VMEM((1, 53, 64, 512), u32),
            pltpu.VMEM((1, 512, 256), u32),
            pltpu.VMEM((1, 11 * 64, 256), u32),
            pltpu.VMEM((NA, D, TA), bf16),
            pltpu.VMEM((14, QROWS, 128), f32),
            pltpu.SMEM((1,), i32),
            pltpu.SemaphoreType.DMA((6,)),
            pltpu.SemaphoreType.DMA((4 * LAG,)),
            pltpu.SemaphoreType.DMA((NA,)),
        ],
        compiler_params=pltpu.CompilerParams(vmem_limit_bytes=116 * 1024 * 1024),
    )(xt, A_wqkv, A_wo, B_w_gate, B_w_up, wdt)
    return out_t.T[None]
```

```python
import functools
import math

import jax
import jax.numpy as jnp
from jax import lax
import jax.experimental.pallas as pl
import jax.experimental.pallas.tpu as pltpu

S, D, F = 2048, 576, 4608
H, DH, W, DIL = 32, 18, 8, 2
NQ = 14 * 128
NH = NQ // 2
HALO = 16
QROWS = S + 2 * HALO + 8
TA = 256
TF = 512
FH = F // 2
LAG = TF // TA
EVERY = 6
KPOST, DPOST, DLHS = 5, 1, 110
SUB, ELN, EPOST = 3, 1, 2
C1, C2 = (6, 7), 3
EREM = 5
CL = 0
EE = 5
HD = (22, 6, 1, 0)
LEAD = 2
NCH = 2
RB = 16
NA = S // TA
NSTEP = 2 * NA
EPS = 1e-5
bf16, f32, u32, i32 = jnp.bfloat16, jnp.float32, jnp.uint32, jnp.int32
NT = (((1,), (1,)), ((), ()))
SCALE = DH ** -0.5
EXP2_C = SCALE * math.log2(math.e)
NEG = -1e9 / SCALE

ORD = (0, 2, 3, 1, 4, 5, 6)
SPEC = {1: (1, (0,)), 4: (0, (1,)), 5: (1, (0, 1)), 6: (0, (0, 1))}
SETS = ((0,), (1,), (0, 1))
QSUM = (0, 2, 3, 5, 6)
SIDX = {n: k for k, n in enumerate(SPEC)}

dot = functools.partial(jnp.dot, preferred_element_type=f32)


def dnt(a, b):
    return lax.dot_general(a, b, NT, preferred_element_type=f32)


def cat0(*xs):
    return xs[0] if len(xs) == 1 else jnp.concatenate(xs, axis=0)


def cat1(*xs):
    return xs[0] if len(xs) == 1 else jnp.concatenate(xs, axis=1)


def tb(x):
    return x.T.astype(bf16)


def pkb(x):
    return pltpu.bitcast(x.astype(bf16), u32)


def pkt(x):
    return pltpu.bitcast(tb(x), u32)


def up(x):
    return pltpu.bitcast(x, bf16)


def _chain_sum(load, fn):
    acc = None
    for r in range(0, D, 8 * NCH):
        t = fn(load(r, 8 * NCH))
        acc = t if acc is None else acc + t
    return jnp.sum(acc, axis=0, keepdims=True)


def _ln_t(load, m=None):
    if m is None:
        m = _chain_sum(load, lambda v: v) * (1.0 / D)
    r = lax.rsqrt(_chain_sum(load, lambda v: (v - m) * (v - m)) * (1.0 / D) + EPS)
    return load(0, D) * r - m * r


def _ln_steps(load, m, out):
    st = {}

    def wide(gate, v):
        v = jnp.broadcast_to(v, (16, TA))
        return cat1(gate(v[:, :128]), gate(v[:, 128:]))

    def var(r0, gate):
        mg = wide(gate, m)
        for r in range(r0, r0 + 96, 16):
            d = load(r, 16) - mg
            st["acc"] = d * d if r == 0 else st["acc"] + d * d

    def norm(c, gate):
        if c == 0:
            st["r"] = lax.rsqrt(jnp.sum(st["acc"], axis=0, keepdims=True) * (1.0 / D) + EPS)
            st["mr"] = jnp.broadcast_to(m * st["r"], (16, TA))
        rg = wide(gate, st["r"])
        z = [load(r, 16) * rg - st["mr"] for r in range(128 * c, min(128 * c + 128, D), 16)]
        out.append(cat0(*(z if c < 4 else z + z)).T)

    return [functools.partial(var, r) for r in range(0, D, 96)] + [functools.partial(norm, c) for c in range(5)]


def _prep_wqkv(c, wqkv_ref, wq_ref, cq_ref, t1_ref):
    n = min(256, D - 256 * c)
    wp = pltpu.bitcast(wqkv_ref[256 * c:256 * c + n, :], u32)
    if n < 256:
        wp = cat0(wp, jnp.zeros(((256 - n) // 2, 3 * D), u32))
    t1_ref[c] = wp.T

    def rows(t, d):
        return t1_ref[c, pl.ds(t * D + d, H, stride=DH), :]

    parts = []
    for t in range(3):
        parts += [rows(t, d) for d in (0, 2, 4, 6, 1, 3, 5, 7, 8, 10, 12, 14, 9, 11, 13, 15)]
    parts += [rows(0, 16), rows(0, 17), rows(2, 16), rows(2, 17)]
    parts += [rows(1, 16), rows(1, 17), jnp.zeros((32, 128), u32), jnp.zeros((32, 128), u32)]
    for t in range(7):
        w = [cat0(*parts[4 * k:4 * k + 4]).T[:n // 2] for k in (t, t + 7)]
        for k, v in zip((t, t + 7), w):
            wq_ref[128 * c:128 * c + n // 2, 128 * k:128 * k + 128] = v
        cols = slice(128 * t, 128 * t + 128)
        if c == 2:
            cq_ref[640:, cols] = pkb(unp(w[0]) + unp(w[1]))
        if c == 1:
            for r in range(0, 128, 8):
                ops = rhs7(*[unp(wq_ref[r:r + 8, 128 * k:128 * k + 128]) for k in (t, t + 7)],
                           *[unp(v[r:r + 8]) for v in w])
                for k, m in enumerate(QSUM):
                    cq_ref[128 * k + r:128 * k + r + 8, cols] = pkb(ops[m]())


def _share_lhs(load, rows, dst):
    lo = lax.broadcasted_iota(i32, (16, 128), 1) < 64

    def step(r, gate):
        blk = [[load(q, i, r, gate) for i in range(2)] for q in range(2)]
        for c in range(2):
            ops = [lhs7(b[0][c], b[0][2 + c], b[1][c], b[1][2 + c]) for b in blk]
            for n in range(7):
                x1, x2 = ops[0][n](), ops[1][n]()
                if c == 1 and n in SPEC:
                    r1, r2 = blk[0][SPEC[n][0]][4], blk[1][SPEC[n][0]][4]
                    dst[unit(28 + SIDX[n], rows, r // 2, 8)] = pkb(jnp.where(lo, r1, x2))
                    x1, x2 = jnp.where(lo, x1, x1 - x2), jnp.where(lo, x2, r2 - r1)
                dst[unit(4 * n + c, rows, r // 2, 8)] = pkb(x1)
                dst[unit(4 * n + 2 + c, rows, r // 2, 8)] = pkb(x2)
        return x1

    return [functools.partial(step, r) for r in range(0, 2 * rows, 16)]


def _prep_wo(wo_ref, cw_ref, t2_ref):
    wo = cat1(pltpu.bitcast(wo_ref[...], u32), jnp.zeros((D // 2, 64), u32))
    for c in range(5):
        t2_ref[c] = wo[:, c * 128:(c + 1) * 128]
    wt = []
    for c in range(5):
        wt.append(cat0(*[t2_ref[c, pl.ds(p, H, stride=DH // 2), :] for p in tuple(range(8)) + (8,) * 4]).T)
    wt = cat0(*wt)
    odd = lax.broadcasted_iota(i32, (16, 128), 1) % 64 >= 32

    def load(q, i, r, gate):
        o = 288 * i + 144 * q + r
        out = []
        for c in range(3):
            w = gate(wt[o:o + 16, 128 * c:128 * c + 128])
            out += [pltpu.bitcast(w << 16, f32), pltpu.bitcast(w & jnp.uint32(0xFFFF0000), f32)]
        return out[:4] + [jnp.where(odd, out[5], out[4])]

    return _share_lhs(load, 72, cw_ref)


def _base(s):
    return s % NA * TA if isinstance(s, int) else pl.multiple_of((s % NA) * TA, TA)


def _attn_lhs(s, x_ref, pa):
    item = s % NA
    z = _ln_t(lambda r, n: x_ref[item, r:r + n, :])
    zt = cat0(z, z[512:]).T

    def load(q, i, r, gate):
        o = 128 * q + 64 * i + r
        return [zt[o:o + 16, 128 * c:128 * c + 128] for c in range(5)]

    for st in _share_lhs(load, 32, pa):
        st(None)


def _attn_proj(s, q, sh, pc, pa, wq_ref, cq_ref, qkv_ref):
    item = s % NA
    t0 = _base(s)
    lo = lax.broadcasted_iota(i32, (64, 128), 1) < 64
    for t in range(7):
        def wts(n, r, k):
            c = 128 * t
            if n in QSUM:
                return cq_ref[128 * QSUM.index(n) + r:128 * QSUM.index(n) + r + k, c:c + 128]
            return wq_ref[r:r + k, c:c + 128] if n == 1 else wq_ref[128 + r:128 + r + k, NH + c:NH + c + 128]

        def wrem(n):
            c = 128 * t + (NH if n == 4 else 0)
            return (wq_ref[256:, c:c + 128] if n in (1, 4) else cq_ref[640:, c:c + 128])

        p = [None] * 7
        for n in ORD:
            x = pc.pre(pa[64 * n + 32 * q:64 * n + 32 * q + 32, :])
            if n in SPEC:
                if q == 0:
                    sh[t, n] = dot(up(pa[unit(28 + SIDX[n], 32)]), up(cat0(wrem(n), wts(n, 96, 32))))
                w = cat0(wts(n, 0, 96), wrem(n)) if q else wts(n, 0, 128)
                p[n] = dot(up(x), up(w)) + sh[t, n]
            else:
                p[n] = dot(up(x), up(wts(n, 0, 128)))
            pc.tick(p[n])
        y = out4(p)
        for i in range(2):
            for j in range(2):
                c, v = t + 7 * j, y[i][j]
                if c == 13:
                    v = jnp.where(lo, v, 0.0)
                qkv_ref[c, pl.ds(t0 + (HALO + 128 * q + 64 * i), 64), :] = v
                if q == 0 and i == 0 and c >= 4 and not (isinstance(s, int) and s):
                    hrow = 0 if isinstance(s, int) else pl.multiple_of(jnp.where(item == 0, 0, S + HALO), HALO)
                    qkv_ref[c, pl.ds(hrow, HALO), :] = jnp.broadcast_to(v[0:1], (HALO, 128))


def _attn_core(s, b, qkv_ref, gate):
    t0 = _base(s)
    qi = (0, 1, 2, 3, 12)
    ki = (4, 5, 6, 7, 13)
    vi = (8, 9, 10, 11, 12)
    r0 = t0 + (b * RB + HALO)
    q = [cat0(*[gate(qkv_ref[c, pl.ds(r0 + r, 16), :]) for r in range(0, RB, 16)]) for c in qi]
    ls = []
    for w in range(W):
        acc = None
        for c in range(5):
            t = q[c] * qkv_ref[ki[c], pl.ds(r0 - DIL * w, RB), :]
            acc = t if acc is None else acc + t
        acc = acc + pltpu.roll(acc, 64, 1)
        acc = acc + pltpu.roll(acc, 32, 1)
        if w > 0 and b == 0 and not (isinstance(s, int) and s):
            pos = t0 + lax.broadcasted_iota(i32, (HALO, 128), 0)
            top = jnp.where(pos >= DIL * w, acc[:HALO], NEG)
            acc = top if RB == HALO else cat0(top, acc[HALO:])
        ls.append(acc)
    m = functools.reduce(jnp.maximum, ls)
    pr = [jnp.exp2((l - m) * EXP2_C) for l in ls]
    inv = 1.0 / functools.reduce(jnp.add, pr)
    out = []
    for c in range(5):
        acc = None
        for w in range(W):
            t = pr[w] * qkv_ref[vi[c], pl.ds(r0 - DIL * w, RB), :]
            acc = t if acc is None else acc + t
        out.append(acc * inv)
    return out


def _attn_rhs(b, a0, a1, at):
    lo = lax.broadcasted_iota(i32, (RB, 128), 1) < 64
    rem = (a0[4], a1[4], a0[4] + a1[4])
    rem = [(r, pltpu.roll(r, 64, 1)) for r in rem]
    for c in range(2):
        ops = rhs7(a0[c], a1[c], a0[2 + c], a1[2 + c])
        for n in range(7):
            v = ops[n]()
            at[unit(2 * n + c, 64, b * RB // 2, RB // 2)] = pkb(v)
            if c == 1 and n in SPEC:
                hi, low = rem[SETS.index(SPEC[n][1])]
                at[unit(14 + 2 * SIDX[n], 64, b * RB // 2, RB // 2)] = pkb(jnp.where(lo, v, hi))
                at[unit(15 + 2 * SIDX[n], 64, b * RB // 2, RB // 2)] = pkb(jnp.where(lo, low, v))


def lhs7(a11, a12, a21, a22):
    return (lambda: a11 + a22, lambda: a21 + a22, lambda: a11, lambda: a22,
            lambda: a11 + a12, lambda: a21 - a11, lambda: a12 - a22)


def rhs7(b11, b12, b21, b22):
    return (lambda: b11 + b22, lambda: b11, lambda: b12 - b22, lambda: b21 - b11,
            lambda: b22, lambda: b11 + b12, lambda: b21 + b22)


def out4(m):
    m1, m2, m3, m4, m5, m6, m7 = m
    return [[m1 + m4 - m5 + m7, m3 + m5], [m2 + m4, m1 + m3 - m2 + m6]]


def unit(u, rows, off=0, n=None):
    off = rows * (u // 2) + off
    n = rows if n is None else n
    r = slice(off, off + n) if isinstance(off, int) else pl.ds(pl.multiple_of(off, 8), n)
    return r, slice(128 * (u % 2), 128 * (u % 2) + 128)


def _attn_post(s, pc, at, x_ref, cw_ref, lm_ref):
    item = s % NA
    sh, y = {}, []
    for q in range(2):
        p = [None] * 7
        for n in ORD:
            w = up(cw_ref[144 * n + 72 * q:144 * n + 72 * q + 72, :])
            if n in SPEC:
                if q == 0:
                    sh[n] = dnt(up(cw_ref[unit(28 + SIDX[n], 72)]), up(at[unit(15 + 2 * SIDX[n], 64)]))
                last = at[unit(14 + 2 * SIDX[n] if q else 2 * n + 1, 64)]
                p[n] = dnt(w, up(cat1(at[unit(2 * n, 64)], last))) + sh[n]
            else:
                p[n] = dnt(w, up(at[64 * n:64 * n + 64, :]))
            pc.tick(p[n])
        y.append(out4(p))
    xt = x_ref[item] + cat0(*[cat1(*y[q][i]) for i in range(2) for q in range(2)])
    x_ref[item] = xt
    m = _chain_sum(lambda r, n: xt[r:r + n], lambda v: v) * (1.0 / D)
    zt = []
    dst = lm_ref.at[(s // LAG) % 2, s % LAG]
    lo = lax.broadcasted_iota(i32, (16, 128), 1) < 64

    def step(r, n, gate):
        def blk(q, i, k):
            o = 64 * i + 32 * q + r
            return zt[k][o:o + 16]

        g11, g22 = (gate, lambda v: v) if n in (0, 2, 4, 5) else (lambda v: v, gate)
        inner = [lhs7(*[lhs7(g11(blk(q, i, k)), blk(q, i, 2 + k), blk(q, 2 + i, k), g22(blk(q, 2 + i, 2 + k)))[n]()
                        for i in range(2) for k in range(2)]) for q in range(2)]
        for l in range(7):
            x1, x2 = inner[0][l](), inner[1][l]()
            if n in SPEC and l in SPEC:
                i = 2 * SPEC[n][0] + SPEC[l][0]
                r1, r2 = blk(0, i, 4), blk(1, i, 4)
                dst[unit(98 + 4 * SIDX[n] + SIDX[l], 16, r // 2, 8)] = pkb(jnp.where(lo, r1, x2))
                x1, x2 = jnp.where(lo, x1, x1 - x2), jnp.where(lo, x2, r2 - r1)
            dst[unit(2 * (7 * n + l), 16, r // 2, 8)] = pkb(x1)
            dst[unit(2 * (7 * n + l) + 1, 16, r // 2, 8)] = pkb(x2)
        return x1

    return (_ln_steps(lambda r, n: x_ref[item, r:r + n, :], m, zt),
            [functools.partial(step, r, n) for r in (0, 16) for n in range(7)])


class Pacer:
    def __init__(self, live):
        self.live, self.todo, self.wait, self.due, self.sub, self.done = live, [], 0, [], 1, []

    def add(self, steps, every, delay=0, lag=0):
        if not self.todo:
            self.wait = delay
        self.todo += [(st, every, lag) for st in steps]

    def run(self, toks):
        st, self.wait, lag = self.todo.pop(0)
        if lag and len(self.done) >= lag and self.done[-lag] is not None:
            toks = toks + [self.done[-lag]]

        def gate(v):
            if v is None:
                return toks[0]
            for t in toks:
                v = jnp.where(self.live, v, t if v.dtype == t.dtype else pltpu.bitcast(t, v.dtype))
            return v

        self.done.append(st(gate))

    def tick(self, p):
        for k in range(self.sub):
            self.wait -= 1
            if self.todo and self.wait <= 0:
                o = p.shape[0] // self.sub * k
                self.run([p[o:o + 16, :128]])

    def by(self, count, load):
        self.due.append([count, load()])

    def pre(self, w):
        for d in self.due:
            d[0] -= 1
        while self.due and self.due[0][0] <= 0:
            v = jnp.where(self.live[:8], w[:8, :128], self.due.pop(0)[1])
            w = cat0(cat1(v, w[:8, 128:]) if w.shape[1] > 128 else v, w[8:])
        return w

    def flush(self):
        while self.todo:
            self.run([])


def wunit(p, part, off=0, n=32):
    if part == 2:
        p, part = (49, p) if p < 2 else (50 + p % 2, p // 2 - 1)
    return unit(p, 64, 32 * part + off, n)


def _row(ref, r, c, n):
    c = 128 * c if isinstance(c, int) else pl.multiple_of(128 * c, 128)
    r = r if isinstance(r, int) else pl.multiple_of(r, 16)
    v = pltpu.bitcast(ref[pl.ds(r, 16), pl.ds(c, 128 * n)], u32)
    return [v[:, 128 * k:128 * k + 128] for k in range(n)]


def unp(v):
    return up(v).astype(f32)


class Chain:
    def __init__(self, live):
        self.live, self.tok = live, None

    def stage(self, blocks, emit, lead=LEAD):
        tok, self.tok = self.tok, None
        for k, (idx, v) in enumerate(emit([unp(v if tok is None else jnp.where(self.live, v, tok)) for v in blocks])):
            v = pkb(v)
            idx[0][idx[1]] = v
            if k <= lead:
                self.tok = v

    def two_level(self, fn, blk, where):
        quad = lambda a, b: [blk[2 * a + i][2 * b + j] for i in range(2) for j in range(2)]
        got = {}

        def emit(keys, ns, vals):
            for k, key in enumerate(keys):
                got[key] = vals[4 * k:4 * k + 4]
            for n in ns:
                q = [got.get(c, (None,) * 4) for c in ((0, 0), (0, 1), (1, 0), (1, 1))]
                inner = fn(*[fn(*[c[x] for c in q])[n]() for x in range(4)])
                for l in range(7):
                    yield where(7 * n + l), inner[l]()

        plan = ((1, 4, 0), (5, 2), (3, 6)) if fn is rhs7 else ((2, 3, 0), (4, 6), (1, 5))
        return [functools.partial(self.stage, sum((quad(*k) for k in keys), []), functools.partial(emit, keys, ns))
                for keys, ns in zip((((0, 0), (1, 1)), ((0, 1),), ((1, 0),)), plan)]


def _shift(ref, off, most):
    return ref.at[pl.ds(off if isinstance(off, int) else pl.multiple_of(off, 8), ref.shape[0] - most)]


def _combine_proj(half, live, wg_ref, wu_ref, c_ref):
    lo = lax.broadcasted_iota(i32, (8, 128), 1) < 64

    def row(r, tile):
        if tile < 8:
            return _row((wg_ref, wu_ref)[tile % 2], r, 4 * (tile // 2), 4)
        out = []
        for g, u in zip(_row(wg_ref, r, 16, 2), _row(wu_ref, r, 16, 2)):
            w = pltpu.roll(jnp.where(lo, u, g), 64, 1)
            out += [jnp.where(lo, g, w), jnp.where(lo, w, u)]
        return out

    def body(j, carry):
        ch = Chain(live)
        for tile in (0, 8, 1, 2, 3, 4, 5, 6, 7):
            dst = _shift(c_ref.at[half * 9 + tile], 8 * j, 24)

            def emit(r):
                for a, (x, y) in enumerate(((r[0], r[1]), (r[2], r[3]), (r[0] + r[2], r[1] + r[3]))):
                    for b, v in enumerate((x, y, x + y)):
                        yield (dst, wunit(3 * a + b, 2, 0, 8)), v

            for part in range(2):
                blk = [row(128 * k + 64 * part + 16 * j, tile) for k in range(4)]
                for st in ch.two_level(rhs7, blk, lambda p: (dst, wunit(p, part, 0, 8))):
                    st()
            ch.stage(row(512 + 16 * j, tile), emit, 0)
        return carry

    lax.fori_loop(0, 4, body, 0)


def _down_unit(ch, j, w_ref, c, dst):
    dst = _shift(dst, 8 * j, 64)
    blk = [_row(w_ref, 144 * k + 16 * j, c, 4) for k in range(4)]
    return ch.two_level(lhs7, blk, lambda p: (dst, unit(p, 72, 0, 8)))


def _combine_down(half, live, wdt_ref, cd_ref, cr_ref):
    def body(j, carry):
        ch = Chain(live)
        for t in range(4):
            for st in _down_unit(ch, j, wdt_ref, 4 * t, cd_ref.at[1 + half * 4 + t]):
                st()
        dst = _shift(cr_ref.at[half], 8 * j, 64)
        for c in range(2):
            r = 144 * c + 16 * j
            ch.stage(_row(wdt_ref, r, 16, 2) + _row(wdt_ref, 288 + r, 16, 2),
                     lambda a: [((dst, unit(n, 144, 72 * c, 8)), lhs7(*a)[n]()) for n in range(7)])
        return carry

    lax.fori_loop(0, 9, body, 0)


def _proj_pass(lm, w, q, sh, pc):
    def lhs(u):
        return up(pc.pre(cat0(*[lm.at[a][unit(u, 16)] for a in range(LAG)])))

    def wts(a, b):
        return up(cat0(w[wunit(*a)], w[wunit(*b)]))

    def prod(n, l):
        p = 7 * n + l
        if n in SPEC and l in SPEC:
            wr = (3 * SETS.index(SPEC[n][1]) + SETS.index(SPEC[l][1]), 2)
            if q == 0:
                sh[p] = dot(lhs(98 + 4 * SIDX[n] + SIDX[l]), wts(wr, (p, 1)))
            return dot(lhs(2 * p + q), wts((p, 0), wr if q else (p, 1))) + sh[p]
        return dot(lhs(2 * p + q), wts((p, 0), (p, 1)))

    ms = [None] * 7
    for n in ORD:
        p = [None] * 7
        for l in ORD:
            p[l] = prod(n, l)
            pc.tick(p[l])
        ms[n] = out4(p)
    return ms


def _col(ms, ii, ji, jo, rows, gate):
    m1, m2, m3, m4, m5, m6, m7 = [m[ii][ji][rows] for m in ms]
    if jo == 0:
        a = gate(m4)
        return a + m1 - m5 + m7, a + m2
    a = gate(m3)
    return a + m5, a + m1 - m2 + m6


def _mix(a, b):
    lo = lax.broadcasted_iota(i32, a.shape, 1) < 64
    return jnp.where(lo, a, b) * pltpu.roll(jnp.where(lo, b, a), 64, 1)


def _build_steps(mg, mu, t, q, rb, merged=False):
    def step(e, r, blk, k, ns, gate):
        rows = slice(32 * k[1] + r, 32 * k[1] + r + 16)
        blk[k] = []
        for ki in range(2):
            if merged:
                a, b = [_col((mg, mu)[k[0]], e, ji, ki, rows, gate) for ji in range(2)]
                blk[k] += [_mix(a[0], b[0]), _mix(a[1], b[1])]
            else:
                g, u = _col(mg, e, ki, k[0], rows, gate), _col(mu, e, ki, k[0], rows, gate)
                blk[k] += [g[0] * u[0], g[1] * u[1]]
        o = 32 * e + 16 * q + r // 2
        for n in ns:
            quad = [blk.get(c, (None,) * 4) for c in ((0, 0), (0, 1), (1, 0), (1, 1))]
            inner = rhs7(*[rhs7(*[c[x] for c in quad])[n]() for x in range(4)])
            for l in range(7):
                rb.at[7 * n + l][o:o + 8, 128 * t:128 * t + 128] = pkb(inner[l]())

    steps = []
    for e in range(2):
        for r in (0, 16):
            blk = {}
            for k, ns in (((0, 0), (1,)), ((1, 1), (4, 0)), ((0, 1), (5, 2)), ((1, 0), (3, 6))):
                steps.append(functools.partial(step, e, r, blk, k, ns))
    return steps


def _rem_steps(ms, q, rb):
    def step(ii, r, gate):
        h = []
        for jo in range(2):
            for item in range(2):
                rows = slice(32 * item + r, 32 * item + r + 16)
                a, b = [_col(ms, ii, ji, jo, rows, gate) for ji in range(2)]
                h.append([_mix(a[io], b[io]) for io in range(2)])
        for io in range(2):
            ops = rhs7(*[v[io] for v in h])
            for n in range(7):
                o, cc = 32 * ii + 16 * q + r // 2, 256 * (n % 2) + 128 * io
                rb.at[49 + n // 2][o:o + 8, cc:cc + 128] = pkb(ops[n]())

    return [functools.partial(step, ii, r) for ii in range(2) for r in (0, 16)]


def _ffn_pos(lm, wa, wb, t, pc, rb):
    sa, sb = {}, {}
    for q in range(2):
        g = _proj_pass(lm, wa, q, sa, pc)
        u = _proj_pass(lm, wb, q, sb, pc)
        pc.add(_build_steps(g, u, t, q, rb), EVERY, 4)


def _ffn_down(tile, wts, rhs, rem, pc, x_ref, mid=lambda k: None, put=None):
    ms = [None] * 7

    def rdot(n):
        r = dnt(*rem(n))
        pc.tick(r)
        return r

    def group(n, base):
        if rem and n != ORD[0]:
            base = rdot(n) if base is None else base + rdot(n)
        p = [None] * 7
        for l in ORD:
            p[l] = dnt(up(pc.pre(wts(7 * n + l))), up(rhs(7 * n + l)))
            pc.tick(p[l])
        m1, m2, m3, m4, m5, m6, m7 = p
        if base is None:
            m = out4(p)
        else:
            b = [[base[144 * i:144 * i + 144, 128 * j:128 * j + 128] for j in range(2)] for i in range(2)]
            m = [[b[0][0] + m1 + m4 - m5 + m7, b[0][1] + m3 + m5],
                 [b[1][0] + m4 + m2, b[1][1] + m1 + m3 - m2 + m6]]
        base = cat0(cat1(*m[0]), cat1(*m[1]))
        if rem and n == ORD[0]:
            base = base + rdot(n)
        return base

    def xs(io, a):
        return x_ref.at[tile * LAG + a, 288 * io:288 * io + 288, :]

    def keep(io, a, v):
        xs(io, a)[...] = v

    put = put or keep
    for k, n in enumerate(ORD):
        mid(k)
        if n == 5:
            put(1, 1, group(n, xs(1, 1)[...] + ms[0] + ms[2] - ms[1]))
        elif n == 6:
            put(0, 0, group(n, xs(0, 0)[...] + ms[0] + ms[3] - ms[4]))
        else:
            ms[n] = group(n, None)
            if n == 1:
                put(1, 0, xs(1, 0)[...] + ms[3] + ms[1])
            elif n == 4:
                put(0, 1, xs(0, 1)[...] + ms[2] + ms[4])
    pc.flush()


def _kernel(xt_hbm, wqkv_hbm, wo_hbm, wg_hbm, wu_hbm, wdt_hbm, o_hbm,
            xb_ref, wqkv_ref, wo_ref, wg_ref, wu_ref, wdt_ref, wm_ref,
            cgu_ref, cd_ref, cr_ref, wq_ref, cq_ref, cw_ref, t1_ref, t2_ref, x_ref,
            lm_ref, rb_ref, mb_ref, pa_ref, at_ref, ob_ref, qkv_ref, one_ref, sem_in, sem_w, sem_out):
    def cp_wqkv(c):
        rows = pl.ds(256 * c, min(256, D - 256 * c))
        return pltpu.make_async_copy(wqkv_hbm.at[rows], wqkv_ref.at[rows], sem_in.at[c])

    cp_x0 = pltpu.make_async_copy(xt_hbm.at[:, pl.ds(0, TF)], xb_ref.at[:, pl.ds(0, TF)], sem_in.at[3])
    cp_wo = pltpu.make_async_copy(wo_hbm, wo_ref, sem_in.at[4])
    cp_x1 = pltpu.make_async_copy(xt_hbm.at[:, pl.ds(TF, S - TF)], xb_ref.at[:, pl.ds(TF, S - TF)], sem_in.at[5])

    def cp_w(half, n):
        src, dst = ((wg_hbm, wg_ref), (wu_hbm, wu_ref), (wdt_hbm, wdt_ref))[n]
        return pltpu.make_async_copy(src.at[:, pl.ds(half * FH, FH)], dst, sem_w.at[half * 3 + n])

    def cp_m(half):
        return pltpu.make_async_copy(wdt_hbm.at[:, pl.ds(half * FH + 2048, 256)],
                                     wm_ref.at[:, pl.ds(half * 256, 256)], sem_w.at[3 * LAG + half])

    def cp_out(it):
        o = it * TA
        sl = pl.ds(o if isinstance(o, int) else pl.multiple_of(o, TA), TA)
        return pltpu.make_async_copy(ob_ref.at[it], o_hbm.at[:, sl], sem_out.at[it])

    def flags():
        one = one_ref[0]
        return Pacer(jnp.full((16, 128), one, i32) > 0), one - 1

    nb = TA // 2 // RB

    def cores(s, att, at, blocks):
        def step(b, gate):
            att[b] = _attn_core(s, b, qkv_ref, gate)
            if b >= nb:
                _attn_rhs(b - nb, att[b - nb], att[b], at)
            return att[b][0]
        return [functools.partial(step, b) for b in blocks]

    def first():
        for a in range(LAG):
            x_ref[a] = xb_ref[:, a * TA:(a + 1) * TA].astype(f32)
            _attn_lhs(a, x_ref, pa_ref.at[a])

    cp_wqkv(2).start()
    cp_x0.start()
    cp_wqkv(0).start()
    one_ref[0] = 1
    for m, n in [(0, 0), (0, 1), (0, 4)] + [(1, n) for n in range(7)]:
        mb_ref[m, n] = jnp.full((2, 2, 64, 128), 1.0 if m and n in (2, 3) else 0.0, f32)
    cp_wqkv(2).wait()
    _prep_wqkv(2, wqkv_ref, wq_ref, cq_ref, t1_ref)
    cp_x0.wait()
    cp_wqkv(1).start()
    first()
    cp_wqkv(0).wait()
    cp_wo.start()
    _prep_wqkv(0, wqkv_ref, wq_ref, cq_ref, t1_ref)
    cp_wqkv(1).wait()
    cp_w(0, 0).start()
    _prep_wqkv(1, wqkv_ref, wq_ref, cq_ref, t1_ref)
    cp_wo.wait()
    for n in range(1, 3):
        cp_w(0, n).start()

    def head():
        pc, z = flags()
        sh, att = ({}, {}), ({}, {})
        pc.add(_prep_wo(wo_ref, cw_ref.at[0], t2_ref), 3, HD[0])
        for a in range(LAG):
            for q in range(2):
                _attn_proj(a, q, sh[a], pc, pa_ref.at[a], wq_ref, cq_ref, qkv_ref)
                last = a == 1 and q == 1
                pc.flush()
                pc.add(cores(a, att[a], at_ref.at[a], range(q * nb, (q + 1) * nb)), HD[2] if last else HD[1], 1,
                       HD[3] if a else 0)
        ln, build = _attn_post(0, pc, at_ref.at[0], x_ref, cw_ref.at[z], lm_ref)
        pc.flush()
        pc.sub = SUB
        pc.add(ln, 1)
        pc.add(build, 2, lag=2)
        ln, build = _attn_post(1, pc, at_ref.at[1], x_ref, cw_ref.at[z], lm_ref)
        pc.add(ln, 1)
        pc.add(build, 1, lag=2)
        pc.flush()

    head()
    cp_x1.start()

    def wait_w(f, ns):
        for half in range(LAG):
            @pl.when(f == half)
            def _():
                for n in ns:
                    cp_w(half, n).wait()

    def wait_weights(f):
        @pl.when(f < LAG)
        def _():
            live = jnp.full((8, 128), one_ref[0], i32) > 0
            wait_w(f, (0, 1))
            _combine_proj(f, live, wg_ref, wu_ref, cgu_ref)
            wait_w(f, (2,))
            _combine_down(f, live, wdt_ref, cd_ref, cr_ref)

        @pl.when(f == 0)
        def _():
            cp_x1.wait()
            for n in range(3):
                cp_w(1, n).start()
            for half in range(LAG):
                cp_m(half).start()

            def conv(a, carry):
                x_ref[a] = xb_ref[:, pl.ds(pl.multiple_of(a * TA, TA), TA)].astype(f32)
                return carry

            lax.fori_loop(LAG, NA, conv, 0)

    def emit(it):
        ob_ref[it] = x_ref[it].astype(bf16)
        cp_out(it).start()

    def start_out(f):
        @pl.when(jnp.logical_and(f >= NA, f % LAG == LAG - 1))
        def _():
            for a in range(LAG):
                emit(f - NA - (LAG - 1) + a)

    def fused(s, carry):
        f = s - LAG
        wait_weights(f)
        pc, z = flags()
        half = f % LAG
        lm, rb, rbl = lm_ref.at[(f // LAG) % 2], rb_ref.at[0], rb_ref.at[z]
        _attn_lhs(s, x_ref, pa_ref.at[0])
        pc.by(DLHS, lambda: pa_ref[z, :8, :128])
        for t in range(4):
            _ffn_pos(lm, cgu_ref.at[half * 9 + 2 * t], cgu_ref.at[half * 9 + 2 * t + 1], t, pc, rb)
        sm, sh, att = {}, {}, {}
        for q in range(2):
            pc.add(_rem_steps(_proj_pass(lm, cgu_ref.at[half * 9 + 8], q, sm, pc), q, rb), EREM)
        _attn_proj(s, 0, sh, pc, pa_ref.at[z], wq_ref, cq_ref, qkv_ref)
        pc.flush()
        pc.add(cores(s, att, at_ref.at[0], range(C1[0])), C1[1], 4, CL)
        _attn_proj(s, 1, sh, pc, pa_ref.at[z], wq_ref, cq_ref, qkv_ref)
        pc.flush()
        pc.add(cores(s, att, at_ref.at[0], range(C1[0], 2 * nb)), C2, 1, CL)

        def mid(k):
            if k == KPOST:
                pc.flush()
                ln, build = _attn_post(s, pc, at_ref.at[z], x_ref, cw_ref.at[0], lm_ref)
                pc.sub = SUB
                pc.add(ln, ELN, DPOST)
                pc.add(build, EPOST)

        def rem(n):
            cc = 256 * (n % 2)
            return (up(cr_ref.at[half][unit(n, 144)]),
                    up(cat0(rbl[49 + n // 2, :, cc:cc + 128], rbl[49 + n // 2, :, cc + 128:cc + 256])))

        _ffn_down((f // LAG) % (S // TF),
                  lambda p: cat1(*[cd_ref.at[1 + half * 4 + t][unit(p, 72)] for t in range(4)]),
                  lambda p: rbl[p], rem, pc, x_ref, mid=mid)
        start_out(f)
        return carry

    lax.fori_loop(LAG, NSTEP, fused, 0)

    last, lm, rb = S // TF - 1, lm_ref.at[(NSTEP // LAG - 1) % 2], rb_ref.at[0]
    for half in range(LAG):
        cp_m(half).wait()
    pc, _ = flags()
    ch = Chain(pc.live[:8])

    def ninth(st, gate):
        ch.tok = pltpu.bitcast(gate(None)[:8], u32)
        st()

    blocks = [(ii, ji) for ii in range(2) for ji in range(2)]
    held = [[[[mb_ref.at[m, n, ii, ji] for ji in range(2)] for ii in range(2)] for n in range(7)] for m in range(2)]
    pc.add([functools.partial(ninth, st) for j in range(9) for st in _down_unit(ch, j, wm_ref, 0, cd_ref.at[0])], 3, 4)
    sa, sb = {}, {}
    pc.add(_build_steps(_proj_pass(lm, cgu_ref.at[8], 0, sa, pc), _proj_pass(lm, cgu_ref.at[17], 0, sb, pc),
                        0, 0, rb, True), 4, 2)

    def hold(ms, ko, ii, ki, r, gate):
        a, b = [_col(ms, ii, ji, ki, slice(r, r + 16), gate) for ji in range(2)]
        h = _mix(a[0], b[0]), _mix(a[1], b[1])
        mb_ref[0, 3 - ko, ii, ki, r:r + 16] = h[1 - ko]
        mb_ref[0, 6 - ko, ii, ki, r:r + 16] = h[ko] - h[1 - ko]
        return a[0]

    for ko, sm in enumerate((sa, sb)):
        ms = _proj_pass(lm, cgu_ref.at[8 + 9 * ko], 1, sm, pc)
        pc.add([functools.partial(hold, ms, ko, ii, ki, r) for ii, ki in blocks for r in range(0, 64, 16)], 2, 1, 4 * ko)
    pc.flush()

    def epi(c, carry):
        pc, z = flags()
        w = 2 * c + c // 4
        sa, sb = {}, {}
        pc.add(_build_steps(*held, 0, 1, rb), EE, 2)
        g, u = _proj_pass(lm, cgu_ref.at[w], 0, sa, pc), _proj_pass(lm, cgu_ref.at[w + 1], 0, sb, pc)
        pc.flush()
        _ffn_down(last, lambda p: cd_ref.at[c][unit(p, 72)], lambda p: rb_ref[z, p, :, :128], None, pc, x_ref)
        pc.add(_build_steps(g, u, 0, 0, rb), EE, 2)
        for m, sm in enumerate((sa, sb)):
            ms = _proj_pass(lm, cgu_ref.at[w + m], 1, sm, pc)
            for n in range(7):
                for ii, ji in blocks:
                    mb_ref[m, n, ii, ji] = ms[n][ii][ji]
        pc.flush()
        return carry

    lax.fori_loop(0, 8, epi, 0)
    pc.add(_build_steps(*held, 0, 1, rb), 1)
    pc.flush()

    def cp_last(io, a):
        it, rows = NA - LAG + a, pl.ds(288 * io, 288)
        return pltpu.make_async_copy(ob_ref.at[it, rows], o_hbm.at[rows, pl.ds(it * TA, TA)],
                                     sem_out.at[it + LAG * io])

    def put(io, a, v):
        ob_ref[NA - LAG + a, 288 * io:288 * io + 288, :] = v.astype(bf16)

    def mid(k):
        if k == 6:
            cp_last(1, 0).start()
            cp_last(0, 1).start()

    _ffn_down(last, lambda p: cd_ref.at[8][unit(p, 72)], lambda p: rb[p, :, :128], None, pc, x_ref, mid, put)
    cp_last(1, 1).start()
    cp_last(0, 0).start()
    for it in range(NA - LAG):
        cp_out(it).wait()
    for io, a in blocks:
        cp_last(io, a).wait()


@jax.jit
def pallas_interleave_layers__sliding_local_dilated__glu_gated_bilinear__prompt_kernel(
    A_x, A_wqkv, A_wo, B_x, B_w_gate, B_w_up, B_w_down):
    xt = A_x[0].T
    wdt = B_w_down.T
    hbm = pl.BlockSpec(memory_space=pl.ANY)
    out_t = pl.pallas_call(
        _kernel,
        in_specs=[hbm] * 6,
        out_specs=hbm,
        out_shape=jax.ShapeDtypeStruct((D, S), bf16),
        scratch_shapes=[
            pltpu.VMEM((D, S), bf16),
            pltpu.VMEM((D, 3 * D), bf16),
            pltpu.VMEM((D, D), bf16),
            pltpu.VMEM((D, FH), bf16),
            pltpu.VMEM((D, FH), bf16),
            pltpu.VMEM((D, FH), bf16),
            pltpu.VMEM((D, 512), bf16),
            pltpu.VMEM((18, 54 * 32, 256), u32),
            pltpu.VMEM((9, 25 * 72 + 8, 256), u32),
            pltpu.VMEM((2, 4 * 144, 256), u32),
            pltpu.VMEM((D // 2, NQ), u32),
            pltpu.VMEM((672, NH), u32),
            pltpu.VMEM((1, 16 * 72, 256), u32),
            pltpu.VMEM((3, 3 * D, 128), u32),
            pltpu.VMEM((5, D // 2, 128), u32),
            pltpu.VMEM((NA, D, TA), f32),
            pltpu.VMEM((2, LAG, 57 * 16, 256), u32),
            pltpu.VMEM((1, 53, 64, 512), u32),
            pltpu.VMEM((2, 7, 2, 2, 64, 128), f32),
            pltpu.VMEM((LAG, 512, 256), u32),
            pltpu.VMEM((LAG, 11 * 64, 256), u32),
            pltpu.VMEM((NA, D, TA), bf16),
            pltpu.VMEM((14, QROWS, 128), f32),
            pltpu.SMEM((1,), i32),
            pltpu.SemaphoreType.DMA((6,)),
            pltpu.SemaphoreType.DMA((4 * LAG,)),
            pltpu.SemaphoreType.DMA((NA + LAG,)),
        ],
        compiler_params=pltpu.CompilerParams(vmem_limit_bytes=116 * 1024 * 1024),
    )(xt, A_wqkv, A_wo, B_w_gate, B_w_up, wdt)
    return out_t.T[None]
```

```python
import functools
import math

import jax
import jax.numpy as jnp
from jax import lax
import jax.experimental.pallas as pl
import jax.experimental.pallas.tpu as pltpu

S, D, F = 2048, 576, 4608
H, DH, W, DIL = 32, 18, 8, 2
NQ = 14 * 128
NH = NQ // 2
HALO = 16
QROWS = S + 2 * HALO + 8
TA = 256
TF = 512
FH = F // 2
LAG = TF // TA
EVERY = 3
KPOST, DPOST, DLHS = 5, 1, 110
SUB, ELN, EPOST = 3, 1, 2
C1, C2 = (6, 7), 3
EREM = 5
CL = 0
EE = 3
HD = (22, 6, 1, 0)
LEAD = 2
NCH = 2
RB = 16
NA = S // TA
NSTEP = 2 * NA
EPS = 1e-5
bf16, f32, u32, i32 = jnp.bfloat16, jnp.float32, jnp.uint32, jnp.int32
NT = (((1,), (1,)), ((), ()))
SCALE = DH ** -0.5
EXP2_C = SCALE * math.log2(math.e)
NEG = -1e9 / SCALE

ORD = (0, 2, 3, 1, 4, 5, 6)
SPEC = {1: (1, (0,)), 4: (0, (1,)), 5: (1, (0, 1)), 6: (0, (0, 1))}
SETS = ((0,), (1,), (0, 1))
QSUM = (0, 2, 3, 5, 6)
SIDX = {n: k for k, n in enumerate(SPEC)}

dot = functools.partial(jnp.dot, preferred_element_type=f32)


def dnt(a, b):
    return lax.dot_general(a, b, NT, preferred_element_type=f32)


def cat0(*xs):
    return xs[0] if len(xs) == 1 else jnp.concatenate(xs, axis=0)


def cat1(*xs):
    return xs[0] if len(xs) == 1 else jnp.concatenate(xs, axis=1)


def tb(x):
    return x.T.astype(bf16)


def pkb(x):
    return pltpu.bitcast(x.astype(bf16), u32)


def pkt(x):
    return pltpu.bitcast(tb(x), u32)


def up(x):
    return pltpu.bitcast(x, bf16)


def _chain_sum(load, fn):
    acc = None
    for r in range(0, D, 8 * NCH):
        t = fn(load(r, 8 * NCH))
        acc = t if acc is None else acc + t
    return jnp.sum(acc, axis=0, keepdims=True)


def _ln_t(load, m=None):
    if m is None:
        m = _chain_sum(load, lambda v: v) * (1.0 / D)
    r = lax.rsqrt(_chain_sum(load, lambda v: (v - m) * (v - m)) * (1.0 / D) + EPS)
    return load(0, D) * r - m * r


def _ln_steps(load, m, out):
    st = {}

    def wide(gate, v):
        v = jnp.broadcast_to(v, (16, TA))
        return cat1(gate(v[:, :128]), gate(v[:, 128:]))

    def var(r0, gate):
        mg = wide(gate, m)
        for r in range(r0, r0 + 96, 16):
            d = load(r, 16) - mg
            st["acc"] = d * d if r == 0 else st["acc"] + d * d

    def norm(c, gate):
        if c == 0:
            st["r"] = lax.rsqrt(jnp.sum(st["acc"], axis=0, keepdims=True) * (1.0 / D) + EPS)
            st["mr"] = jnp.broadcast_to(m * st["r"], (16, TA))
        rg = wide(gate, st["r"])
        z = [load(r, 16) * rg - st["mr"] for r in range(128 * c, min(128 * c + 128, D), 16)]
        out.append(cat0(*(z if c < 4 else z + z)).T)

    return [functools.partial(var, r) for r in range(0, D, 96)] + [functools.partial(norm, c) for c in range(5)]


def _prep_wqkv(c, wqkv_ref, wq_ref, cq_ref, t1_ref):
    n = min(256, D - 256 * c)
    wp = pltpu.bitcast(wqkv_ref[256 * c:256 * c + n, :], u32)
    if n < 256:
        wp = cat0(wp, jnp.zeros(((256 - n) // 2, 3 * D), u32))
    t1_ref[c] = wp.T

    def rows(t, d):
        return t1_ref[c, pl.ds(t * D + d, H, stride=DH), :]

    parts = []
    for t in range(3):
        parts += [rows(t, d) for d in (0, 2, 4, 6, 1, 3, 5, 7, 8, 10, 12, 14, 9, 11, 13, 15)]
    parts += [rows(0, 16), rows(0, 17), rows(2, 16), rows(2, 17)]
    parts += [rows(1, 16), rows(1, 17), jnp.zeros((32, 128), u32), jnp.zeros((32, 128), u32)]
    for t in range(7):
        w = [cat0(*parts[4 * k:4 * k + 4]).T[:n // 2] for k in (t, t + 7)]
        for k, v in zip((t, t + 7), w):
            wq_ref[128 * c:128 * c + n // 2, 128 * k:128 * k + 128] = v
        cols = slice(128 * t, 128 * t + 128)
        if c == 2:
            cq_ref[640:, cols] = pkb(unp(w[0]) + unp(w[1]))
        if c == 1:
            for r in range(0, 128, 8):
                ops = rhs7(*[unp(wq_ref[r:r + 8, 128 * k:128 * k + 128]) for k in (t, t + 7)],
                           *[unp(v[r:r + 8]) for v in w])
                for k, m in enumerate(QSUM):
                    cq_ref[128 * k + r:128 * k + r + 8, cols] = pkb(ops[m]())


def _share_lhs(load, rows, dst):
    lo = lax.broadcasted_iota(i32, (16, 128), 1) < 64

    def step(r, gate):
        blk = [[load(q, i, r, gate) for i in range(2)] for q in range(2)]
        for c in range(2):
            ops = [lhs7(b[0][c], b[0][2 + c], b[1][c], b[1][2 + c]) for b in blk]
            for n in range(7):
                x1, x2 = ops[0][n](), ops[1][n]()
                if c == 1 and n in SPEC:
                    r1, r2 = blk[0][SPEC[n][0]][4], blk[1][SPEC[n][0]][4]
                    dst[unit(28 + SIDX[n], rows, r // 2, 8)] = pkb(jnp.where(lo, r1, x2))
                    x1, x2 = jnp.where(lo, x1, x1 - x2), jnp.where(lo, x2, r2 - r1)
                dst[unit(4 * n + c, rows, r // 2, 8)] = pkb(x1)
                dst[unit(4 * n + 2 + c, rows, r // 2, 8)] = pkb(x2)
        return x1

    return [functools.partial(step, r) for r in range(0, 2 * rows, 16)]


def _prep_wo(wo_ref, cw_ref, t2_ref):
    wo = cat1(pltpu.bitcast(wo_ref[...], u32), jnp.zeros((D // 2, 64), u32))
    for c in range(5):
        t2_ref[c] = wo[:, c * 128:(c + 1) * 128]
    wt = []
    for c in range(5):
        wt.append(cat0(*[t2_ref[c, pl.ds(p, H, stride=DH // 2), :] for p in tuple(range(8)) + (8,) * 4]).T)
    wt = cat0(*wt)
    odd = lax.broadcasted_iota(i32, (16, 128), 1) % 64 >= 32

    def load(q, i, r, gate):
        o = 288 * i + 144 * q + r
        out = []
        for c in range(3):
            w = gate(wt[o:o + 16, 128 * c:128 * c + 128])
            out += [pltpu.bitcast(w << 16, f32), pltpu.bitcast(w & jnp.uint32(0xFFFF0000), f32)]
        return out[:4] + [jnp.where(odd, out[5], out[4])]

    return _share_lhs(load, 72, cw_ref)


def _base(s):
    return s % NA * TA if isinstance(s, int) else pl.multiple_of((s % NA) * TA, TA)


def _attn_lhs(s, x_ref, pa):
    item = s % NA
    z = _ln_t(lambda r, n: x_ref[item, r:r + n, :])
    zt = cat0(z, z[512:]).T

    def load(q, i, r, gate):
        o = 128 * q + 64 * i + r
        return [zt[o:o + 16, 128 * c:128 * c + 128] for c in range(5)]

    for st in _share_lhs(load, 32, pa):
        st(None)


def _attn_proj(s, q, sh, pc, pa, wq_ref, cq_ref, qkv_ref):
    item = s % NA
    t0 = _base(s)
    lo = lax.broadcasted_iota(i32, (64, 128), 1) < 64
    for t in range(7):
        def wts(n, r, k):
            c = 128 * t
            if n in QSUM:
                return cq_ref[128 * QSUM.index(n) + r:128 * QSUM.index(n) + r + k, c:c + 128]
            return wq_ref[r:r + k, c:c + 128] if n == 1 else wq_ref[128 + r:128 + r + k, NH + c:NH + c + 128]

        def wrem(n):
            c = 128 * t + (NH if n == 4 else 0)
            return (wq_ref[256:, c:c + 128] if n in (1, 4) else cq_ref[640:, c:c + 128])

        p = [None] * 7
        for n in ORD:
            x = pc.pre(pa[64 * n + 32 * q:64 * n + 32 * q + 32, :])
            if n in SPEC:
                if q == 0:
                    sh[t, n] = dot(up(pa[unit(28 + SIDX[n], 32)]), up(cat0(wrem(n), wts(n, 96, 32))))
                w = cat0(wts(n, 0, 96), wrem(n)) if q else wts(n, 0, 128)
                p[n] = dot(up(x), up(w)) + sh[t, n]
            else:
                p[n] = dot(up(x), up(wts(n, 0, 128)))
            pc.tick(p[n])
        y = out4(p)
        for i in range(2):
            for j in range(2):
                c, v = t + 7 * j, y[i][j]
                if c == 13:
                    v = jnp.where(lo, v, 0.0)
                qkv_ref[c, pl.ds(t0 + (HALO + 128 * q + 64 * i), 64), :] = v
                if q == 0 and i == 0 and c >= 4 and not (isinstance(s, int) and s):
                    hrow = 0 if isinstance(s, int) else pl.multiple_of(jnp.where(item == 0, 0, S + HALO), HALO)
                    qkv_ref[c, pl.ds(hrow, HALO), :] = jnp.broadcast_to(v[0:1], (HALO, 128))


def _attn_core(s, b, qkv_ref, gate):
    t0 = _base(s)
    qi = (0, 1, 2, 3, 12)
    ki = (4, 5, 6, 7, 13)
    vi = (8, 9, 10, 11, 12)
    r0 = t0 + (b * RB + HALO)
    q = [cat0(*[gate(qkv_ref[c, pl.ds(r0 + r, 16), :]) for r in range(0, RB, 16)]) for c in qi]
    ls = []
    for w in range(W):
        acc = None
        for c in range(5):
            t = q[c] * qkv_ref[ki[c], pl.ds(r0 - DIL * w, RB), :]
            acc = t if acc is None else acc + t
        acc = acc + pltpu.roll(acc, 64, 1)
        acc = acc + pltpu.roll(acc, 32, 1)
        if w > 0 and b == 0 and not (isinstance(s, int) and s):
            pos = t0 + lax.broadcasted_iota(i32, (HALO, 128), 0)
            top = jnp.where(pos >= DIL * w, acc[:HALO], NEG)
            acc = top if RB == HALO else cat0(top, acc[HALO:])
        ls.append(acc)
    m = functools.reduce(jnp.maximum, ls)
    pr = [jnp.exp2((l - m) * EXP2_C) for l in ls]
    inv = 1.0 / functools.reduce(jnp.add, pr)
    out = []
    for c in range(5):
        acc = None
        for w in range(W):
            t = pr[w] * qkv_ref[vi[c], pl.ds(r0 - DIL * w, RB), :]
            acc = t if acc is None else acc + t
        out.append(acc * inv)
    return out


def _attn_rhs(b, a0, a1, at):
    lo = lax.broadcasted_iota(i32, (RB, 128), 1) < 64
    rem = (a0[4], a1[4], a0[4] + a1[4])
    rem = [(r, pltpu.roll(r, 64, 1)) for r in rem]
    for c in range(2):
        ops = rhs7(a0[c], a1[c], a0[2 + c], a1[2 + c])
        for n in range(7):
            v = ops[n]()
            at[unit(2 * n + c, 64, b * RB // 2, RB // 2)] = pkb(v)
            if c == 1 and n in SPEC:
                hi, low = rem[SETS.index(SPEC[n][1])]
                at[unit(14 + 2 * SIDX[n], 64, b * RB // 2, RB // 2)] = pkb(jnp.where(lo, v, hi))
                at[unit(15 + 2 * SIDX[n], 64, b * RB // 2, RB // 2)] = pkb(jnp.where(lo, low, v))


def lhs7(a11, a12, a21, a22):
    return (lambda: a11 + a22, lambda: a21 + a22, lambda: a11, lambda: a22,
            lambda: a11 + a12, lambda: a21 - a11, lambda: a12 - a22)


def rhs7(b11, b12, b21, b22):
    return (lambda: b11 + b22, lambda: b11, lambda: b12 - b22, lambda: b21 - b11,
            lambda: b22, lambda: b11 + b12, lambda: b21 + b22)


def out4(m):
    m1, m2, m3, m4, m5, m6, m7 = m
    return [[m1 + m4 - m5 + m7, m3 + m5], [m2 + m4, m1 + m3 - m2 + m6]]


def unit(u, rows, off=0, n=None):
    off = rows * (u // 2) + off
    n = rows if n is None else n
    r = slice(off, off + n) if isinstance(off, int) else pl.ds(pl.multiple_of(off, 8), n)
    return r, slice(128 * (u % 2), 128 * (u % 2) + 128)


def _attn_post(s, pc, at, x_ref, cw_ref, lm_ref):
    item = s % NA
    sh, y = {}, []
    for q in range(2):
        p = [None] * 7
        for n in ORD:
            w = up(cw_ref[144 * n + 72 * q:144 * n + 72 * q + 72, :])
            if n in SPEC:
                if q == 0:
                    sh[n] = dnt(up(cw_ref[unit(28 + SIDX[n], 72)]), up(at[unit(15 + 2 * SIDX[n], 64)]))
                last = at[unit(14 + 2 * SIDX[n] if q else 2 * n + 1, 64)]
                p[n] = dnt(w, up(cat1(at[unit(2 * n, 64)], last))) + sh[n]
            else:
                p[n] = dnt(w, up(at[64 * n:64 * n + 64, :]))
            pc.tick(p[n])
        y.append(out4(p))
    xt = x_ref[item] + cat0(*[cat1(*y[q][i]) for i in range(2) for q in range(2)])
    x_ref[item] = xt
    m = _chain_sum(lambda r, n: xt[r:r + n], lambda v: v) * (1.0 / D)
    zt = []
    dst = lm_ref.at[(s // LAG) % 2, s % LAG]
    lo = lax.broadcasted_iota(i32, (16, 128), 1) < 64

    def step(r, n, gate):
        def blk(q, i, k):
            o = 64 * i + 32 * q + r
            return zt[k][o:o + 16]

        g11, g22 = (gate, lambda v: v) if n in (0, 2, 4, 5) else (lambda v: v, gate)
        inner = [lhs7(*[lhs7(g11(blk(q, i, k)), blk(q, i, 2 + k), blk(q, 2 + i, k), g22(blk(q, 2 + i, 2 + k)))[n]()
                        for i in range(2) for k in range(2)]) for q in range(2)]
        for l in range(7):
            x1, x2 = inner[0][l](), inner[1][l]()
            if n in SPEC and l in SPEC:
                i = 2 * SPEC[n][0] + SPEC[l][0]
                r1, r2 = blk(0, i, 4), blk(1, i, 4)
                dst[unit(98 + 4 * SIDX[n] + SIDX[l], 16, r // 2, 8)] = pkb(jnp.where(lo, r1, x2))
                x1, x2 = jnp.where(lo, x1, x1 - x2), jnp.where(lo, x2, r2 - r1)
            dst[unit(2 * (7 * n + l), 16, r // 2, 8)] = pkb(x1)
            dst[unit(2 * (7 * n + l) + 1, 16, r // 2, 8)] = pkb(x2)
        return x1

    return (_ln_steps(lambda r, n: x_ref[item, r:r + n, :], m, zt),
            [functools.partial(step, r, n) for r in (0, 16) for n in range(7)])


class Pacer:
    def __init__(self, live):
        self.live, self.todo, self.wait, self.due, self.sub, self.done = live, [], 0, [], 1, []

    def add(self, steps, every, delay=0, lag=0):
        if not self.todo:
            self.wait = delay
        self.todo += [(st, every, lag) for st in steps]

    def run(self, toks):
        st, self.wait, lag = self.todo.pop(0)
        if lag and len(self.done) >= lag and self.done[-lag] is not None:
            toks = toks + [self.done[-lag]]

        def gate(v):
            if v is None:
                return toks[0]
            for t in toks:
                v = jnp.where(self.live, v, t if v.dtype == t.dtype else pltpu.bitcast(t, v.dtype))
            return v

        self.done.append(st(gate))

    def tick(self, p):
        for k in range(self.sub):
            self.wait -= 1
            if self.todo and self.wait <= 0:
                o = p.shape[0] // self.sub * k
                self.run([p[o:o + 16, :128]])

    def by(self, count, load):
        self.due.append([count, load()])

    def pre(self, w):
        for d in self.due:
            d[0] -= 1
        while self.due and self.due[0][0] <= 0:
            v = jnp.where(self.live[:8], w[:8, :128], self.due.pop(0)[1])
            w = cat0(cat1(v, w[:8, 128:]) if w.shape[1] > 128 else v, w[8:])
        return w

    def flush(self):
        while self.todo:
            self.run([])


def wunit(p, part, off=0, n=32):
    if part == 2:
        p, part = (49, p) if p < 2 else (50 + p % 2, p // 2 - 1)
    return unit(p, 64, 32 * part + off, n)


def _row(ref, r, c, n):
    c = 128 * c if isinstance(c, int) else pl.multiple_of(128 * c, 128)
    r = r if isinstance(r, int) else pl.multiple_of(r, 16)
    v = pltpu.bitcast(ref[pl.ds(r, 16), pl.ds(c, 128 * n)], u32)
    return [v[:, 128 * k:128 * k + 128] for k in range(n)]


def unp(v):
    return up(v).astype(f32)


class Chain:
    def __init__(self, live):
        self.live, self.tok = live, None

    def stage(self, blocks, emit, lead=LEAD):
        tok, self.tok = self.tok, None
        for k, (idx, v) in enumerate(emit([unp(v if tok is None else jnp.where(self.live, v, tok)) for v in blocks])):
            v = pkb(v)
            idx[0][idx[1]] = v
            if k <= lead:
                self.tok = v

    def two_level(self, fn, blk, where):
        quad = lambda a, b: [blk[2 * a + i][2 * b + j] for i in range(2) for j in range(2)]
        got = {}

        def emit(keys, ns, vals):
            for k, key in enumerate(keys):
                got[key] = vals[4 * k:4 * k + 4]
            for n in ns:
                q = [got.get(c, (None,) * 4) for c in ((0, 0), (0, 1), (1, 0), (1, 1))]
                inner = fn(*[fn(*[c[x] for c in q])[n]() for x in range(4)])
                for l in range(7):
                    yield where(7 * n + l), inner[l]()

        plan = ((1, 4, 0), (5, 2), (3, 6)) if fn is rhs7 else ((2, 3, 0), (4, 6), (1, 5))
        return [functools.partial(self.stage, sum((quad(*k) for k in keys), []), functools.partial(emit, keys, ns))
                for keys, ns in zip((((0, 0), (1, 1)), ((0, 1),), ((1, 0),)), plan)]


def _shift(ref, off, most):
    return ref.at[pl.ds(off if isinstance(off, int) else pl.multiple_of(off, 8), ref.shape[0] - most)]


def _combine_proj(half, live, wg_ref, wu_ref, c_ref):
    lo = lax.broadcasted_iota(i32, (8, 128), 1) < 64

    def row(r, tile):
        if tile < 8:
            return _row((wg_ref, wu_ref)[tile % 2], r, 4 * (tile // 2), 4)
        out = []
        for g, u in zip(_row(wg_ref, r, 16, 2), _row(wu_ref, r, 16, 2)):
            w = pltpu.roll(jnp.where(lo, u, g), 64, 1)
            out += [jnp.where(lo, g, w), jnp.where(lo, w, u)]
        return out

    def body(j, carry):
        ch = Chain(live)
        for tile in (0, 8, 1, 2, 3, 4, 5, 6, 7):
            dst = _shift(c_ref.at[half * 9 + tile], 8 * j, 24)

            def emit(r):
                for a, (x, y) in enumerate(((r[0], r[1]), (r[2], r[3]), (r[0] + r[2], r[1] + r[3]))):
                    for b, v in enumerate((x, y, x + y)):
                        yield (dst, wunit(3 * a + b, 2, 0, 8)), v

            for part in range(2):
                blk = [row(128 * k + 64 * part + 16 * j, tile) for k in range(4)]
                for st in ch.two_level(rhs7, blk, lambda p: (dst, wunit(p, part, 0, 8))):
                    st()
            ch.stage(row(512 + 16 * j, tile), emit, 0)
        return carry

    lax.fori_loop(0, 4, body, 0)


def _down_unit(ch, j, w_ref, c, dst):
    dst = _shift(dst, 8 * j, 64)
    blk = [_row(w_ref, 144 * k + 16 * j, c, 4) for k in range(4)]
    return ch.two_level(lhs7, blk, lambda p: (dst, unit(p, 72, 0, 8)))


def _combine_down(half, live, wdt_ref, cd_ref, cr_ref):
    def body(j, carry):
        ch = Chain(live)
        for t in range(4):
            for st in _down_unit(ch, j, wdt_ref, 4 * t, cd_ref.at[1 + half * 4 + t]):
                st()
        dst = _shift(cr_ref.at[half], 8 * j, 64)
        for c in range(2):
            r = 144 * c + 16 * j
            ch.stage(_row(wdt_ref, r, 16, 2) + _row(wdt_ref, 288 + r, 16, 2),
                     lambda a: [((dst, unit(n, 144, 72 * c, 8)), lhs7(*a)[n]()) for n in range(7)])
        return carry

    lax.fori_loop(0, 9, body, 0)


def _proj_pass(lm, w, q, sh, pc):
    def lhs(u):
        return up(pc.pre(cat0(*[lm.at[a][unit(u, 16)] for a in range(LAG)])))

    def wts(a, b):
        return up(cat0(w[wunit(*a)], w[wunit(*b)]))

    def prod(n, l):
        p = 7 * n + l
        if n in SPEC and l in SPEC:
            wr = (3 * SETS.index(SPEC[n][1]) + SETS.index(SPEC[l][1]), 2)
            if q == 0:
                sh[p] = dot(lhs(98 + 4 * SIDX[n] + SIDX[l]), wts(wr, (p, 1)))
            return dot(lhs(2 * p + q), wts((p, 0), wr if q else (p, 1))) + sh[p]
        return dot(lhs(2 * p + q), wts((p, 0), (p, 1)))

    ms = [None] * 7
    for n in ORD:
        p = [None] * 7
        for l in ORD:
            p[l] = prod(n, l)
            pc.tick(p[l])
        ms[n] = out4(p)
    return ms


def _col(ms, ii, ji, jo, rows, gate):
    m1, m2, m3, m4, m5, m6, m7 = [m[ii][ji][rows] for m in ms]
    if jo == 0:
        a = gate(m4)
        return a + m1 - m5 + m7, a + m2
    a = gate(m3)
    return a + m5, a + m1 - m2 + m6


def _mix(a, b):
    lo = lax.broadcasted_iota(i32, a.shape, 1) < 64
    return jnp.where(lo, a, b) * pltpu.roll(jnp.where(lo, b, a), 64, 1)


def _build_steps(mg, mu, t, q, rb, merged=False):
    def form(e, r, blk, k, gate):
        rows = slice(32 * k[1] + r, 32 * k[1] + r + 16)
        blk[k] = []
        for ki in range(2):
            if merged:
                a, b = [_col((mg, mu)[k[0]], e, ji, ki, rows, gate) for ji in range(2)]
                blk[k] += [_mix(a[0], b[0]), _mix(a[1], b[1])]
            else:
                g, u = _col(mg, e, ki, k[0], rows, gate), _col(mu, e, ki, k[0], rows, gate)
                blk[k] += [g[0] * u[0], g[1] * u[1]]

    def emit(e, r, blk, k, n, gate):
        o = 32 * e + 16 * q + r // 2
        quad = [[gate(v) for v in blk[c]] if c == k else blk.get(c, (None,) * 4)
                for c in ((0, 0), (0, 1), (1, 0), (1, 1))]
        inner = rhs7(*[rhs7(*[c[x] for c in quad])[n]() for x in range(4)])
        for l in range(7):
            rb.at[7 * n + l][o:o + 8, 128 * t:128 * t + 128] = pkb(inner[l]())

    def both(e, r, blk, k, n, gate):
        form(e, r, blk, k, gate)
        emit(e, r, blk, k, n, lambda v: v)

    steps = []
    for e in range(2):
        for r in (0, 16):
            blk = {}
            for k, ns in (((0, 0), (1,)), ((1, 1), (4, 0)), ((0, 1), (5, 2)), ((1, 0), (3, 6))):
                steps.append(functools.partial(both, e, r, blk, k, ns[0]))
                steps += [functools.partial(emit, e, r, blk, k, n) for n in ns[1:]]
    return steps


def _rem_steps(ms, q, rb):
    def step(ii, r, gate):
        h = []
        for jo in range(2):
            for item in range(2):
                rows = slice(32 * item + r, 32 * item + r + 16)
                a, b = [_col(ms, ii, ji, jo, rows, gate) for ji in range(2)]
                h.append([_mix(a[io], b[io]) for io in range(2)])
        for io in range(2):
            ops = rhs7(*[v[io] for v in h])
            for n in range(7):
                o, cc = 32 * ii + 16 * q + r // 2, 256 * (n % 2) + 128 * io
                rb.at[49 + n // 2][o:o + 8, cc:cc + 128] = pkb(ops[n]())

    return [functools.partial(step, ii, r) for ii in range(2) for r in (0, 16)]


def _ffn_pos(lm, wa, wb, t, pc, rb):
    sa, sb = {}, {}
    for q in range(2):
        g = _proj_pass(lm, wa, q, sa, pc)
        u = _proj_pass(lm, wb, q, sb, pc)
        pc.add(_build_steps(g, u, t, q, rb), EVERY, 4)


def _ffn_down(tile, wts, rhs, rem, pc, x_ref, mid=lambda k: None, put=None):
    ms = [None] * 7

    def rdot(n):
        r = dnt(*rem(n))
        pc.tick(r)
        return r

    def group(n, base):
        if rem and n != ORD[0]:
            base = rdot(n) if base is None else base + rdot(n)
        p = [None] * 7
        for l in ORD:
            p[l] = dnt(up(pc.pre(wts(7 * n + l))), up(rhs(7 * n + l)))
            pc.tick(p[l])
        m1, m2, m3, m4, m5, m6, m7 = p
        if base is None:
            m = out4(p)
        else:
            b = [[base[144 * i:144 * i + 144, 128 * j:128 * j + 128] for j in range(2)] for i in range(2)]
            m = [[b[0][0] + m1 + m4 - m5 + m7, b[0][1] + m3 + m5],
                 [b[1][0] + m4 + m2, b[1][1] + m1 + m3 - m2 + m6]]
        base = cat0(cat1(*m[0]), cat1(*m[1]))
        if rem and n == ORD[0]:
            base = base + rdot(n)
        return base

    def xs(io, a):
        return x_ref.at[tile * LAG + a, 288 * io:288 * io + 288, :]

    def keep(io, a, v):
        xs(io, a)[...] = v

    put = put or keep
    for k, n in enumerate(ORD):
        mid(k)
        if n == 5:
            put(1, 1, group(n, xs(1, 1)[...] + ms[0] + ms[2] - ms[1]))
        elif n == 6:
            put(0, 0, group(n, xs(0, 0)[...] + ms[0] + ms[3] - ms[4]))
        else:
            ms[n] = group(n, None)
            if n == 1:
                put(1, 0, xs(1, 0)[...] + ms[3] + ms[1])
            elif n == 4:
                put(0, 1, xs(0, 1)[...] + ms[2] + ms[4])
    pc.flush()


def _kernel(xt_hbm, wqkv_hbm, wo_hbm, wg_hbm, wu_hbm, wdt_hbm, o_hbm,
            xb_ref, wqkv_ref, wo_ref, wg_ref, wu_ref, wdt_ref, wm_ref,
            cgu_ref, cd_ref, cr_ref, wq_ref, cq_ref, cw_ref, t1_ref, t2_ref, x_ref,
            lm_ref, rb_ref, mb_ref, pa_ref, at_ref, ob_ref, qkv_ref, one_ref, sem_in, sem_w, sem_out):
    def cp_wqkv(c):
        rows = pl.ds(256 * c, min(256, D - 256 * c))
        return pltpu.make_async_copy(wqkv_hbm.at[rows], wqkv_ref.at[rows], sem_in.at[c])

    cp_x0 = pltpu.make_async_copy(xt_hbm.at[:, pl.ds(0, TF)], xb_ref.at[:, pl.ds(0, TF)], sem_in.at[3])
    cp_wo = pltpu.make_async_copy(wo_hbm, wo_ref, sem_in.at[4])
    cp_x1 = pltpu.make_async_copy(xt_hbm.at[:, pl.ds(TF, S - TF)], xb_ref.at[:, pl.ds(TF, S - TF)], sem_in.at[5])

    def cp_w(half, n):
        src, dst = ((wg_hbm, wg_ref), (wu_hbm, wu_ref), (wdt_hbm, wdt_ref))[n]
        return pltpu.make_async_copy(src.at[:, pl.ds(half * FH, FH)], dst, sem_w.at[half * 3 + n])

    def cp_m(half):
        return pltpu.make_async_copy(wdt_hbm.at[:, pl.ds(half * FH + 2048, 256)],
                                     wm_ref.at[:, pl.ds(half * 256, 256)], sem_w.at[3 * LAG + half])

    def cp_out(it):
        o = it * TA
        sl = pl.ds(o if isinstance(o, int) else pl.multiple_of(o, TA), TA)
        return pltpu.make_async_copy(ob_ref.at[it], o_hbm.at[:, sl], sem_out.at[it])

    def flags():
        one = one_ref[0]
        return Pacer(jnp.full((16, 128), one, i32) > 0), one - 1

    nb = TA // 2 // RB

    def cores(s, att, at, blocks):
        def step(b, gate):
            att[b] = _attn_core(s, b, qkv_ref, gate)
            if b >= nb:
                _attn_rhs(b - nb, att[b - nb], att[b], at)
            return att[b][0]
        return [functools.partial(step, b) for b in blocks]

    def first():
        for a in range(LAG):
            x_ref[a] = xb_ref[:, a * TA:(a + 1) * TA].astype(f32)
            _attn_lhs(a, x_ref, pa_ref.at[a])

    cp_wqkv(2).start()
    cp_x0.start()
    cp_wqkv(0).start()
    one_ref[0] = 1
    for m, n in [(0, 0), (0, 1), (0, 4)] + [(1, n) for n in range(7)]:
        mb_ref[m, n] = jnp.full((2, 2, 64, 128), 1.0 if m and n in (2, 3) else 0.0, f32)
    cp_wqkv(2).wait()
    _prep_wqkv(2, wqkv_ref, wq_ref, cq_ref, t1_ref)
    cp_x0.wait()
    cp_wqkv(1).start()
    first()
    cp_wqkv(0).wait()
    cp_wo.start()
    _prep_wqkv(0, wqkv_ref, wq_ref, cq_ref, t1_ref)
    cp_wqkv(1).wait()
    cp_w(0, 0).start()
    _prep_wqkv(1, wqkv_ref, wq_ref, cq_ref, t1_ref)
    cp_wo.wait()
    for n in range(1, 3):
        cp_w(0, n).start()

    def head():
        pc, z = flags()
        sh, att = ({}, {}), ({}, {})
        pc.add(_prep_wo(wo_ref, cw_ref.at[0], t2_ref), 3, HD[0])
        for a in range(LAG):
            for q in range(2):
                _attn_proj(a, q, sh[a], pc, pa_ref.at[a], wq_ref, cq_ref, qkv_ref)
                last = a == 1 and q == 1
                pc.flush()
                pc.add(cores(a, att[a], at_ref.at[a], range(q * nb, (q + 1) * nb)), HD[2] if last else HD[1], 1,
                       HD[3] if a else 0)
        ln, build = _attn_post(0, pc, at_ref.at[0], x_ref, cw_ref.at[z], lm_ref)
        pc.flush()
        pc.sub = SUB
        pc.add(ln, 1)
        pc.add(build, 2, lag=2)
        ln, build = _attn_post(1, pc, at_ref.at[1], x_ref, cw_ref.at[z], lm_ref)
        pc.add(ln, 1)
        pc.add(build, 1, lag=2)
        pc.flush()

    head()
    cp_x1.start()

    def wait_w(f, ns):
        for half in range(LAG):
            @pl.when(f == half)
            def _():
                for n in ns:
                    cp_w(half, n).wait()

    def wait_weights(f):
        @pl.when(f < LAG)
        def _():
            live = jnp.full((8, 128), one_ref[0], i32) > 0
            wait_w(f, (0, 1))
            _combine_proj(f, live, wg_ref, wu_ref, cgu_ref)
            wait_w(f, (2,))
            _combine_down(f, live, wdt_ref, cd_ref, cr_ref)

        @pl.when(f == 0)
        def _():
            cp_x1.wait()
            for n in range(3):
                cp_w(1, n).start()
            for half in range(LAG):
                cp_m(half).start()

            def conv(a, carry):
                x_ref[a] = xb_ref[:, pl.ds(pl.multiple_of(a * TA, TA), TA)].astype(f32)
                return carry

            lax.fori_loop(LAG, NA, conv, 0)

    def emit(it):
        ob_ref[it] = x_ref[it].astype(bf16)
        cp_out(it).start()

    def start_out(f):
        @pl.when(jnp.logical_and(f >= NA, f % LAG == LAG - 1))
        def _():
            for a in range(LAG):
                emit(f - NA - (LAG - 1) + a)

    def fused(s, carry):
        f = s - LAG
        wait_weights(f)
        pc, z = flags()
        half = f % LAG
        lm, rb, rbl = lm_ref.at[(f // LAG) % 2], rb_ref.at[0], rb_ref.at[z]
        _attn_lhs(s, x_ref, pa_ref.at[0])
        pc.by(DLHS, lambda: pa_ref[z, :8, :128])
        for t in range(4):
            _ffn_pos(lm, cgu_ref.at[half * 9 + 2 * t], cgu_ref.at[half * 9 + 2 * t + 1], t, pc, rb)
        sm, sh, att = {}, {}, {}
        for q in range(2):
            pc.add(_rem_steps(_proj_pass(lm, cgu_ref.at[half * 9 + 8], q, sm, pc), q, rb), EREM)
        _attn_proj(s, 0, sh, pc, pa_ref.at[z], wq_ref, cq_ref, qkv_ref)
        pc.flush()
        pc.add(cores(s, att, at_ref.at[0], range(C1[0])), C1[1], 4, CL)
        _attn_proj(s, 1, sh, pc, pa_ref.at[z], wq_ref, cq_ref, qkv_ref)
        pc.flush()
        pc.add(cores(s, att, at_ref.at[0], range(C1[0], 2 * nb)), C2, 1, CL)

        def mid(k):
            if k == KPOST:
                pc.flush()
                ln, build = _attn_post(s, pc, at_ref.at[z], x_ref, cw_ref.at[0], lm_ref)
                pc.sub = SUB
                pc.add(ln, ELN, DPOST)
                pc.add(build, EPOST)

        def rem(n):
            cc = 256 * (n % 2)
            return (up(cr_ref.at[half][unit(n, 144)]),
                    up(cat0(rbl[49 + n // 2, :, cc:cc + 128], rbl[49 + n // 2, :, cc + 128:cc + 256])))

        _ffn_down((f // LAG) % (S // TF),
                  lambda p: cat1(*[cd_ref.at[1 + half * 4 + t][unit(p, 72)] for t in range(4)]),
                  lambda p: rbl[p], rem, pc, x_ref, mid=mid)
        start_out(f)
        return carry

    lax.fori_loop(LAG, NSTEP, fused, 0)

    last, lm, rb = S // TF - 1, lm_ref.at[(NSTEP // LAG - 1) % 2], rb_ref.at[0]
    for half in range(LAG):
        cp_m(half).wait()
    pc, _ = flags()
    ch = Chain(pc.live[:8])

    def ninth(st, gate):
        ch.tok = pltpu.bitcast(gate(None)[:8], u32)
        st()

    blocks = [(ii, ji) for ii in range(2) for ji in range(2)]
    held = [[[[mb_ref.at[m, n, ii, ji] for ji in range(2)] for ii in range(2)] for n in range(7)] for m in range(2)]
    pc.add([functools.partial(ninth, st) for j in range(9) for st in _down_unit(ch, j, wm_ref, 0, cd_ref.at[0])], 3, 4)
    sa, sb = {}, {}
    pc.add(_build_steps(_proj_pass(lm, cgu_ref.at[8], 0, sa, pc), _proj_pass(lm, cgu_ref.at[17], 0, sb, pc),
                        0, 0, rb, True), 2, 2)

    def hold(ms, ko, ii, ki, r, gate):
        a, b = [_col(ms, ii, ji, ki, slice(r, r + 16), gate) for ji in range(2)]
        h = _mix(a[0], b[0]), _mix(a[1], b[1])
        mb_ref[0, 3 - ko, ii, ki, r:r + 16] = h[1 - ko]
        mb_ref[0, 6 - ko, ii, ki, r:r + 16] = h[ko] - h[1 - ko]
        return a[0]

    for ko, sm in enumerate((sa, sb)):
        ms = _proj_pass(lm, cgu_ref.at[8 + 9 * ko], 1, sm, pc)
        pc.add([functools.partial(hold, ms, ko, ii, ki, r) for ii, ki in blocks for r in range(0, 64, 16)], 2, 1, 4 * ko)
    pc.flush()

    def epi(c, carry):
        pc, z = flags()
        w = 2 * c + c // 4
        sa, sb = {}, {}
        pc.add(_build_steps(*held, 0, 1, rb), EE, 2)
        g, u = _proj_pass(lm, cgu_ref.at[w], 0, sa, pc), _proj_pass(lm, cgu_ref.at[w + 1], 0, sb, pc)
        pc.flush()
        _ffn_down(last, lambda p: cd_ref.at[c][unit(p, 72)], lambda p: rb_ref[z, p, :, :128], None, pc, x_ref)
        pc.add(_build_steps(g, u, 0, 0, rb), EE, 2)
        for m, sm in enumerate((sa, sb)):
            ms = _proj_pass(lm, cgu_ref.at[w + m], 1, sm, pc)
            for n in range(7):
                for ii, ji in blocks:
                    mb_ref[m, n, ii, ji] = ms[n][ii][ji]
        pc.flush()
        return carry

    lax.fori_loop(0, 8, epi, 0)
    pc.add(_build_steps(*held, 0, 1, rb), 1)
    pc.flush()

    def cp_last(io, a):
        it, rows = NA - LAG + a, pl.ds(288 * io, 288)
        return pltpu.make_async_copy(ob_ref.at[it, rows], o_hbm.at[rows, pl.ds(it * TA, TA)],
                                     sem_out.at[it + LAG * io])

    def put(io, a, v):
        ob_ref[NA - LAG + a, 288 * io:288 * io + 288, :] = v.astype(bf16)

    def mid(k):
        if k == 6:
            cp_last(1, 0).start()
            cp_last(0, 1).start()

    _ffn_down(last, lambda p: cd_ref.at[8][unit(p, 72)], lambda p: rb[p, :, :128], None, pc, x_ref, mid, put)
    cp_last(1, 1).start()
    cp_last(0, 0).start()
    for it in range(NA - LAG):
        cp_out(it).wait()
    for io, a in blocks:
        cp_last(io, a).wait()


@jax.jit
def pallas_interleave_layers__sliding_local_dilated__glu_gated_bilinear__prompt_kernel(
    A_x, A_wqkv, A_wo, B_x, B_w_gate, B_w_up, B_w_down):
    xt = A_x[0].T
    wdt = B_w_down.T
    hbm = pl.BlockSpec(memory_space=pl.ANY)
    out_t = pl.pallas_call(
        _kernel,
        in_specs=[hbm] * 6,
        out_specs=hbm,
        out_shape=jax.ShapeDtypeStruct((D, S), bf16),
        scratch_shapes=[
            pltpu.VMEM((D, S), bf16),
            pltpu.VMEM((D, 3 * D), bf16),
            pltpu.VMEM((D, D), bf16),
            pltpu.VMEM((D, FH), bf16),
            pltpu.VMEM((D, FH), bf16),
            pltpu.VMEM((D, FH), bf16),
            pltpu.VMEM((D, 512), bf16),
            pltpu.VMEM((18, 54 * 32, 256), u32),
            pltpu.VMEM((9, 25 * 72 + 8, 256), u32),
            pltpu.VMEM((2, 4 * 144, 256), u32),
            pltpu.VMEM((D // 2, NQ), u32),
            pltpu.VMEM((672, NH), u32),
            pltpu.VMEM((1, 16 * 72, 256), u32),
            pltpu.VMEM((3, 3 * D, 128), u32),
            pltpu.VMEM((5, D // 2, 128), u32),
            pltpu.VMEM((NA, D, TA), f32),
            pltpu.VMEM((2, LAG, 57 * 16, 256), u32),
            pltpu.VMEM((1, 53, 64, 512), u32),
            pltpu.VMEM((2, 7, 2, 2, 64, 128), f32),
            pltpu.VMEM((LAG, 512, 256), u32),
            pltpu.VMEM((LAG, 11 * 64, 256), u32),
            pltpu.VMEM((NA, D, TA), bf16),
            pltpu.VMEM((14, QROWS, 128), f32),
            pltpu.SMEM((1,), i32),
            pltpu.SemaphoreType.DMA((6,)),
            pltpu.SemaphoreType.DMA((4 * LAG,)),
            pltpu.SemaphoreType.DMA((NA + LAG,)),
        ],
        compiler_params=pltpu.CompilerParams(vmem_limit_bytes=116 * 1024 * 1024),
    )(xt, A_wqkv, A_wo, B_w_gate, B_w_up, wdt)
    return out_t.T[None]
```

```python
import functools
import math

import jax
import jax.numpy as jnp
from jax import lax
import jax.experimental.pallas as pl
import jax.experimental.pallas.tpu as pltpu

S, D, F = 2048, 576, 4608
H, DH, W, DIL = 32, 18, 8, 2
NQ = 14 * 128
NH = NQ // 2
HALO = 16
QROWS = S + 2 * HALO + 8
TA = 256
TF = 512
FH = F // 2
LAG = TF // TA
EVERY = (3, 4, 2, 4, 2, 4, 2)
KPOST, DPOST, DLHS = 5, 1, 30
SUB, ELN, EPOST = 3, 1, 2
C1, C2 = (6, 7), 3
EREM = 5
ED = 2
EV1 = (4, 4, 2, 4, 3, 4, 3)
CL = 0
L1 = (8, (3,) * 6 + (8,) * 5 + (1, 1, 1, 1))
EE = (3, 4, 2, 4, 2, 4, 2)
EF = (3, 4, 2, 3, 2, 4, 2)
HD = (22, 6, 1, 0)
LEAD = 2
NCH = 2
RB = 16
NA = S // TA
NSTEP = 2 * NA
EPS = 1e-5
bf16, f32, u32, i32 = jnp.bfloat16, jnp.float32, jnp.uint32, jnp.int32
NT = (((1,), (1,)), ((), ()))
SCALE = DH ** -0.5
EXP2_C = SCALE * math.log2(math.e)
NEG = -1e9 / SCALE

ORD = (0, 2, 3, 1, 4, 5, 6)
SPEC = {1: (1, (0,)), 4: (0, (1,)), 5: (1, (0, 1)), 6: (0, (0, 1))}
SETS = ((0,), (1,), (0, 1))
QSUM = (0, 2, 3, 5, 6)
SIDX = {n: k for k, n in enumerate(SPEC)}

dot = functools.partial(jnp.dot, preferred_element_type=f32)


def dnt(a, b):
    return lax.dot_general(a, b, NT, preferred_element_type=f32)


def cat0(*xs):
    return xs[0] if len(xs) == 1 else jnp.concatenate(xs, axis=0)


def cat1(*xs):
    return xs[0] if len(xs) == 1 else jnp.concatenate(xs, axis=1)


def tb(x):
    return x.T.astype(bf16)


def pkb(x):
    return pltpu.bitcast(x.astype(bf16), u32)


def pkt(x):
    return pltpu.bitcast(tb(x), u32)


def up(x):
    return pltpu.bitcast(x, bf16)


def _chain_sum(load, fn):
    acc = None
    for r in range(0, D, 8 * NCH):
        t = fn(load(r, 8 * NCH))
        acc = t if acc is None else acc + t
    return jnp.sum(acc, axis=0, keepdims=True)


def _ln_t(load, m=None):
    if m is None:
        m = _chain_sum(load, lambda v: v) * (1.0 / D)
    r = lax.rsqrt(_chain_sum(load, lambda v: (v - m) * (v - m)) * (1.0 / D) + EPS)
    return load(0, D) * r - m * r


def _ln_steps(load, m, out):
    st = {}

    def wide(gate, v):
        v = jnp.broadcast_to(v, (16, TA))
        return cat1(gate(v[:, :128]), gate(v[:, 128:]))

    def var(r0, gate):
        mg = wide(gate, m)
        for r in range(r0, r0 + 96, 16):
            d = load(r, 16) - mg
            st["acc"] = d * d if r == 0 else st["acc"] + d * d

    def norm(c, gate):
        if c == 0:
            st["r"] = lax.rsqrt(jnp.sum(st["acc"], axis=0, keepdims=True) * (1.0 / D) + EPS)
            st["mr"] = jnp.broadcast_to(m * st["r"], (16, TA))
        rg = wide(gate, st["r"])
        z = [load(r, 16) * rg - st["mr"] for r in range(128 * c, min(128 * c + 128, D), 16)]
        out[c] = cat0(*(z if c < 4 else z + z)).T

    return [functools.partial(var, r) for r in range(0, D, 96)] + [functools.partial(norm, c) for c in range(5)]


def _prep_wqkv(c, wqkv_ref, wq_ref, cq_ref, t1_ref):
    n = min(256, D - 256 * c)
    wp = pltpu.bitcast(wqkv_ref[256 * c:256 * c + n, :], u32)
    if n < 256:
        wp = cat0(wp, jnp.zeros(((256 - n) // 2, 3 * D), u32))
    t1_ref[c] = wp.T

    def rows(t, d):
        return t1_ref[c, pl.ds(t * D + d, H, stride=DH), :]

    parts = []
    for t in range(3):
        parts += [rows(t, d) for d in (0, 2, 4, 6, 1, 3, 5, 7, 8, 10, 12, 14, 9, 11, 13, 15)]
    parts += [rows(0, 16), rows(0, 17), rows(2, 16), rows(2, 17)]
    parts += [rows(1, 16), rows(1, 17), jnp.zeros((32, 128), u32), jnp.zeros((32, 128), u32)]
    for t in range(7):
        w = [cat0(*parts[4 * k:4 * k + 4]).T[:n // 2] for k in (t, t + 7)]
        for k, v in zip((t, t + 7), w):
            wq_ref[128 * c:128 * c + n // 2, 128 * k:128 * k + 128] = v
        cols = slice(128 * t, 128 * t + 128)
        if c == 2:
            cq_ref[640:, cols] = pkb(unp(w[0]) + unp(w[1]))
        if c == 1:
            for r in range(0, 128, 8):
                ops = rhs7(*[unp(wq_ref[r:r + 8, 128 * k:128 * k + 128]) for k in (t, t + 7)],
                           *[unp(v[r:r + 8]) for v in w])
                for k, m in enumerate(QSUM):
                    cq_ref[128 * k + r:128 * k + r + 8, cols] = pkb(ops[m]())


def _share_lhs(load, rows, dst):
    lo = lax.broadcasted_iota(i32, (16, 128), 1) < 64

    def step(r, gate):
        blk = [[load(q, i, r, gate) for i in range(2)] for q in range(2)]
        for c in range(2):
            ops = [lhs7(b[0][c], b[0][2 + c], b[1][c], b[1][2 + c]) for b in blk]
            for n in range(7):
                x1, x2 = ops[0][n](), ops[1][n]()
                if c == 1 and n in SPEC:
                    r1, r2 = blk[0][SPEC[n][0]][4], blk[1][SPEC[n][0]][4]
                    dst[unit(28 + SIDX[n], rows, r // 2, 8)] = pkb(jnp.where(lo, r1, x2))
                    x1, x2 = jnp.where(lo, x1, x1 - x2), jnp.where(lo, x2, r2 - r1)
                dst[unit(4 * n + c, rows, r // 2, 8)] = pkb(x1)
                dst[unit(4 * n + 2 + c, rows, r // 2, 8)] = pkb(x2)
        return x1

    return [functools.partial(step, r) for r in range(0, 2 * rows, 16)]


def _prep_wo(wo_ref, cw_ref, t2_ref):
    wo = cat1(pltpu.bitcast(wo_ref[...], u32), jnp.zeros((D // 2, 64), u32))
    for c in range(5):
        t2_ref[c] = wo[:, c * 128:(c + 1) * 128]
    wt = []
    for c in range(5):
        wt.append(cat0(*[t2_ref[c, pl.ds(p, H, stride=DH // 2), :] for p in tuple(range(8)) + (8,) * 4]).T)
    wt = cat0(*wt)
    odd = lax.broadcasted_iota(i32, (16, 128), 1) % 64 >= 32

    def load(q, i, r, gate):
        o = 288 * i + 144 * q + r
        out = []
        for c in range(3):
            w = gate(wt[o:o + 16, 128 * c:128 * c + 128])
            out += [pltpu.bitcast(w << 16, f32), pltpu.bitcast(w & jnp.uint32(0xFFFF0000), f32)]
        return out[:4] + [jnp.where(odd, out[5], out[4])]

    return _share_lhs(load, 72, cw_ref)


def _base(s):
    return s % NA * TA if isinstance(s, int) else pl.multiple_of((s % NA) * TA, TA)


def _attn_lhs(s, x_ref, pa):
    item = s % NA
    z = _ln_t(lambda r, n: x_ref[item, r:r + n, :])
    zt = cat0(z, z[512:]).T

    def load(q, i, r, gate):
        o = 128 * q + 64 * i + r
        return [zt[o:o + 16, 128 * c:128 * c + 128] for c in range(5)]

    for st in _share_lhs(load, 32, pa):
        st(None)


def _attn_lhs_steps(s, x_ref, pa):
    item, zt = s % NA, {}
    rows = lambda r, n: x_ref[item, r:r + n, :]

    def load(q, i, r, gate):
        o = 128 * q + 64 * i + r
        return [zt[c][o:o + 16] for c in range(5)]

    return _ln_steps(rows, _chain_sum(rows, lambda v: v) * (1.0 / D), zt) + _share_lhs(load, 32, pa)


def _attn_proj(s, q, sh, pc, pa, wq_ref, cq_ref, qkv_ref):
    item = s % NA
    t0 = _base(s)
    lo = lax.broadcasted_iota(i32, (64, 128), 1) < 64
    for t in range(7):
        def wts(n, r, k):
            c = 128 * t
            if n in QSUM:
                return cq_ref[128 * QSUM.index(n) + r:128 * QSUM.index(n) + r + k, c:c + 128]
            return wq_ref[r:r + k, c:c + 128] if n == 1 else wq_ref[128 + r:128 + r + k, NH + c:NH + c + 128]

        def wrem(n):
            c = 128 * t + (NH if n == 4 else 0)
            return (wq_ref[256:, c:c + 128] if n in (1, 4) else cq_ref[640:, c:c + 128])

        p = [None] * 7
        for n in ORD:
            x = pc.pre(pa[64 * n + 32 * q:64 * n + 32 * q + 32, :])
            if n in SPEC:
                if q == 0:
                    sh[t, n] = dot(up(pa[unit(28 + SIDX[n], 32)]), up(cat0(wrem(n), wts(n, 96, 32))))
                w = cat0(wts(n, 0, 96), wrem(n)) if q else wts(n, 0, 128)
                p[n] = dot(up(x), up(w)) + sh[t, n]
            else:
                p[n] = dot(up(x), up(wts(n, 0, 128)))
            pc.tick(p[n])
        y = out4(p)
        for i in range(2):
            for j in range(2):
                c, v = t + 7 * j, y[i][j]
                if c == 13:
                    v = jnp.where(lo, v, 0.0)
                qkv_ref[c, pl.ds(t0 + (HALO + 128 * q + 64 * i), 64), :] = v
                if q == 0 and i == 0 and c >= 4 and not (isinstance(s, int) and s):
                    hrow = 0 if isinstance(s, int) else pl.multiple_of(jnp.where(item == 0, 0, S + HALO), HALO)
                    qkv_ref[c, pl.ds(hrow, HALO), :] = jnp.broadcast_to(v[0:1], (HALO, 128))


def _attn_core(s, b, qkv_ref, gate):
    t0 = _base(s)
    qi = (0, 1, 2, 3, 12)
    ki = (4, 5, 6, 7, 13)
    vi = (8, 9, 10, 11, 12)
    r0 = t0 + (b * RB + HALO)
    q = [cat0(*[gate(qkv_ref[c, pl.ds(r0 + r, 16), :]) for r in range(0, RB, 16)]) for c in qi]
    ls = []
    for w in range(W):
        acc = None
        for c in range(5):
            t = q[c] * qkv_ref[ki[c], pl.ds(r0 - DIL * w, RB), :]
            acc = t if acc is None else acc + t
        acc = acc + pltpu.roll(acc, 64, 1)
        acc = acc + pltpu.roll(acc, 32, 1)
        if w > 0 and b == 0 and not (isinstance(s, int) and s):
            pos = t0 + lax.broadcasted_iota(i32, (HALO, 128), 0)
            top = jnp.where(pos >= DIL * w, acc[:HALO], NEG)
            acc = top if RB == HALO else cat0(top, acc[HALO:])
        ls.append(acc)
    m = functools.reduce(jnp.maximum, ls)
    pr = [jnp.exp2((l - m) * EXP2_C) for l in ls]
    inv = 1.0 / functools.reduce(jnp.add, pr)
    out = []
    for c in range(5):
        acc = None
        for w in range(W):
            t = pr[w] * qkv_ref[vi[c], pl.ds(r0 - DIL * w, RB), :]
            acc = t if acc is None else acc + t
        out.append(acc * inv)
    return out


def _attn_rhs(b, a0, a1, at):
    lo = lax.broadcasted_iota(i32, (RB, 128), 1) < 64
    rem = (a0[4], a1[4], a0[4] + a1[4])
    rem = [(r, pltpu.roll(r, 64, 1)) for r in rem]
    for c in range(2):
        ops = rhs7(a0[c], a1[c], a0[2 + c], a1[2 + c])
        for n in range(7):
            v = ops[n]()
            at[unit(2 * n + c, 64, b * RB // 2, RB // 2)] = pkb(v)
            if c == 1 and n in SPEC:
                hi, low = rem[SETS.index(SPEC[n][1])]
                at[unit(14 + 2 * SIDX[n], 64, b * RB // 2, RB // 2)] = pkb(jnp.where(lo, v, hi))
                at[unit(15 + 2 * SIDX[n], 64, b * RB // 2, RB // 2)] = pkb(jnp.where(lo, low, v))


def lhs7(a11, a12, a21, a22):
    return (lambda: a11 + a22, lambda: a21 + a22, lambda: a11, lambda: a22,
            lambda: a11 + a12, lambda: a21 - a11, lambda: a12 - a22)


def rhs7(b11, b12, b21, b22):
    return (lambda: b11 + b22, lambda: b11, lambda: b12 - b22, lambda: b21 - b11,
            lambda: b22, lambda: b11 + b12, lambda: b21 + b22)


def out4(m):
    m1, m2, m3, m4, m5, m6, m7 = m
    return [[m1 + m4 - m5 + m7, m3 + m5], [m2 + m4, m1 + m3 - m2 + m6]]


def unit(u, rows, off=0, n=None):
    off = rows * (u // 2) + off
    n = rows if n is None else n
    r = slice(off, off + n) if isinstance(off, int) else pl.ds(pl.multiple_of(off, 8), n)
    return r, slice(128 * (u % 2), 128 * (u % 2) + 128)


def _attn_post(s, pc, at, x_ref, cw_ref, lm_ref):
    item = s % NA
    sh, y = {}, []
    for q in range(2):
        p = [None] * 7
        for n in ORD:
            w = up(cw_ref[144 * n + 72 * q:144 * n + 72 * q + 72, :])
            if n in SPEC:
                if q == 0:
                    sh[n] = dnt(up(cw_ref[unit(28 + SIDX[n], 72)]), up(at[unit(15 + 2 * SIDX[n], 64)]))
                last = at[unit(14 + 2 * SIDX[n] if q else 2 * n + 1, 64)]
                p[n] = dnt(w, up(cat1(at[unit(2 * n, 64)], last))) + sh[n]
            else:
                p[n] = dnt(w, up(at[64 * n:64 * n + 64, :]))
            pc.tick(p[n])
        y.append(out4(p))
    xt = x_ref[item] + cat0(*[cat1(*y[q][i]) for i in range(2) for q in range(2)])
    x_ref[item] = xt
    m = _chain_sum(lambda r, n: xt[r:r + n], lambda v: v) * (1.0 / D)
    zt = {}
    dst = lm_ref.at[(s // LAG) % 2, s % LAG]
    lo = lax.broadcasted_iota(i32, (16, 128), 1) < 64

    def step(r, n, gate):
        def blk(q, i, k):
            o = 64 * i + 32 * q + r
            return zt[k][o:o + 16]

        g11, g22 = (gate, lambda v: v) if n in (0, 2, 4, 5) else (lambda v: v, gate)
        inner = [lhs7(*[lhs7(g11(blk(q, i, k)), blk(q, i, 2 + k), blk(q, 2 + i, k), g22(blk(q, 2 + i, 2 + k)))[n]()
                        for i in range(2) for k in range(2)]) for q in range(2)]
        for l in range(7):
            x1, x2 = inner[0][l](), inner[1][l]()
            if n in SPEC and l in SPEC:
                i = 2 * SPEC[n][0] + SPEC[l][0]
                r1, r2 = blk(0, i, 4), blk(1, i, 4)
                dst[unit(98 + 4 * SIDX[n] + SIDX[l], 16, r // 2, 8)] = pkb(jnp.where(lo, r1, x2))
                x1, x2 = jnp.where(lo, x1, x1 - x2), jnp.where(lo, x2, r2 - r1)
            dst[unit(2 * (7 * n + l), 16, r // 2, 8)] = pkb(x1)
            dst[unit(2 * (7 * n + l) + 1, 16, r // 2, 8)] = pkb(x2)
        return x1

    return (_ln_steps(lambda r, n: x_ref[item, r:r + n, :], m, zt),
            [functools.partial(step, r, n) for r in (0, 16) for n in range(7)])


class Pacer:
    def __init__(self, live):
        self.live, self.todo, self.wait, self.due, self.sub, self.done = live, [], 0, [], 1, []

    def add(self, steps, every, delay=0, lag=0):
        if not self.todo:
            self.wait = delay
        every = every if isinstance(every, tuple) else (every,)
        self.todo += [(st, every[k % len(every)], lag) for k, st in enumerate(steps)]

    def run(self, toks):
        st, self.wait, lag = self.todo.pop(0)
        if lag and len(self.done) >= lag and self.done[-lag] is not None:
            toks = toks + [self.done[-lag]]

        def gate(v):
            if v is None:
                return toks[0]
            for t in toks:
                v = jnp.where(self.live, v, t if v.dtype == t.dtype else pltpu.bitcast(t, v.dtype))
            return v

        self.done.append(st(gate))

    def tick(self, p):
        for k in range(self.sub):
            self.wait -= 1
            if self.todo and self.wait <= 0:
                o = p.shape[0] // self.sub * k
                self.run([p[o:o + 16, :128]])

    def by(self, count, load):
        self.due.append([count, load()])

    def pre(self, w):
        for d in self.due:
            d[0] -= 1
        while self.due and self.due[0][0] <= 0:
            v = jnp.where(self.live[:8], w[:8, :128], self.due.pop(0)[1])
            w = cat0(cat1(v, w[:8, 128:]) if w.shape[1] > 128 else v, w[8:])
        return w

    def flush(self):
        while self.todo:
            self.run([])


def wunit(p, part, off=0, n=32):
    if part == 2:
        p, part = (49, p) if p < 2 else (50 + p % 2, p // 2 - 1)
    return unit(p, 64, 32 * part + off, n)


def _row(ref, r, c, n):
    c = 128 * c if isinstance(c, int) else pl.multiple_of(128 * c, 128)
    r = r if isinstance(r, int) else pl.multiple_of(r, 16)
    v = pltpu.bitcast(ref[pl.ds(r, 16), pl.ds(c, 128 * n)], u32)
    return [v[:, 128 * k:128 * k + 128] for k in range(n)]


def unp(v):
    return up(v).astype(f32)


class Chain:
    def __init__(self, live):
        self.live, self.tok = live, None

    def stage(self, blocks, emit, lead=LEAD):
        tok, self.tok = self.tok, None
        for k, (idx, v) in enumerate(emit([unp(v if tok is None else jnp.where(self.live, v, tok)) for v in blocks])):
            v = pkb(v)
            idx[0][idx[1]] = v
            if k <= lead:
                self.tok = v

    def two_level(self, fn, blk, where):
        quad = lambda a, b: [blk[2 * a + i][2 * b + j] for i in range(2) for j in range(2)]
        got = {}

        def emit(keys, ns, vals):
            for k, key in enumerate(keys):
                got[key] = vals[4 * k:4 * k + 4]
            for n in ns:
                q = [got.get(c, (None,) * 4) for c in ((0, 0), (0, 1), (1, 0), (1, 1))]
                inner = fn(*[fn(*[c[x] for c in q])[n]() for x in range(4)])
                for l in range(7):
                    yield where(7 * n + l), inner[l]()

        plan = ((1, 4, 0), (5, 2), (3, 6)) if fn is rhs7 else ((2, 3, 0), (4, 6), (1, 5))
        return [functools.partial(self.stage, sum((quad(*k) for k in keys), []), functools.partial(emit, keys, ns))
                for keys, ns in zip((((0, 0), (1, 1)), ((0, 1),), ((1, 0),)), plan)]


def _shift(ref, off, most):
    return ref.at[pl.ds(off if isinstance(off, int) else pl.multiple_of(off, 8), ref.shape[0] - most)]


def _combine_proj(half, live, wg_ref, wu_ref, c_ref):
    lo = lax.broadcasted_iota(i32, (8, 128), 1) < 64

    def row(r, tile):
        if tile < 8:
            return _row((wg_ref, wu_ref)[tile % 2], r, 4 * (tile // 2), 4)
        out = []
        for g, u in zip(_row(wg_ref, r, 16, 2), _row(wu_ref, r, 16, 2)):
            w = pltpu.roll(jnp.where(lo, u, g), 64, 1)
            out += [jnp.where(lo, g, w), jnp.where(lo, w, u)]
        return out

    def body(j, carry):
        ch = Chain(live)
        for tile in (0, 8, 1, 2, 3, 4, 5, 6, 7):
            dst = _shift(c_ref.at[half * 9 + tile], 8 * j, 24)

            def emit(r):
                for a, (x, y) in enumerate(((r[0], r[1]), (r[2], r[3]), (r[0] + r[2], r[1] + r[3]))):
                    for b, v in enumerate((x, y, x + y)):
                        yield (dst, wunit(3 * a + b, 2, 0, 8)), v

            for part in range(2):
                blk = [row(128 * k + 64 * part + 16 * j, tile) for k in range(4)]
                for st in ch.two_level(rhs7, blk, lambda p: (dst, wunit(p, part, 0, 8))):
                    st()
            ch.stage(row(512 + 16 * j, tile), emit, 0)
        return carry

    lax.fori_loop(0, 4, body, 0)


def _down_unit(ch, j, w_ref, c, dst):
    dst = _shift(dst, 8 * j, 64)
    blk = [_row(w_ref, 144 * k + 16 * j, c, 4) for k in range(4)]
    return ch.two_level(lhs7, blk, lambda p: (dst, unit(p, 72, 0, 8)))


def _combine_down(half, live, wdt_ref, cd_ref, cr_ref):
    def body(j, carry):
        ch = Chain(live)
        for t in range(4):
            for st in _down_unit(ch, j, wdt_ref, 4 * t, cd_ref.at[1 + half * 4 + t]):
                st()
        dst = _shift(cr_ref.at[half], 8 * j, 64)
        for c in range(2):
            r = 144 * c + 16 * j
            ch.stage(_row(wdt_ref, r, 16, 2) + _row(wdt_ref, 288 + r, 16, 2),
                     lambda a: [((dst, unit(n, 144, 72 * c, 8)), lhs7(*a)[n]()) for n in range(7)])
        return carry

    lax.fori_loop(0, 9, body, 0)


def _proj_pass(lm, w, q, sh, pc):
    def lhs(u):
        return up(pc.pre(cat0(*[lm.at[a][unit(u, 16)] for a in range(LAG)])))

    def wts(a, b):
        return up(cat0(w[wunit(*a)], w[wunit(*b)]))

    def prod(n, l):
        p = 7 * n + l
        if n in SPEC and l in SPEC:
            wr = (3 * SETS.index(SPEC[n][1]) + SETS.index(SPEC[l][1]), 2)
            if q == 0:
                sh[p] = dot(lhs(98 + 4 * SIDX[n] + SIDX[l]), wts(wr, (p, 1)))
            return dot(lhs(2 * p + q), wts((p, 0), wr if q else (p, 1))) + sh[p]
        return dot(lhs(2 * p + q), wts((p, 0), (p, 1)))

    ms = [None] * 7
    for n in ORD:
        p = [None] * 7
        for l in ORD:
            p[l] = prod(n, l)
            pc.tick(p[l])
        ms[n] = out4(p)
    return ms


def _col(ms, ii, ji, jo, rows, gate):
    m1, m2, m3, m4, m5, m6, m7 = [m[ii][ji][rows] for m in ms]
    if jo == 0:
        a = gate(m4)
        return a + m1 - m5 + m7, a + m2
    a = gate(m3)
    return a + m5, a + m1 - m2 + m6


def _mix(a, b):
    lo = lax.broadcasted_iota(i32, a.shape, 1) < 64
    return jnp.where(lo, a, b) * pltpu.roll(jnp.where(lo, b, a), 64, 1)


def _build_steps(mg, mu, t, q, rb, merged=False):
    def form(e, r, blk, k, gate):
        rows = slice(32 * k[1] + r, 32 * k[1] + r + 16)
        blk[k] = []
        for ki in range(2):
            if merged:
                a, b = [_col((mg, mu)[k[0]], e, ji, ki, rows, gate) for ji in range(2)]
                blk[k] += [_mix(a[0], b[0]), _mix(a[1], b[1])]
            else:
                g, u = _col(mg, e, ki, k[0], rows, gate), _col(mu, e, ki, k[0], rows, gate)
                blk[k] += [g[0] * u[0], g[1] * u[1]]

    def emit(e, r, blk, k, n, gate):
        o = 32 * e + 16 * q + r // 2
        quad = [[gate(v) for v in blk[c]] if c == k else blk.get(c, (None,) * 4)
                for c in ((0, 0), (0, 1), (1, 0), (1, 1))]
        inner = rhs7(*[rhs7(*[c[x] for c in quad])[n]() for x in range(4)])
        for l in range(7):
            rb.at[7 * n + l][o:o + 8, 128 * t:128 * t + 128] = pkb(inner[l]())

    def both(e, r, blk, k, n, gate):
        form(e, r, blk, k, gate)
        emit(e, r, blk, k, n, lambda v: v)

    steps = []
    for e in range(2):
        for r in (0, 16):
            blk = {}
            for k, ns in (((0, 0), (1,)), ((1, 1), (4, 0)), ((0, 1), (5, 2)), ((1, 0), (3, 6))):
                steps.append(functools.partial(both, e, r, blk, k, ns[0]))
                steps += [functools.partial(emit, e, r, blk, k, n) for n in ns[1:]]
    return steps


def _rem_steps(ms, q, rb):
    def step(ii, r, gate):
        h = []
        for jo in range(2):
            for item in range(2):
                rows = slice(32 * item + r, 32 * item + r + 16)
                a, b = [_col(ms, ii, ji, jo, rows, gate) for ji in range(2)]
                h.append([_mix(a[io], b[io]) for io in range(2)])
        for io in range(2):
            ops = rhs7(*[v[io] for v in h])
            for n in range(7):
                o, cc = 32 * ii + 16 * q + r // 2, 256 * (n % 2) + 128 * io
                rb.at[49 + n // 2][o:o + 8, cc:cc + 128] = pkb(ops[n]())

    return [functools.partial(step, ii, r) for ii in range(2) for r in (0, 16)]


def _ffn_pos(lm, wa, wb, t, pc, rb):
    sa, sb = {}, {}
    for q in range(2):
        g = _proj_pass(lm, wa, q, sa, pc)
        u = _proj_pass(lm, wb, q, sb, pc)
        pc.add(_build_steps(g, u, t, q, rb), (EVERY, EV1)[q], ED)


def _ffn_down(tile, wts, rhs, rem, pc, x_ref, mid=lambda k: None, put=None):
    ms = [None] * 7

    def rdot(n):
        r = dnt(*rem(n))
        pc.tick(r)
        return r

    def group(n, base):
        if rem and n != ORD[0]:
            base = rdot(n) if base is None else base + rdot(n)
        p = [None] * 7
        for l in ORD:
            p[l] = dnt(up(pc.pre(wts(7 * n + l))), up(rhs(7 * n + l)))
            pc.tick(p[l])
        m1, m2, m3, m4, m5, m6, m7 = p
        if base is None:
            m = out4(p)
        else:
            b = [[base[144 * i:144 * i + 144, 128 * j:128 * j + 128] for j in range(2)] for i in range(2)]
            m = [[b[0][0] + m1 + m4 - m5 + m7, b[0][1] + m3 + m5],
                 [b[1][0] + m4 + m2, b[1][1] + m1 + m3 - m2 + m6]]
        base = cat0(cat1(*m[0]), cat1(*m[1]))
        if rem and n == ORD[0]:
            base = base + rdot(n)
        return base

    def xs(io, a):
        return x_ref.at[tile * LAG + a, 288 * io:288 * io + 288, :]

    def keep(io, a, v):
        xs(io, a)[...] = v

    put = put or keep
    for k, n in enumerate(ORD):
        mid(k)
        if n == 5:
            put(1, 1, group(n, xs(1, 1)[...] + ms[0] + ms[2] - ms[1]))
        elif n == 6:
            put(0, 0, group(n, xs(0, 0)[...] + ms[0] + ms[3] - ms[4]))
        else:
            ms[n] = group(n, None)
            if n == 1:
                put(1, 0, xs(1, 0)[...] + ms[3] + ms[1])
            elif n == 4:
                put(0, 1, xs(0, 1)[...] + ms[2] + ms[4])
    pc.flush()


def _kernel(xt_hbm, wqkv_hbm, wo_hbm, wg_hbm, wu_hbm, wdt_hbm, o_hbm,
            xb_ref, wqkv_ref, wo_ref, wg_ref, wu_ref, wdt_ref, wm_ref,
            cgu_ref, cd_ref, cr_ref, wq_ref, cq_ref, cw_ref, t1_ref, t2_ref, x_ref,
            lm_ref, rb_ref, mb_ref, pa_ref, at_ref, ob_ref, qkv_ref, one_ref, sem_in, sem_w, sem_out):
    def cp_wqkv(c):
        rows = pl.ds(256 * c, min(256, D - 256 * c))
        return pltpu.make_async_copy(wqkv_hbm.at[rows], wqkv_ref.at[rows], sem_in.at[c])

    cp_x0 = pltpu.make_async_copy(xt_hbm.at[:, pl.ds(0, TF)], xb_ref.at[:, pl.ds(0, TF)], sem_in.at[3])
    cp_wo = pltpu.make_async_copy(wo_hbm, wo_ref, sem_in.at[4])
    cp_x1 = pltpu.make_async_copy(xt_hbm.at[:, pl.ds(TF, S - TF)], xb_ref.at[:, pl.ds(TF, S - TF)], sem_in.at[5])

    def cp_w(half, n):
        src, dst = ((wg_hbm, wg_ref), (wu_hbm, wu_ref), (wdt_hbm, wdt_ref))[n]
        return pltpu.make_async_copy(src.at[:, pl.ds(half * FH, FH)], dst, sem_w.at[half * 3 + n])

    def cp_m(half):
        return pltpu.make_async_copy(wdt_hbm.at[:, pl.ds(half * FH + 2048, 256)],
                                     wm_ref.at[:, pl.ds(half * 256, 256)], sem_w.at[3 * LAG + half])

    def cp_out(it):
        o = it * TA
        sl = pl.ds(o if isinstance(o, int) else pl.multiple_of(o, TA), TA)
        return pltpu.make_async_copy(ob_ref.at[it], o_hbm.at[:, sl], sem_out.at[it])

    def flags():
        one = one_ref[0]
        return Pacer(jnp.full((16, 128), one, i32) > 0), one - 1

    nb = TA // 2 // RB

    def cores(s, att, at, blocks):
        def step(b, gate):
            att[b] = _attn_core(s, b, qkv_ref, gate)
            if b >= nb:
                _attn_rhs(b - nb, att[b - nb], att[b], at)
            return att[b][0]
        return [functools.partial(step, b) for b in blocks]

    def first():
        for a in range(LAG):
            x_ref[a] = xb_ref[:, a * TA:(a + 1) * TA].astype(f32)
            _attn_lhs(a, x_ref, pa_ref.at[a])

    cp_wqkv(2).start()
    cp_x0.start()
    cp_wqkv(0).start()
    one_ref[0] = 1
    for m, n in [(0, 0), (0, 1), (0, 4)] + [(1, n) for n in range(7)]:
        mb_ref[m, n] = jnp.full((2, 2, 64, 128), 1.0 if m and n in (2, 3) else 0.0, f32)
    cp_wqkv(2).wait()
    _prep_wqkv(2, wqkv_ref, wq_ref, cq_ref, t1_ref)
    cp_x0.wait()
    cp_wqkv(1).start()
    first()
    cp_wqkv(0).wait()
    cp_wo.start()
    _prep_wqkv(0, wqkv_ref, wq_ref, cq_ref, t1_ref)
    cp_wqkv(1).wait()
    cp_w(0, 0).start()
    _prep_wqkv(1, wqkv_ref, wq_ref, cq_ref, t1_ref)
    cp_wo.wait()
    for n in range(1, 3):
        cp_w(0, n).start()

    def head():
        pc, z = flags()
        sh, att = ({}, {}), ({}, {})
        pc.add(_prep_wo(wo_ref, cw_ref.at[0], t2_ref), 3, HD[0])
        for a in range(LAG):
            for q in range(2):
                _attn_proj(a, q, sh[a], pc, pa_ref.at[a], wq_ref, cq_ref, qkv_ref)
                last = a == 1 and q == 1
                pc.flush()
                pc.add(cores(a, att[a], at_ref.at[a], range(q * nb, (q + 1) * nb)), HD[2] if last else HD[1], 1,
                       HD[3] if a else 0)
        ln, build = _attn_post(0, pc, at_ref.at[0], x_ref, cw_ref.at[z], lm_ref)
        pc.flush()
        pc.sub = SUB
        pc.add(ln, 1)
        pc.add(build, 2, lag=2)
        ln, build = _attn_post(1, pc, at_ref.at[1], x_ref, cw_ref.at[z], lm_ref)
        pc.add(ln, 1)
        pc.add(build, 1, lag=2)
        pc.flush()

    head()
    cp_x1.start()

    def wait_w(f, ns):
        for half in range(LAG):
            @pl.when(f == half)
            def _():
                for n in ns:
                    cp_w(half, n).wait()

    def wait_weights(f):
        @pl.when(f < LAG)
        def _():
            live = jnp.full((8, 128), one_ref[0], i32) > 0
            wait_w(f, (0, 1))
            _combine_proj(f, live, wg_ref, wu_ref, cgu_ref)
            wait_w(f, (2,))
            _combine_down(f, live, wdt_ref, cd_ref, cr_ref)

        @pl.when(f == 0)
        def _():
            cp_x1.wait()
            for n in range(3):
                cp_w(1, n).start()
            for half in range(LAG):
                cp_m(half).start()

            def conv(a, carry):
                x_ref[a] = xb_ref[:, pl.ds(pl.multiple_of(a * TA, TA), TA)].astype(f32)
                return carry

            lax.fori_loop(LAG, NA, conv, 0)

    def emit(it):
        ob_ref[it] = x_ref[it].astype(bf16)
        cp_out(it).start()

    def start_out(f):
        @pl.when(jnp.logical_and(f >= NA, f % LAG == LAG - 1))
        def _():
            for a in range(LAG):
                emit(f - NA - (LAG - 1) + a)

    def fused(s, carry):
        f = s - LAG
        wait_weights(f)
        pc, z = flags()
        half = f % LAG
        lm, rb, rbl = lm_ref.at[(f // LAG) % 2], rb_ref.at[0], rb_ref.at[z]
        pc.add(_attn_lhs_steps(s, x_ref, pa_ref.at[0]), L1[1], L1[0])
        pc.add([lambda gate: pc.by(DLHS, lambda: pa_ref[z, :8, :128])], 1)
        for t in range(4):
            _ffn_pos(lm, cgu_ref.at[half * 9 + 2 * t], cgu_ref.at[half * 9 + 2 * t + 1], t, pc, rb)
        sm, sh, att = {}, {}, {}
        for q in range(2):
            pc.add(_rem_steps(_proj_pass(lm, cgu_ref.at[half * 9 + 8], q, sm, pc), q, rb), EREM)
        _attn_proj(s, 0, sh, pc, pa_ref.at[z], wq_ref, cq_ref, qkv_ref)
        pc.flush()
        pc.add(cores(s, att, at_ref.at[0], range(C1[0])), C1[1], 4, CL)
        _attn_proj(s, 1, sh, pc, pa_ref.at[z], wq_ref, cq_ref, qkv_ref)
        pc.flush()
        pc.add(cores(s, att, at_ref.at[0], range(C1[0], 2 * nb)), C2, 1, CL)

        def mid(k):
            if k == KPOST:
                pc.flush()
                ln, build = _attn_post(s, pc, at_ref.at[z], x_ref, cw_ref.at[0], lm_ref)
                pc.sub = SUB
                pc.add(ln, ELN, DPOST)
                pc.add(build, EPOST)

        def rem(n):
            cc = 256 * (n % 2)
            return (up(cr_ref.at[half][unit(n, 144)]),
                    up(cat0(rbl[49 + n // 2, :, cc:cc + 128], rbl[49 + n // 2, :, cc + 128:cc + 256])))

        _ffn_down((f // LAG) % (S // TF),
                  lambda p: cat1(*[cd_ref.at[1 + half * 4 + t][unit(p, 72)] for t in range(4)]),
                  lambda p: rbl[p], rem, pc, x_ref, mid=mid)
        start_out(f)
        return carry

    lax.fori_loop(LAG, NSTEP, fused, 0)

    last, lm, rb = S // TF - 1, lm_ref.at[(NSTEP // LAG - 1) % 2], rb_ref.at[0]
    for half in range(LAG):
        cp_m(half).wait()
    pc, _ = flags()
    ch = Chain(pc.live[:8])

    def ninth(st, gate):
        ch.tok = pltpu.bitcast(gate(None)[:8], u32)
        st()

    blocks = [(ii, ji) for ii in range(2) for ji in range(2)]
    held = [[[[mb_ref.at[m, n, ii, ji] for ji in range(2)] for ii in range(2)] for n in range(7)] for m in range(2)]
    pc.add([functools.partial(ninth, st) for j in range(9) for st in _down_unit(ch, j, wm_ref, 0, cd_ref.at[0])], 3, 4)
    sa, sb = {}, {}
    pc.add(_build_steps(_proj_pass(lm, cgu_ref.at[8], 0, sa, pc), _proj_pass(lm, cgu_ref.at[17], 0, sb, pc),
                        0, 0, rb, True), 2, 2)

    def hold(ms, ko, ii, ki, r, gate):
        a, b = [_col(ms, ii, ji, ki, slice(r, r + 16), gate) for ji in range(2)]
        h = _mix(a[0], b[0]), _mix(a[1], b[1])
        mb_ref[0, 3 - ko, ii, ki, r:r + 16] = h[1 - ko]
        mb_ref[0, 6 - ko, ii, ki, r:r + 16] = h[ko] - h[1 - ko]
        return a[0]

    for ko, sm in enumerate((sa, sb)):
        ms = _proj_pass(lm, cgu_ref.at[8 + 9 * ko], 1, sm, pc)
        pc.add([functools.partial(hold, ms, ko, ii, ki, r) for ii, ki in blocks for r in range(0, 64, 16)], 2, 1, 4 * ko)
    pc.flush()

    def epi(c, carry):
        pc, z = flags()
        w = 2 * c + c // 4
        sa, sb = {}, {}
        pc.add(_build_steps(*held, 0, 1, rb), EE, 2)
        g, u = _proj_pass(lm, cgu_ref.at[w], 0, sa, pc), _proj_pass(lm, cgu_ref.at[w + 1], 0, sb, pc)
        pc.flush()
        _ffn_down(last, lambda p: cd_ref.at[c][unit(p, 72)], lambda p: rb_ref[z, p, :, :128], None, pc, x_ref)
        pc.add(_build_steps(g, u, 0, 0, rb), EF, 2)
        for m, sm in enumerate((sa, sb)):
            ms = _proj_pass(lm, cgu_ref.at[w + m], 1, sm, pc)
            for n in range(7):
                for ii, ji in blocks:
                    mb_ref[m, n, ii, ji] = ms[n][ii][ji]
        pc.flush()
        return carry

    lax.fori_loop(0, 8, epi, 0)
    pc.add(_build_steps(*held, 0, 1, rb), 1)
    pc.flush()

    def cp_last(io, a):
        it, rows = NA - LAG + a, pl.ds(288 * io, 288)
        return pltpu.make_async_copy(ob_ref.at[it, rows], o_hbm.at[rows, pl.ds(it * TA, TA)],
                                     sem_out.at[it + LAG * io])

    def put(io, a, v):
        ob_ref[NA - LAG + a, 288 * io:288 * io + 288, :] = v.astype(bf16)

    def mid(k):
        if k == 6:
            cp_last(1, 0).start()
            cp_last(0, 1).start()

    _ffn_down(last, lambda p: cd_ref.at[8][unit(p, 72)], lambda p: rb[p, :, :128], None, pc, x_ref, mid, put)
    cp_last(1, 1).start()
    cp_last(0, 0).start()
    for it in range(NA - LAG):
        cp_out(it).wait()
    for io, a in blocks:
        cp_last(io, a).wait()


@jax.jit
def pallas_interleave_layers__sliding_local_dilated__glu_gated_bilinear__prompt_kernel(
    A_x, A_wqkv, A_wo, B_x, B_w_gate, B_w_up, B_w_down):
    xt = A_x[0].T
    wdt = B_w_down.T
    hbm = pl.BlockSpec(memory_space=pl.ANY)
    out_t = pl.pallas_call(
        _kernel,
        in_specs=[hbm] * 6,
        out_specs=hbm,
        out_shape=jax.ShapeDtypeStruct((D, S), bf16),
        scratch_shapes=[
            pltpu.VMEM((D, S), bf16),
            pltpu.VMEM((D, 3 * D), bf16),
            pltpu.VMEM((D, D), bf16),
            pltpu.VMEM((D, FH), bf16),
            pltpu.VMEM((D, FH), bf16),
            pltpu.VMEM((D, FH), bf16),
            pltpu.VMEM((D, 512), bf16),
            pltpu.VMEM((18, 54 * 32, 256), u32),
            pltpu.VMEM((9, 25 * 72 + 8, 256), u32),
            pltpu.VMEM((2, 4 * 144, 256), u32),
            pltpu.VMEM((D // 2, NQ), u32),
            pltpu.VMEM((672, NH), u32),
            pltpu.VMEM((1, 16 * 72, 256), u32),
            pltpu.VMEM((3, 3 * D, 128), u32),
            pltpu.VMEM((5, D // 2, 128), u32),
            pltpu.VMEM((NA, D, TA), f32),
            pltpu.VMEM((2, LAG, 57 * 16, 256), u32),
            pltpu.VMEM((1, 53, 64, 512), u32),
            pltpu.VMEM((2, 7, 2, 2, 64, 128), f32),
            pltpu.VMEM((LAG, 512, 256), u32),
            pltpu.VMEM((LAG, 11 * 64, 256), u32),
            pltpu.VMEM((NA, D, TA), bf16),
            pltpu.VMEM((14, QROWS, 128), f32),
            pltpu.SMEM((1,), i32),
            pltpu.SemaphoreType.DMA((6,)),
            pltpu.SemaphoreType.DMA((4 * LAG,)),
            pltpu.SemaphoreType.DMA((NA + LAG,)),
        ],
        compiler_params=pltpu.CompilerParams(vmem_limit_bytes=116 * 1024 * 1024),
    )(xt, A_wqkv, A_wo, B_w_gate, B_w_up, wdt)
    return out_t.T[None]
```

```python
import functools
import math

import jax
import jax.numpy as jnp
from jax import lax
import jax.experimental.pallas as pl
import jax.experimental.pallas.tpu as pltpu

S, D, F = 2048, 576, 4608
H, DH, W, DIL = 32, 18, 8, 2
NQ = 14 * 128
NH = NQ // 2
HALO = 16
QROWS = S + 2 * HALO + 8
TA = 256
TF = 512
FH = F // 2
LAG = TF // TA
EVERY = (3, 4, 2, 4, 2, 4, 2)
KPOST, DPOST, DLHS = 5, 1, 30
SUB, ELN, EPOST = 3, 1, 2
C1, C2 = (6, 7), (3, 3, 3, 4)
EREM = 5
ED = 2
EV1 = (4, 4, 2, 4, 3, 4, 3)
CL = 0
XN = (4, 4, 3)
XB = (3, 3, 1, 3, 1, 3, 2)
L1 = (8, (3,) * 6 + (8,) * 5 + (1, 1, 1, 1))
EE = (3, 4, 2, 4, 2, 4, 2)
EF = (3, 4, 2, 3, 2, 4, 2)
HD = (22, 6, 1, 0)
LEAD = 2
NCH = 2
RB = 16
NA = S // TA
NSTEP = 2 * NA
EPS = 1e-5
bf16, f32, u32, i32 = jnp.bfloat16, jnp.float32, jnp.uint32, jnp.int32
NT = (((1,), (1,)), ((), ()))
SCALE = DH ** -0.5
EXP2_C = SCALE * math.log2(math.e)
NEG = -1e9 / SCALE

ORD = (0, 2, 3, 1, 4, 5, 6)
SPEC = {1: (1, (0,)), 4: (0, (1,)), 5: (1, (0, 1)), 6: (0, (0, 1))}
SETS = ((0,), (1,), (0, 1))
QSUM = (0, 2, 3, 5, 6)
SIDX = {n: k for k, n in enumerate(SPEC)}

dot = functools.partial(jnp.dot, preferred_element_type=f32)


def dnt(a, b):
    return lax.dot_general(a, b, NT, preferred_element_type=f32)


def cat0(*xs):
    return xs[0] if len(xs) == 1 else jnp.concatenate(xs, axis=0)


def cat1(*xs):
    return xs[0] if len(xs) == 1 else jnp.concatenate(xs, axis=1)


def tb(x):
    return x.T.astype(bf16)


def pkb(x):
    return pltpu.bitcast(x.astype(bf16), u32)


def pkt(x):
    return pltpu.bitcast(tb(x), u32)


def up(x):
    return pltpu.bitcast(x, bf16)


def _chain_sum(load, fn):
    acc = None
    for r in range(0, D, 8 * NCH):
        t = fn(load(r, 8 * NCH))
        acc = t if acc is None else acc + t
    return jnp.sum(acc, axis=0, keepdims=True)


def _ln_t(load, m=None):
    if m is None:
        m = _chain_sum(load, lambda v: v) * (1.0 / D)
    r = lax.rsqrt(_chain_sum(load, lambda v: (v - m) * (v - m)) * (1.0 / D) + EPS)
    return load(0, D) * r - m * r


def _ln_steps(load, m, out):
    st = {}

    def wide(gate, v):
        v = jnp.broadcast_to(v, (16, TA))
        return cat1(gate(v[:, :128]), gate(v[:, 128:]))

    def var(r0, gate):
        mg = wide(gate, m)
        for r in range(r0, r0 + 96, 16):
            d = load(r, 16) - mg
            st["acc"] = d * d if r == 0 else st["acc"] + d * d

    def norm(c, gate):
        if c == 0:
            st["r"] = lax.rsqrt(jnp.sum(st["acc"], axis=0, keepdims=True) * (1.0 / D) + EPS)
            st["mr"] = jnp.broadcast_to(m * st["r"], (16, TA))
        rg = wide(gate, st["r"])
        z = [load(r, 16) * rg - st["mr"] for r in range(128 * c, min(128 * c + 128, D), 16)]
        out[c] = cat0(*(z if c < 4 else z + z)).T

    return [functools.partial(var, r) for r in range(0, D, 96)] + [functools.partial(norm, c) for c in range(5)]


def _prep_wqkv(c, wqkv_ref, wq_ref, cq_ref, t1_ref):
    n = min(256, D - 256 * c)
    wp = pltpu.bitcast(wqkv_ref[256 * c:256 * c + n, :], u32)
    if n < 256:
        wp = cat0(wp, jnp.zeros(((256 - n) // 2, 3 * D), u32))
    t1_ref[c] = wp.T

    def rows(t, d):
        return t1_ref[c, pl.ds(t * D + d, H, stride=DH), :]

    parts = []
    for t in range(3):
        parts += [rows(t, d) for d in (0, 2, 4, 6, 1, 3, 5, 7, 8, 10, 12, 14, 9, 11, 13, 15)]
    parts += [rows(0, 16), rows(0, 17), rows(2, 16), rows(2, 17)]
    parts += [rows(1, 16), rows(1, 17), jnp.zeros((32, 128), u32), jnp.zeros((32, 128), u32)]
    for t in range(7):
        w = [cat0(*parts[4 * k:4 * k + 4]).T[:n // 2] for k in (t, t + 7)]
        for k, v in zip((t, t + 7), w):
            wq_ref[128 * c:128 * c + n // 2, 128 * k:128 * k + 128] = v
        cols = slice(128 * t, 128 * t + 128)
        if c == 2:
            cq_ref[640:, cols] = pkb(unp(w[0]) + unp(w[1]))
        if c == 1:
            for r in range(0, 128, 8):
                ops = rhs7(*[unp(wq_ref[r:r + 8, 128 * k:128 * k + 128]) for k in (t, t + 7)],
                           *[unp(v[r:r + 8]) for v in w])
                for k, m in enumerate(QSUM):
                    cq_ref[128 * k + r:128 * k + r + 8, cols] = pkb(ops[m]())


def _share_lhs(load, rows, dst):
    lo = lax.broadcasted_iota(i32, (16, 128), 1) < 64

    def step(r, gate):
        blk = [[load(q, i, r, gate) for i in range(2)] for q in range(2)]
        for c in range(2):
            ops = [lhs7(b[0][c], b[0][2 + c], b[1][c], b[1][2 + c]) for b in blk]
            for n in range(7):
                x1, x2 = ops[0][n](), ops[1][n]()
                if c == 1 and n in SPEC:
                    r1, r2 = blk[0][SPEC[n][0]][4], blk[1][SPEC[n][0]][4]
                    dst[unit(28 + SIDX[n], rows, r // 2, 8)] = pkb(jnp.where(lo, r1, x2))
                    x1, x2 = jnp.where(lo, x1, x1 - x2), jnp.where(lo, x2, r2 - r1)
                dst[unit(4 * n + c, rows, r // 2, 8)] = pkb(x1)
                dst[unit(4 * n + 2 + c, rows, r // 2, 8)] = pkb(x2)
        return x1

    return [functools.partial(step, r) for r in range(0, 2 * rows, 16)]


def _prep_wo(wo_ref, cw_ref, t2_ref):
    wo = cat1(pltpu.bitcast(wo_ref[...], u32), jnp.zeros((D // 2, 64), u32))
    for c in range(5):
        t2_ref[c] = wo[:, c * 128:(c + 1) * 128]
    wt = []
    for c in range(5):
        wt.append(cat0(*[t2_ref[c, pl.ds(p, H, stride=DH // 2), :] for p in tuple(range(8)) + (8,) * 4]).T)
    wt = cat0(*wt)
    odd = lax.broadcasted_iota(i32, (16, 128), 1) % 64 >= 32

    def load(q, i, r, gate):
        o = 288 * i + 144 * q + r
        out = []
        for c in range(3):
            w = gate(wt[o:o + 16, 128 * c:128 * c + 128])
            out += [pltpu.bitcast(w << 16, f32), pltpu.bitcast(w & jnp.uint32(0xFFFF0000), f32)]
        return out[:4] + [jnp.where(odd, out[5], out[4])]

    return _share_lhs(load, 72, cw_ref)


def _base(s):
    return s % NA * TA if isinstance(s, int) else pl.multiple_of((s % NA) * TA, TA)


def _attn_lhs(s, x_ref, pa):
    item = s % NA
    z = _ln_t(lambda r, n: x_ref[item, r:r + n, :])
    zt = cat0(z, z[512:]).T

    def load(q, i, r, gate):
        o = 128 * q + 64 * i + r
        return [zt[o:o + 16, 128 * c:128 * c + 128] for c in range(5)]

    for st in _share_lhs(load, 32, pa):
        st(None)


def _attn_lhs_steps(s, x_ref, pa):
    item, zt = s % NA, {}
    rows = lambda r, n: x_ref[item, r:r + n, :]

    def load(q, i, r, gate):
        o = 128 * q + 64 * i + r
        return [zt[c][o:o + 16] for c in range(5)]

    return _ln_steps(rows, _chain_sum(rows, lambda v: v) * (1.0 / D), zt) + _share_lhs(load, 32, pa)


def _attn_proj(s, q, sh, pc, pa, wq_ref, cq_ref, qkv_ref):
    item = s % NA
    t0 = _base(s)
    lo = lax.broadcasted_iota(i32, (64, 128), 1) < 64
    for t in range(7):
        def wts(n, r, k):
            c = 128 * t
            if n in QSUM:
                return cq_ref[128 * QSUM.index(n) + r:128 * QSUM.index(n) + r + k, c:c + 128]
            return wq_ref[r:r + k, c:c + 128] if n == 1 else wq_ref[128 + r:128 + r + k, NH + c:NH + c + 128]

        def wrem(n):
            c = 128 * t + (NH if n == 4 else 0)
            return (wq_ref[256:, c:c + 128] if n in (1, 4) else cq_ref[640:, c:c + 128])

        p = [None] * 7
        for n in ORD:
            x = pc.pre(pa[64 * n + 32 * q:64 * n + 32 * q + 32, :])
            if n in SPEC:
                if q == 0:
                    sh[t, n] = dot(up(pa[unit(28 + SIDX[n], 32)]), up(cat0(wrem(n), wts(n, 96, 32))))
                w = cat0(wts(n, 0, 96), wrem(n)) if q else wts(n, 0, 128)
                p[n] = dot(up(x), up(w)) + sh[t, n]
            else:
                p[n] = dot(up(x), up(wts(n, 0, 128)))
            pc.tick(p[n])
        y = out4(p)
        for i in range(2):
            for j in range(2):
                c, v = t + 7 * j, y[i][j]
                if c == 13:
                    v = jnp.where(lo, v, 0.0)
                qkv_ref[c, pl.ds(t0 + (HALO + 128 * q + 64 * i), 64), :] = v
                if q == 0 and i == 0 and c >= 4 and not (isinstance(s, int) and s):
                    hrow = 0 if isinstance(s, int) else pl.multiple_of(jnp.where(item == 0, 0, S + HALO), HALO)
                    qkv_ref[c, pl.ds(hrow, HALO), :] = jnp.broadcast_to(v[0:1], (HALO, 128))


def _attn_core(s, b, qkv_ref, gate):
    t0 = _base(s)
    qi = (0, 1, 2, 3, 12)
    ki = (4, 5, 6, 7, 13)
    vi = (8, 9, 10, 11, 12)
    r0 = t0 + (b * RB + HALO)
    q = [cat0(*[gate(qkv_ref[c, pl.ds(r0 + r, 16), :]) for r in range(0, RB, 16)]) for c in qi]
    ls = []
    for w in range(W):
        acc = None
        for c in range(5):
            t = q[c] * qkv_ref[ki[c], pl.ds(r0 - DIL * w, RB), :]
            acc = t if acc is None else acc + t
        acc = acc + pltpu.roll(acc, 64, 1)
        acc = acc + pltpu.roll(acc, 32, 1)
        if w > 0 and b == 0 and not (isinstance(s, int) and s):
            pos = t0 + lax.broadcasted_iota(i32, (HALO, 128), 0)
            top = jnp.where(pos >= DIL * w, acc[:HALO], NEG)
            acc = top if RB == HALO else cat0(top, acc[HALO:])
        ls.append(acc)
    m = functools.reduce(jnp.maximum, ls)
    pr = [jnp.exp2((l - m) * EXP2_C) for l in ls]
    inv = 1.0 / functools.reduce(jnp.add, pr)
    out = []
    for c in range(5):
        acc = None
        for w in range(W):
            t = pr[w] * qkv_ref[vi[c], pl.ds(r0 - DIL * w, RB), :]
            acc = t if acc is None else acc + t
        out.append(acc * inv)
    return out


def _attn_rhs(b, a0, a1, at):
    lo = lax.broadcasted_iota(i32, (RB, 128), 1) < 64
    rem = (a0[4], a1[4], a0[4] + a1[4])
    rem = [(r, pltpu.roll(r, 64, 1)) for r in rem]
    for c in range(2):
        ops = rhs7(a0[c], a1[c], a0[2 + c], a1[2 + c])
        for n in range(7):
            v = ops[n]()
            at[unit(2 * n + c, 64, b * RB // 2, RB // 2)] = pkb(v)
            if c == 1 and n in SPEC:
                hi, low = rem[SETS.index(SPEC[n][1])]
                at[unit(14 + 2 * SIDX[n], 64, b * RB // 2, RB // 2)] = pkb(jnp.where(lo, v, hi))
                at[unit(15 + 2 * SIDX[n], 64, b * RB // 2, RB // 2)] = pkb(jnp.where(lo, low, v))


def lhs7(a11, a12, a21, a22):
    return (lambda: a11 + a22, lambda: a21 + a22, lambda: a11, lambda: a22,
            lambda: a11 + a12, lambda: a21 - a11, lambda: a12 - a22)


def rhs7(b11, b12, b21, b22):
    return (lambda: b11 + b22, lambda: b11, lambda: b12 - b22, lambda: b21 - b11,
            lambda: b22, lambda: b11 + b12, lambda: b21 + b22)


def out4(m):
    m1, m2, m3, m4, m5, m6, m7 = m
    return [[m1 + m4 - m5 + m7, m3 + m5], [m2 + m4, m1 + m3 - m2 + m6]]


def unit(u, rows, off=0, n=None):
    off = rows * (u // 2) + off
    n = rows if n is None else n
    r = slice(off, off + n) if isinstance(off, int) else pl.ds(pl.multiple_of(off, 8), n)
    return r, slice(128 * (u % 2), 128 * (u % 2) + 128)


def _attn_post(s, pc, at, x_ref, cw_ref, lm_ref):
    item = s % NA
    sh, y = {}, []
    for q in range(2):
        p = [None] * 7
        for n in ORD:
            w = up(cw_ref[144 * n + 72 * q:144 * n + 72 * q + 72, :])
            if n in SPEC:
                if q == 0:
                    sh[n] = dnt(up(cw_ref[unit(28 + SIDX[n], 72)]), up(at[unit(15 + 2 * SIDX[n], 64)]))
                last = at[unit(14 + 2 * SIDX[n] if q else 2 * n + 1, 64)]
                p[n] = dnt(w, up(cat1(at[unit(2 * n, 64)], last))) + sh[n]
            else:
                p[n] = dnt(w, up(at[64 * n:64 * n + 64, :]))
            pc.tick(p[n])
        y.append(out4(p))
    xt = x_ref[item] + cat0(*[cat1(*y[q][i]) for i in range(2) for q in range(2)])
    x_ref[item] = xt
    m = _chain_sum(lambda r, n: xt[r:r + n], lambda v: v) * (1.0 / D)
    zt = {}
    dst = lm_ref.at[(s // LAG) % 2, s % LAG]
    lo = lax.broadcasted_iota(i32, (16, 128), 1) < 64

    def step(r, n, gate):
        def blk(q, i, k):
            o = 64 * i + 32 * q + r
            return zt[k][o:o + 16]

        g11, g22 = (gate, lambda v: v) if n in (0, 2, 4, 5) else (lambda v: v, gate)
        inner = [lhs7(*[lhs7(g11(blk(q, i, k)), blk(q, i, 2 + k), blk(q, 2 + i, k), g22(blk(q, 2 + i, 2 + k)))[n]()
                        for i in range(2) for k in range(2)]) for q in range(2)]
        for l in range(7):
            x1, x2 = inner[0][l](), inner[1][l]()
            if n in SPEC and l in SPEC:
                i = 2 * SPEC[n][0] + SPEC[l][0]
                r1, r2 = blk(0, i, 4), blk(1, i, 4)
                dst[unit(98 + 4 * SIDX[n] + SIDX[l], 16, r // 2, 8)] = pkb(jnp.where(lo, r1, x2))
                x1, x2 = jnp.where(lo, x1, x1 - x2), jnp.where(lo, x2, r2 - r1)
            dst[unit(2 * (7 * n + l), 16, r // 2, 8)] = pkb(x1)
            dst[unit(2 * (7 * n + l) + 1, 16, r // 2, 8)] = pkb(x2)
        return x1

    return (_ln_steps(lambda r, n: x_ref[item, r:r + n, :], m, zt),
            [functools.partial(step, r, n) for r in (0, 16) for n in range(7)])


class Pacer:
    def __init__(self, live):
        self.live, self.todo, self.wait, self.due, self.sub, self.done = live, [], 0, [], 1, []

    def add(self, steps, every, delay=0, lag=0):
        if not self.todo:
            self.wait = delay
        every = every if isinstance(every, tuple) else (every,)
        self.todo += [(st, every[k % len(every)], lag) for k, st in enumerate(steps)]

    def run(self, toks):
        st, self.wait, lag = self.todo.pop(0)
        if lag and len(self.done) >= lag and self.done[-lag] is not None:
            toks = toks + [self.done[-lag]]

        def gate(v):
            if v is None:
                return toks[0]
            for t in toks:
                v = jnp.where(self.live, v, t if v.dtype == t.dtype else pltpu.bitcast(t, v.dtype))
            return v

        self.done.append(st(gate))

    def tick(self, p):
        for k in range(self.sub):
            self.wait -= 1
            if self.todo and self.wait <= 0:
                o = p.shape[0] // self.sub * k
                self.run([p[o:o + 16, :128]])

    def by(self, count, load):
        self.due.append([count, load()])

    def pre(self, w):
        for d in self.due:
            d[0] -= 1
        while self.due and self.due[0][0] <= 0:
            v = jnp.where(self.live[:8], w[:8, :128], self.due.pop(0)[1])
            w = cat0(cat1(v, w[:8, 128:]) if w.shape[1] > 128 else v, w[8:])
        return w

    def flush(self):
        while self.todo:
            self.run([])


def wunit(p, part, off=0, n=32):
    if part == 2:
        p, part = (49, p) if p < 2 else (50 + p % 2, p // 2 - 1)
    return unit(p, 64, 32 * part + off, n)


def _row(ref, r, c, n):
    c = 128 * c if isinstance(c, int) else pl.multiple_of(128 * c, 128)
    r = r if isinstance(r, int) else pl.multiple_of(r, 16)
    v = pltpu.bitcast(ref[pl.ds(r, 16), pl.ds(c, 128 * n)], u32)
    return [v[:, 128 * k:128 * k + 128] for k in range(n)]


def unp(v):
    return up(v).astype(f32)


class Chain:
    def __init__(self, live):
        self.live, self.tok = live, None

    def stage(self, blocks, emit, lead=LEAD):
        tok, self.tok = self.tok, None
        for k, (idx, v) in enumerate(emit([unp(v if tok is None else jnp.where(self.live, v, tok)) for v in blocks])):
            v = pkb(v)
            idx[0][idx[1]] = v
            if k <= lead:
                self.tok = v

    def two_level(self, fn, blk, where):
        quad = lambda a, b: [blk[2 * a + i][2 * b + j] for i in range(2) for j in range(2)]
        got = {}

        def emit(keys, ns, vals):
            for k, key in enumerate(keys):
                got[key] = vals[4 * k:4 * k + 4]
            for n in ns:
                q = [got.get(c, (None,) * 4) for c in ((0, 0), (0, 1), (1, 0), (1, 1))]
                inner = fn(*[fn(*[c[x] for c in q])[n]() for x in range(4)])
                for l in range(7):
                    yield where(7 * n + l), inner[l]()

        plan = ((1, 4, 0), (5, 2), (3, 6)) if fn is rhs7 else ((2, 3, 0), (4, 6), (1, 5))
        return [functools.partial(self.stage, sum((quad(*k) for k in keys), []), functools.partial(emit, keys, ns))
                for keys, ns in zip((((0, 0), (1, 1)), ((0, 1),), ((1, 0),)), plan)]


def _shift(ref, off, most):
    return ref.at[pl.ds(off if isinstance(off, int) else pl.multiple_of(off, 8), ref.shape[0] - most)]


def _combine_proj(half, live, wg_ref, wu_ref, c_ref):
    lo = lax.broadcasted_iota(i32, (8, 128), 1) < 64

    def row(r, tile):
        if tile < 8:
            return _row((wg_ref, wu_ref)[tile % 2], r, 4 * (tile // 2), 4)
        out = []
        for g, u in zip(_row(wg_ref, r, 16, 2), _row(wu_ref, r, 16, 2)):
            w = pltpu.roll(jnp.where(lo, u, g), 64, 1)
            out += [jnp.where(lo, g, w), jnp.where(lo, w, u)]
        return out

    def body(j, carry):
        ch = Chain(live)
        for tile in (0, 8, 1, 2, 3, 4, 5, 6, 7):
            dst = _shift(c_ref.at[half * 9 + tile], 8 * j, 24)

            def emit(r):
                for a, (x, y) in enumerate(((r[0], r[1]), (r[2], r[3]), (r[0] + r[2], r[1] + r[3]))):
                    for b, v in enumerate((x, y, x + y)):
                        yield (dst, wunit(3 * a + b, 2, 0, 8)), v

            for part in range(2):
                blk = [row(128 * k + 64 * part + 16 * j, tile) for k in range(4)]
                for st in ch.two_level(rhs7, blk, lambda p: (dst, wunit(p, part, 0, 8))):
                    st()
            ch.stage(row(512 + 16 * j, tile), emit, 0)
        return carry

    lax.fori_loop(0, 4, body, 0)


def _down_unit(ch, j, w_ref, c, dst):
    dst = _shift(dst, 8 * j, 64)
    blk = [_row(w_ref, 144 * k + 16 * j, c, 4) for k in range(4)]
    return ch.two_level(lhs7, blk, lambda p: (dst, unit(p, 72, 0, 8)))


def _combine_down(half, live, wdt_ref, cd_ref, cr_ref):
    def body(j, carry):
        ch = Chain(live)
        for t in range(4):
            for st in _down_unit(ch, j, wdt_ref, 4 * t, cd_ref.at[1 + half * 4 + t]):
                st()
        dst = _shift(cr_ref.at[half], 8 * j, 64)
        for c in range(2):
            r = 144 * c + 16 * j
            ch.stage(_row(wdt_ref, r, 16, 2) + _row(wdt_ref, 288 + r, 16, 2),
                     lambda a: [((dst, unit(n, 144, 72 * c, 8)), lhs7(*a)[n]()) for n in range(7)])
        return carry

    lax.fori_loop(0, 9, body, 0)


def _proj_pass(lm, w, q, sh, pc):
    def lhs(u):
        return up(pc.pre(cat0(*[lm.at[a][unit(u, 16)] for a in range(LAG)])))

    def wts(a, b):
        return up(cat0(w[wunit(*a)], w[wunit(*b)]))

    def prod(n, l):
        p = 7 * n + l
        if n in SPEC and l in SPEC:
            wr = (3 * SETS.index(SPEC[n][1]) + SETS.index(SPEC[l][1]), 2)
            if q == 0:
                sh[p] = dot(lhs(98 + 4 * SIDX[n] + SIDX[l]), wts(wr, (p, 1)))
            return dot(lhs(2 * p + q), wts((p, 0), wr if q else (p, 1))) + sh[p]
        return dot(lhs(2 * p + q), wts((p, 0), (p, 1)))

    ms = [None] * 7
    for n in ORD:
        p = [None] * 7
        for l in ORD:
            p[l] = prod(n, l)
            pc.tick(p[l])
        ms[n] = out4(p)
    return ms


def _col(ms, ii, ji, jo, rows, gate):
    m1, m2, m3, m4, m5, m6, m7 = [m[ii][ji][rows] for m in ms]
    if jo == 0:
        a = gate(m4)
        return a + m1 - m5 + m7, a + m2
    a = gate(m3)
    return a + m5, a + m1 - m2 + m6


def _mix(a, b):
    lo = lax.broadcasted_iota(i32, a.shape, 1) < 64
    return jnp.where(lo, a, b) * pltpu.roll(jnp.where(lo, b, a), 64, 1)


def _build_steps(mg, mu, t, q, rb, merged=False):
    def form(e, r, blk, k, gate):
        rows = slice(32 * k[1] + r, 32 * k[1] + r + 16)
        blk[k] = []
        for ki in range(2):
            if merged:
                a, b = [_col((mg, mu)[k[0]], e, ji, ki, rows, gate) for ji in range(2)]
                blk[k] += [_mix(a[0], b[0]), _mix(a[1], b[1])]
            else:
                g, u = _col(mg, e, ki, k[0], rows, gate), _col(mu, e, ki, k[0], rows, gate)
                blk[k] += [g[0] * u[0], g[1] * u[1]]

    def emit(e, r, blk, k, n, gate):
        o = 32 * e + 16 * q + r // 2
        quad = [[gate(v) for v in blk[c]] if c == k else blk.get(c, (None,) * 4)
                for c in ((0, 0), (0, 1), (1, 0), (1, 1))]
        inner = rhs7(*[rhs7(*[c[x] for c in quad])[n]() for x in range(4)])
        for l in range(7):
            rb.at[7 * n + l][o:o + 8, 128 * t:128 * t + 128] = pkb(inner[l]())

    def both(e, r, blk, k, n, gate):
        form(e, r, blk, k, gate)
        emit(e, r, blk, k, n, lambda v: v)

    steps = []
    for e in range(2):
        for r in (0, 16):
            blk = {}
            for k, ns in (((0, 0), (1,)), ((1, 1), (4, 0)), ((0, 1), (5, 2)), ((1, 0), (3, 6))):
                steps.append(functools.partial(both, e, r, blk, k, ns[0]))
                steps += [functools.partial(emit, e, r, blk, k, n) for n in ns[1:]]
    return steps


def _rem_steps(ms, q, rb):
    def step(ii, r, gate):
        h = []
        for jo in range(2):
            for item in range(2):
                rows = slice(32 * item + r, 32 * item + r + 16)
                a, b = [_col(ms, ii, ji, jo, rows, gate) for ji in range(2)]
                h.append([_mix(a[io], b[io]) for io in range(2)])
        for io in range(2):
            ops = rhs7(*[v[io] for v in h])
            for n in range(7):
                o, cc = 32 * ii + 16 * q + r // 2, 256 * (n % 2) + 128 * io
                rb.at[49 + n // 2][o:o + 8, cc:cc + 128] = pkb(ops[n]())

    return [functools.partial(step, ii, r) for ii in range(2) for r in (0, 16)]


def _ffn_pos(lm, wa, wb, t, pc, rb):
    sa, sb = {}, {}
    for q in range(2):
        g = _proj_pass(lm, wa, q, sa, pc)
        u = _proj_pass(lm, wb, q, sb, pc)
        pc.add(_build_steps(g, u, t, q, rb), (EVERY, EV1)[q], ED)


def _ffn_down(tile, wts, rhs, rem, pc, x_ref, mid=lambda k: None, put=None):
    ms = [None] * 7

    def rdot(n):
        r = dnt(*rem(n))
        pc.tick(r)
        return r

    def group(n, base):
        if rem and n != ORD[0]:
            base = rdot(n) if base is None else base + rdot(n)
        p = [None] * 7
        for l in ORD:
            p[l] = dnt(up(pc.pre(wts(7 * n + l))), up(rhs(7 * n + l)))
            pc.tick(p[l])
        m1, m2, m3, m4, m5, m6, m7 = p
        if base is None:
            m = out4(p)
        else:
            b = [[base[144 * i:144 * i + 144, 128 * j:128 * j + 128] for j in range(2)] for i in range(2)]
            m = [[b[0][0] + m1 + m4 - m5 + m7, b[0][1] + m3 + m5],
                 [b[1][0] + m4 + m2, b[1][1] + m1 + m3 - m2 + m6]]
        base = cat0(cat1(*m[0]), cat1(*m[1]))
        if rem and n == ORD[0]:
            base = base + rdot(n)
        return base

    def xs(io, a):
        return x_ref.at[tile * LAG + a, 288 * io:288 * io + 288, :]

    def keep(io, a, v):
        xs(io, a)[...] = v

    put = put or keep
    for k, n in enumerate(ORD):
        mid(k)
        if n == 5:
            put(1, 1, group(n, xs(1, 1)[...] + ms[0] + ms[2] - ms[1]))
        elif n == 6:
            put(0, 0, group(n, xs(0, 0)[...] + ms[0] + ms[3] - ms[4]))
        else:
            ms[n] = group(n, None)
            if n == 1:
                put(1, 0, xs(1, 0)[...] + ms[3] + ms[1])
            elif n == 4:
                put(0, 1, xs(0, 1)[...] + ms[2] + ms[4])
    pc.flush()


def _kernel(xt_hbm, wqkv_hbm, wo_hbm, wg_hbm, wu_hbm, wdt_hbm, o_hbm,
            xb_ref, wqkv_ref, wo_ref, wg_ref, wu_ref, wdt_ref, wm_ref,
            cgu_ref, cd_ref, cr_ref, wq_ref, cq_ref, cw_ref, t1_ref, t2_ref, x_ref,
            lm_ref, rb_ref, mb_ref, pa_ref, at_ref, ob_ref, qkv_ref, one_ref, sem_in, sem_w, sem_out):
    def cp_wqkv(c):
        rows = pl.ds(256 * c, min(256, D - 256 * c))
        return pltpu.make_async_copy(wqkv_hbm.at[rows], wqkv_ref.at[rows], sem_in.at[c])

    cp_x0 = pltpu.make_async_copy(xt_hbm.at[:, pl.ds(0, TF)], xb_ref.at[:, pl.ds(0, TF)], sem_in.at[3])
    cp_wo = pltpu.make_async_copy(wo_hbm, wo_ref, sem_in.at[4])
    cp_x1 = pltpu.make_async_copy(xt_hbm.at[:, pl.ds(TF, S - TF)], xb_ref.at[:, pl.ds(TF, S - TF)], sem_in.at[5])

    def cp_w(half, n):
        src, dst = ((wg_hbm, wg_ref), (wu_hbm, wu_ref), (wdt_hbm, wdt_ref))[n]
        return pltpu.make_async_copy(src.at[:, pl.ds(half * FH, FH)], dst, sem_w.at[half * 3 + n])

    def cp_m(half):
        return pltpu.make_async_copy(wdt_hbm.at[:, pl.ds(half * FH + 2048, 256)],
                                     wm_ref.at[:, pl.ds(half * 256, 256)], sem_w.at[3 * LAG + half])

    def cp_out(it):
        o = it * TA
        sl = pl.ds(o if isinstance(o, int) else pl.multiple_of(o, TA), TA)
        return pltpu.make_async_copy(ob_ref.at[it], o_hbm.at[:, sl], sem_out.at[it])

    def flags():
        one = one_ref[0]
        return Pacer(jnp.full((16, 128), one, i32) > 0), one - 1

    nb = TA // 2 // RB

    def cores(s, att, at, blocks):
        def step(b, gate):
            att[b] = _attn_core(s, b, qkv_ref, gate)
            if b >= nb:
                _attn_rhs(b - nb, att[b - nb], att[b], at)
            return att[b][0]
        return [functools.partial(step, b) for b in blocks]

    def first():
        for a in range(LAG):
            x_ref[a] = xb_ref[:, a * TA:(a + 1) * TA].astype(f32)
            _attn_lhs(a, x_ref, pa_ref.at[a])

    cp_wqkv(2).start()
    cp_x0.start()
    cp_wqkv(0).start()
    one_ref[0] = 1
    for m, n in [(0, 0), (0, 1), (0, 4)] + [(1, n) for n in range(7)]:
        mb_ref[m, n] = jnp.full((2, 2, 64, 128), 1.0 if m and n in (2, 3) else 0.0, f32)
    cp_wqkv(2).wait()
    _prep_wqkv(2, wqkv_ref, wq_ref, cq_ref, t1_ref)
    cp_x0.wait()
    cp_wqkv(1).start()
    first()
    cp_wqkv(0).wait()
    cp_wo.start()
    _prep_wqkv(0, wqkv_ref, wq_ref, cq_ref, t1_ref)
    cp_wqkv(1).wait()
    cp_w(0, 0).start()
    _prep_wqkv(1, wqkv_ref, wq_ref, cq_ref, t1_ref)
    cp_wo.wait()
    for n in range(1, 3):
        cp_w(0, n).start()

    def head():
        pc, z = flags()
        sh, att = ({}, {}), ({}, {})
        pc.add(_prep_wo(wo_ref, cw_ref.at[0], t2_ref), 3, HD[0])
        for a in range(LAG):
            for q in range(2):
                _attn_proj(a, q, sh[a], pc, pa_ref.at[a], wq_ref, cq_ref, qkv_ref)
                last = a == 1 and q == 1
                pc.flush()
                pc.add(cores(a, att[a], at_ref.at[a], range(q * nb, (q + 1) * nb)), HD[2] if last else HD[1], 1,
                       HD[3] if a else 0)
        ln, build = _attn_post(0, pc, at_ref.at[0], x_ref, cw_ref.at[z], lm_ref)
        pc.flush()
        pc.sub = SUB
        pc.add(ln, 1)
        pc.add(build, 2, lag=2)
        ln, build = _attn_post(1, pc, at_ref.at[1], x_ref, cw_ref.at[z], lm_ref)
        pc.add(ln, 1)
        pc.add(build, 1, lag=2)
        pc.flush()

    head()
    cp_x1.start()

    def wait_w(f, ns):
        for half in range(LAG):
            @pl.when(f == half)
            def _():
                for n in ns:
                    cp_w(half, n).wait()

    def wait_weights(f):
        @pl.when(f < LAG)
        def _():
            live = jnp.full((8, 128), one_ref[0], i32) > 0
            wait_w(f, (0, 1))
            _combine_proj(f, live, wg_ref, wu_ref, cgu_ref)
            wait_w(f, (2,))
            _combine_down(f, live, wdt_ref, cd_ref, cr_ref)

        @pl.when(f == 0)
        def _():
            cp_x1.wait()
            for n in range(3):
                cp_w(1, n).start()
            for half in range(LAG):
                cp_m(half).start()

            def conv(a, carry):
                x_ref[a] = xb_ref[:, pl.ds(pl.multiple_of(a * TA, TA), TA)].astype(f32)
                return carry

            lax.fori_loop(LAG, NA, conv, 0)

    def emit(it):
        ob_ref[it] = x_ref[it].astype(bf16)
        cp_out(it).start()

    def start_out(f):
        @pl.when(jnp.logical_and(f >= NA, f % LAG == LAG - 1))
        def _():
            for a in range(LAG):
                emit(f - NA - (LAG - 1) + a)

    def fused(s, carry):
        f = s - LAG
        wait_weights(f)
        pc, z = flags()
        half = f % LAG
        lm, rb, rbl = lm_ref.at[(f // LAG) % 2], rb_ref.at[0], rb_ref.at[z]
        pc.add(_attn_lhs_steps(s, x_ref, pa_ref.at[0]), L1[1], L1[0])
        pc.add([lambda gate: pc.by(DLHS, lambda: pa_ref[z, :8, :128])], 1)
        for t in range(4):
            _ffn_pos(lm, cgu_ref.at[half * 9 + 2 * t], cgu_ref.at[half * 9 + 2 * t + 1], t, pc, rb)
        sm, sh, att = {}, {}, {}
        for q in range(2):
            pc.add(_rem_steps(_proj_pass(lm, cgu_ref.at[half * 9 + 8], q, sm, pc), q, rb), EREM)
        _attn_proj(s, 0, sh, pc, pa_ref.at[z], wq_ref, cq_ref, qkv_ref)
        pc.flush()
        pc.add(cores(s, att, at_ref.at[0], range(C1[0])), C1[1], 4, CL)
        _attn_proj(s, 1, sh, pc, pa_ref.at[z], wq_ref, cq_ref, qkv_ref)
        pc.flush()
        pc.add(cores(s, att, at_ref.at[0], range(C1[0], 2 * nb)), C2, 1, CL)

        def mid(k):
            if k == KPOST:
                pc.flush()
                ln, build = _attn_post(s, pc, at_ref.at[z], x_ref, cw_ref.at[0], lm_ref)
                pc.sub = SUB
                pc.add(ln, ELN, DPOST)
                pc.add(build, EPOST)

        def rem(n):
            cc = 256 * (n % 2)
            return (up(cr_ref.at[half][unit(n, 144)]),
                    up(cat0(rbl[49 + n // 2, :, cc:cc + 128], rbl[49 + n // 2, :, cc + 128:cc + 256])))

        _ffn_down((f // LAG) % (S // TF),
                  lambda p: cat1(*[cd_ref.at[1 + half * 4 + t][unit(p, 72)] for t in range(4)]),
                  lambda p: rbl[p], rem, pc, x_ref, mid=mid)
        start_out(f)
        return carry

    lax.fori_loop(LAG, NSTEP, fused, 0)

    last, lm, rb = S // TF - 1, lm_ref.at[(NSTEP // LAG - 1) % 2], rb_ref.at[0]
    for half in range(LAG):
        cp_m(half).wait()
    pc, _ = flags()
    ch = Chain(pc.live[:8])

    def ninth(st, gate):
        ch.tok = pltpu.bitcast(gate(None)[:8], u32)
        st()

    blocks = [(ii, ji) for ii in range(2) for ji in range(2)]
    held = [[[[mb_ref.at[m, n, ii, ji] for ji in range(2)] for ii in range(2)] for n in range(7)] for m in range(2)]
    pc.add([functools.partial(ninth, st) for j in range(9) for st in _down_unit(ch, j, wm_ref, 0, cd_ref.at[0])], XN, 2)
    sa, sb = {}, {}
    pc.add(_build_steps(_proj_pass(lm, cgu_ref.at[8], 0, sa, pc), _proj_pass(lm, cgu_ref.at[17], 0, sb, pc),
                        0, 0, rb, True), XB, 1)

    def hold(ms, ko, ii, ki, r, gate):
        a, b = [_col(ms, ii, ji, ki, slice(r, r + 16), gate) for ji in range(2)]
        h = _mix(a[0], b[0]), _mix(a[1], b[1])
        mb_ref[0, 3 - ko, ii, ki, r:r + 16] = h[1 - ko]
        mb_ref[0, 6 - ko, ii, ki, r:r + 16] = h[ko] - h[1 - ko]
        return a[0]

    for ko, sm in enumerate((sa, sb)):
        ms = _proj_pass(lm, cgu_ref.at[8 + 9 * ko], 1, sm, pc)
        pc.add([functools.partial(hold, ms, ko, ii, ki, r) for ii, ki in blocks for r in range(0, 64, 16)], 2, 1, 4 * ko)
    pc.flush()

    def epi(c, carry):
        pc, z = flags()
        w = 2 * c + c // 4
        sa, sb = {}, {}
        pc.add(_build_steps(*held, 0, 1, rb), EE, 2)
        g, u = _proj_pass(lm, cgu_ref.at[w], 0, sa, pc), _proj_pass(lm, cgu_ref.at[w + 1], 0, sb, pc)
        pc.flush()
        _ffn_down(last, lambda p: cd_ref.at[c][unit(p, 72)], lambda p: rb_ref[z, p, :, :128], None, pc, x_ref)
        pc.add(_build_steps(g, u, 0, 0, rb), EF, 2)
        for m, sm in enumerate((sa, sb)):
            ms = _proj_pass(lm, cgu_ref.at[w + m], 1, sm, pc)
            for n in range(7):
                for ii, ji in blocks:
                    mb_ref[m, n, ii, ji] = ms[n][ii][ji]
        pc.flush()
        return carry

    lax.fori_loop(0, 8, epi, 0)
    pc.add(_build_steps(*held, 0, 1, rb), 1)
    pc.flush()

    def cp_last(io, a):
        it, rows = NA - LAG + a, pl.ds(288 * io, 288)
        return pltpu.make_async_copy(ob_ref.at[it, rows], o_hbm.at[rows, pl.ds(it * TA, TA)],
                                     sem_out.at[it + LAG * io])

    def put(io, a, v):
        ob_ref[NA - LAG + a, 288 * io:288 * io + 288, :] = v.astype(bf16)

    def mid(k):
        if k == 6:
            cp_last(1, 0).start()
            cp_last(0, 1).start()

    _ffn_down(last, lambda p: cd_ref.at[8][unit(p, 72)], lambda p: rb[p, :, :128], None, pc, x_ref, mid, put)
    cp_last(1, 1).start()
    cp_last(0, 0).start()
    for it in range(NA - LAG):
        cp_out(it).wait()
    for io, a in blocks:
        cp_last(io, a).wait()


@jax.jit
def pallas_interleave_layers__sliding_local_dilated__glu_gated_bilinear__prompt_kernel(
    A_x, A_wqkv, A_wo, B_x, B_w_gate, B_w_up, B_w_down):
    xt = A_x[0].T
    wdt = B_w_down.T
    hbm = pl.BlockSpec(memory_space=pl.ANY)
    out_t = pl.pallas_call(
        _kernel,
        in_specs=[hbm] * 6,
        out_specs=hbm,
        out_shape=jax.ShapeDtypeStruct((D, S), bf16),
        scratch_shapes=[
            pltpu.VMEM((D, S), bf16),
            pltpu.VMEM((D, 3 * D), bf16),
            pltpu.VMEM((D, D), bf16),
            pltpu.VMEM((D, FH), bf16),
            pltpu.VMEM((D, FH), bf16),
            pltpu.VMEM((D, FH), bf16),
            pltpu.VMEM((D, 512), bf16),
            pltpu.VMEM((18, 54 * 32, 256), u32),
            pltpu.VMEM((9, 25 * 72 + 8, 256), u32),
            pltpu.VMEM((2, 4 * 144, 256), u32),
            pltpu.VMEM((D // 2, NQ), u32),
            pltpu.VMEM((672, NH), u32),
            pltpu.VMEM((1, 16 * 72, 256), u32),
            pltpu.VMEM((3, 3 * D, 128), u32),
            pltpu.VMEM((5, D // 2, 128), u32),
            pltpu.VMEM((NA, D, TA), f32),
            pltpu.VMEM((2, LAG, 57 * 16, 256), u32),
            pltpu.VMEM((1, 53, 64, 512), u32),
            pltpu.VMEM((2, 7, 2, 2, 64, 128), f32),
            pltpu.VMEM((LAG, 512, 256), u32),
            pltpu.VMEM((LAG, 11 * 64, 256), u32),
            pltpu.VMEM((NA, D, TA), bf16),
            pltpu.VMEM((14, QROWS, 128), f32),
            pltpu.SMEM((1,), i32),
            pltpu.SemaphoreType.DMA((6,)),
            pltpu.SemaphoreType.DMA((4 * LAG,)),
            pltpu.SemaphoreType.DMA((NA + LAG,)),
        ],
        compiler_params=pltpu.CompilerParams(vmem_limit_bytes=116 * 1024 * 1024),
    )(xt, A_wqkv, A_wo, B_w_gate, B_w_up, wdt)
    return out_t.T[None]
```
